```python
import jax
import jax.numpy as jnp

def _softmax(x, axis=-1):
    return jax.nn.softmax(x, axis=axis)
def _gelu(x):
    return jax.nn.gelu(x, approximate=True)
def _silu(x):
    return jax.nn.silu(x)
def _sigmoid(x):
    return jax.nn.sigmoid(x)
def _layernorm(x, axis=-1, eps=1e-5):
    m = jnp.mean(x, axis=axis, keepdims=True)
    v = jnp.var(x, axis=axis, keepdims=True)
    return (x - m) / jnp.sqrt(v + eps)
def _scatter_add(tgt, idx, src, axis=0):
    return tgt.at[idx].add(src)
def _segment_sum(src, seg, n):
    return jax.ops.segment_sum(src, seg, n)
class _Rng:
    def __init__(self, key):
        self._k = key
    def _next(self):
        self._k, sub = jax.random.split(self._k)
        return sub
    def normal(self, shape):
        return jax.random.normal(self._next(), shape, dtype=jnp.bfloat16)
    def randint(self, lo, hi, shape):
        return jax.random.randint(self._next(), shape, lo, hi, dtype=jnp.int32)
    def uniform(self, shape, lo=0.0, hi=1.0):
        return jax.random.uniform(self._next(), shape, jnp.bfloat16, lo, hi)
    def permutation(self, n):
        return jax.random.permutation(self._next(), n)


kernel_name = 'gated_mix__ssm_conv_h3__compressed_kv_cla__prompt'

def setup_inputs():
    _rng = _Rng(jax.random.key(int.from_bytes(__import__("os").urandom(4), "little")))
    _w = (lambda a: (lambda t: t.astype(jnp.bfloat16) if jnp.issubdtype(t.dtype, jnp.floating) else t)(jnp.asarray(a)))
    def _A_setup():
        B, S, D = 1, 2048, 1024
        ks = 4
        return {
            "q": _w((lambda *s: _rng.normal(s) * 0.05)(B, S, D)),
            "k": _w((lambda *s: _rng.normal(s) * 0.05)(B, S, D)),
            "v": _w((lambda *s: _rng.normal(s) * 0.05)(B, S, D)),
            "shift_k": _w((lambda *s: _rng.normal(s) * 0.05)(D, ks) * 0.5),
            "ssm_k": _w((lambda *s: _rng.normal(s) * 0.05)(D, S) * (1.0 / S ** 0.5)),
            "ssm_D": _w((lambda *s: _rng.normal(s) * 0.05)(D)),
        }
    _A_in = _A_setup()

    def _B_setup():
        B, H, Sq, Sk, D, M = 1, 32, 2048, 2048, 128, 1024
        Dc = 4 * D
        return {
            "x": _w((lambda *s: _rng.normal(s) * 0.05)(B, Sq, M)),
            "c_kv": _w((lambda *s: _rng.normal(s) * 0.05)(B, Sk, Dc)),
            "w_q": _w((lambda *s: _rng.normal(s) * 0.05)(M, H, D) * (M ** -0.5)),
            "w_uk": _w((lambda *s: _rng.normal(s) * 0.05)(Dc, H, D) * (Dc ** -0.5)),
            "w_uv": _w((lambda *s: _rng.normal(s) * 0.05)(Dc, H, D) * (Dc ** -0.5)),
            "w_o": _w((lambda *s: _rng.normal(s) * 0.05)(H, D, M) * ((H * D) ** -0.5)),
        }
    _B_in = _B_setup()

    return {
        "A_q": _A_in["q"],
        "A_k": _A_in["k"],
        "A_v": _A_in["v"],
        "A_shift_k": _A_in["shift_k"],
        "A_ssm_k": _A_in["ssm_k"],
        "A_ssm_D": _A_in["ssm_D"],
        "B_x": _B_in["x"],
        "B_c_kv": _B_in["c_kv"],
        "B_w_q": _B_in["w_q"],
        "B_w_uk": _B_in["w_uk"],
        "B_w_uv": _B_in["w_uv"],
        "B_w_o": _B_in["w_o"],
        "gate_w": _w((lambda *s: _rng.normal(s) * 0.05)(1024)),
    }

def reference(A_q, A_k, A_v, A_shift_k, A_ssm_k, A_ssm_D, B_x, B_c_kv, B_w_q, B_w_uk, B_w_uv, B_w_o, gate_w):
    def _A_ref(q, k, v, shift_k, ssm_k, ssm_D):
        B, S, D = q.shape
        ks = shift_k.shape[-1]
        k_pad = jnp.pad(k, ((0, 0), (ks - 1, 0), (0, 0)))
        k_shift = jnp.zeros_like(k)
        for t in range(ks):
            k_shift = k_shift + k_pad[:, t:t + S, :] * shift_k[:, ks - 1 - t][None, None, :]
        kv = k_shift * v
        L = 2 * S
        kv_pad = jnp.pad(kv, ((0, 0), (0, S), (0, 0)))
        kf_pad = jnp.pad(ssm_k, ((0, 0), (0, S)))
        kv_f = (lambda x, axes=(-2,-1): jnp.fft.rfft2(x.astype(jnp.float32), axes=axes))(kv_pad[:, None, :, :], axes=(1, 2))
        kf_f = (lambda x, axes=(-2,-1): jnp.fft.rfft2(x.astype(jnp.float32), axes=axes))(kf_pad[:, None, :], axes=(1, 2))
        kf_f = (lambda x, *d: x.transpose(*d))(kf_f, 1, 2, 0)
        y_f = kv_f * kf_f[None, :, :, :]
        y = (lambda x, s, axes=(-2,-1): jnp.fft.irfft2(x, s=s, axes=axes).astype(jnp.bfloat16))(y_f, (1, L), axes=(1, 2))[:, 0, :S, :]
        y = y + kv * ssm_D[None, None, :]
        return q * y

    def _B_ref(x, c_kv, w_q, w_uk, w_uv, w_o):
        B, Sq, M = x.shape[0], x.shape[1], x.shape[2]
        Sk = c_kv.shape[1]
        H, D = w_q.shape[1], w_q.shape[2]
        q = jnp.einsum("bqm,mhd->bhqd", x, w_q)
        k = jnp.einsum("bkc,chd->bhkd", c_kv, w_uk)
        v = jnp.einsum("bkc,chd->bhkd", c_kv, w_uv)
        scores = jnp.einsum("bhqd,bhkd->bhqk", q, k) * (D ** -0.5)
        off = Sk - Sq
        qi = jnp.arange(Sq)[:, None]
        kj = jnp.arange(Sk)[None, :]
        cmask = kj <= (qi + off)
        scores = jnp.where(cmask[None, None], scores, -1e9)
        p = _softmax(scores, axis=-1)
        ctx = jnp.einsum("bhqk,bhkd->bhqd", p, v)
        return jnp.einsum("bhqd,hdm->bqm", ctx, w_o)

    x = A_q
    g = _sigmoid((x * gate_w).sum(-1, keepdims=True))
    a = _A_ref(x, A_k, A_v, A_shift_k, A_ssm_k, A_ssm_D)
    b = _B_ref(x, B_c_kv, B_w_q, B_w_uk, B_w_uv, B_w_o)
    return g * a + (1 - g) * b
```

```python
import numpy as np
import jax
import jax.numpy as jnp
from jax import lax
import jax.experimental.pallas as pl
import jax.experimental.pallas.tpu as pltpu
import ml_dtypes

S, DM, H, HD, DC, KS = 2048, 1024, 32, 128, 512, 4
C = 128
NCH = S // C
NP = H // 2
NT = DM // 128
BQ = 256
F32, BF16 = jnp.float32, jnp.bfloat16
NTD = (((1,), (1,)), ((), ()))
ORDER = 0

def _dft_consts():
    N = 2 * C
    f = np.arange(C, dtype=np.float64)[:, None] + 0.5
    t = np.arange(C, dtype=np.float64)[None, :]
    ang = 2 * np.pi * f * t / N
    Fm = np.concatenate([np.cos(ang), -np.sin(ang)], 0)
    Gm = np.concatenate([np.cos(ang).T, -np.sin(ang).T], 1) * (2.0 / N)
    return Fm.astype(ml_dtypes.bfloat16), Gm.astype(ml_dtypes.bfloat16)
_F, _G = _dft_consts()

def dot(a, b):
    return jnp.dot(a, b, preferred_element_type=F32)

def dot_nt(a, b):
    return lax.dot_general(a, b, NTD, preferred_element_type=F32)

def unpack_head(w, hh):
    if hh == 0:
        return pltpu.bitcast(w << 16, F32).astype(BF16)
    return pltpu.bitcast(w & jnp.uint32(0xFFFF0000), F32).astype(BF16)

def kernel(gw, shk, ssmd, f_ref, g_ref, aq_hbm, ak_hbm, av_hbm, ssmk_hbm, c_hbm, wq_hbm, wk_hbm, wv_hbm, wo_hbm,
           o_hbm,
           x_s, c_s, wq_b, wk_b, wv_b, q_s, k_s, v_s, ctx_s, gate_s, ak_b, av_b, hk_b, wo_b, o_b, uf, hf, zf, ga_s,
           sem_in, sem_w, sem_t, sem_o):

    def wcopies(p, slot):
        return [pltpu.make_async_copy(src.bitcast(jnp.uint32).at[:, p, :], dst.at[slot], sem_w.at[i, slot])
                for i, (src, dst) in enumerate(((wk_hbm, wk_b), (wv_hbm, wv_b), (wq_hbm, wq_b)))]

    def tcopies(c, slot):
        cs = pl.ds(pl.multiple_of(c * 128, 128), 128)
        return [pltpu.make_async_copy(ak_hbm.at[0, :, cs], ak_b.at[slot], sem_t.at[0, slot]),
                pltpu.make_async_copy(av_hbm.at[0, :, cs], av_b.at[slot], sem_t.at[1, slot]),
                pltpu.make_async_copy(ssmk_hbm.at[cs, :], hk_b.at[slot], sem_t.at[2, slot]),
                pltpu.make_async_copy(wo_hbm.at[:, :, cs], wo_b.at[slot], sem_t.at[3, slot])]

    def ocopy(c, slot):
        cs = pl.ds(pl.multiple_of(c * 128, 128), 128)
        return pltpu.make_async_copy(o_b.at[slot], o_hbm.at[0, :, cs], sem_o.at[slot])

    cp_c = pltpu.make_async_copy(c_hbm.at[0], c_s, sem_in.at[0])
    cp_x = pltpu.make_async_copy(aq_hbm.at[0], x_s, sem_in.at[1])
    cp_c.start()
    w0 = wcopies(0, 0)
    for cp in w0:
        cp.start()
    cp_x.start()
    for cp in wcopies(1, 1):
        cp.start()

    qscale = float((HD ** -0.5) * np.log2(np.e))

    def proj_pieces(slot):
        def kv(dst, wb, hh):
            def f():
                dst[slot, hh] = dot(c_s[...], unpack_head(wb[slot], hh)).astype(BF16)
            return f
        def qq(hh, half):
            def f():
                rs = slice(half * (S // 2), (half + 1) * (S // 2))
                q_s[slot, hh, rs] = (dot(x_s[rs], unpack_head(wq_b[slot], hh)) * qscale).astype(BF16)
            return f
        return ([kv(k_s, wk_b, 0), kv(v_s, wv_b, 0), kv(k_s, wk_b, 1), kv(v_s, wv_b, 1)],
                [qq(0, 0), qq(0, 1), qq(1, 0), qq(1, 1)])

    def attn_unit(p, slot, hh, i, mid):
        L0 = i * BQ
        hb = BQ // 2
        row = lax.broadcasted_iota(jnp.int32, (hb, hb), 0)
        col = lax.broadcasted_iota(jnp.int32, (hb, hb), 1)
        tri = col <= row
        q = q_s[slot, hh, L0:L0 + BQ]
        sa = dot_nt(q, k_s[slot, hh, 0:L0 + hb])
        sb = dot_nt(q[hb:], k_s[slot, hh, L0 + hb:L0 + BQ])
        if mid is not None:
            mid()
        sb = jnp.where(tri, sb, -1e9)
        top = sa[:hb]
        dg = jnp.where(tri, top[:, L0:], -1e9)
        top = dg if i == 0 else jnp.concatenate([top[:, :L0], dg], axis=1)
        bot = jnp.concatenate([sa[hb:], sb], axis=1)
        pt = jnp.exp2(top - jnp.max(top, axis=-1, keepdims=True))
        pb = jnp.exp2(bot - jnp.max(bot, axis=-1, keepdims=True))
        lt = jnp.sum(pt, axis=-1, keepdims=True)
        lb = jnp.sum(pb, axis=-1, keepdims=True)
        pa = jnp.concatenate([pt.astype(BF16), pb[:, :L0 + hb].astype(BF16)], axis=0)
        oa = dot(pa, v_s[slot, hh, 0:L0 + hb])
        ob = dot(pb[:, L0 + hb:].astype(BF16), v_s[slot, hh, L0 + hb:L0 + BQ])
        ls = slice(hh * 128, hh * 128 + 128)
        ctx_s[p, L0:L0 + hb, ls] = (oa[:hb] * (1.0 / lt)).astype(BF16)
        ctx_s[p, L0 + hb:L0 + BQ, ls] = ((oa[hb:] + ob) * (1.0 / lb)).astype(BF16)

    def attention(p, slot, pieces):
        units = [(hh, i) for hh in range(2) for i in range(S // BQ)]
        if ORDER == 1:
            units = [(hh, i) for i in range(S // BQ) for hh in range(2)]
        elif ORDER == 2:
            units = [(hh, i) for i in reversed(range(S // BQ)) for hh in range(2)]
        n = len(units)
        for u, (hh, i) in enumerate(units):
            mid = None
            if pieces and u % 2 == 0:
                mid = pieces[u // 2]
            attn_unit(p, slot, hh, i, mid)

    cp_c.wait()
    w0[0].wait()
    w0[1].wait()
    kvp, qp = proj_pieces(0)
    for f in kvp:
        f()
    w0[2].wait()
    cp_x.wait()
    for f in qp:
        f()
    gwf = gw[...].astype(F32)
    for r in range(NCH):
        rs = slice(r * C, (r + 1) * C)
        gl = jnp.sum(x_s[rs].astype(F32) * gwf, axis=-1, keepdims=True)
        gate_s[rs] = jnp.broadcast_to(jax.nn.sigmoid(gl), (C, 128))

    def pair_step(p, carry):
        slot = p % 2
        for cp in wcopies(p + 1, 1 - slot):
            cp.wait()
        @pl.when(p + 2 < NP)
        def _():
            for cp in wcopies(p + 2, slot):
                cp.start()
        @pl.when(p == NP - 2)
        def _():
            for cp in tcopies(0, 0):
                cp.start()
        kvp, qp = proj_pieces(1 - slot)
        attention(p, slot, kvp + qp)
        return carry
    lax.fori_loop(0, NP - 1, pair_step, 0)
    attention(NP - 1, (NP - 1) % 2, None)

    def tile_step(c, carry):
        slot = c % 2
        for cp in tcopies(c, slot):
            cp.wait()
        @pl.when(c + 1 < NT)
        def _():
            for cp in tcopies(c + 1, 1 - slot):
                cp.start()
        @pl.when(c >= 2)
        def _():
            ocopy(c - 2, slot).wait()
        cs = pl.ds(pl.multiple_of(c * 128, 128), 128)
        acc = [None]
        def oproj(j):
            w = wo_b[slot, 2 * j:2 * j + 2].reshape(256, 128)
            d = dot(ctx_s[j], w)
            acc[0] = d if acc[0] is None else acc[0] + d
        oproj(0)
        kk = ak_b[slot].astype(F32)
        sh = shk[c].astype(F32)
        rows = lax.broadcasted_iota(jnp.int32, (8, 128), 0)
        ksf = kk * sh[0:1, :]
        for j in range(1, KS):
            kr = pltpu.roll(kk, j, 0)
            kr = jnp.concatenate([jnp.where(rows >= j, kr[:8], 0.0), kr[8:]], axis=0)
            ksf = ksf + kr * sh[j:j + 1, :]
        kv = (ksf * av_b[slot].astype(F32)).astype(BF16)
        Fm = f_ref[...]
        for j in range(NCH):
            hf[j] = dot_nt(Fm, hk_b[slot, :, j * C:(j + 1) * C])
        oproj(1)
        for j in range(NCH):
            uf[j] = dot(Fm, kv[j * C:(j + 1) * C])
        ga_s[...] = kv.astype(F32) * ssmd[c].astype(F32)
        oproj(2)
        sgn = (1 - 2 * (rows & 1)).astype(F32)
        nxt = 3
        for ft in range(C // 8):
            re = slice(ft * 8, ft * 8 + 8)
            im = slice(C + ft * 8, C + ft * 8 + 8)
            hc = [hf[0, re]] + [hf[m, re] - sgn * hf[m - 1, im] for m in range(1, NCH)]
            hd = [hf[0, im]] + [hf[m, im] + sgn * hf[m - 1, re] for m in range(1, NCH)]
            ua = [uf[j, re] for j in range(NCH)]
            ub = [uf[j, im] for j in range(NCH)]
            def toep(u, h):
                out = []
                for i in range(NCH):
                    a = u[0] * h[i]
                    for j in range(1, i + 1):
                        a = a + u[j] * h[i - j]
                    out.append(a)
                return out
            k1 = toep([a + b for a, b in zip(ua, ub)], hc)
            k2 = toep(ua, [d - c_ for c_, d in zip(hc, hd)])
            k3 = toep(ub, [d + c_ for c_, d in zip(hc, hd)])
            for i in range(NCH):
                zf[i, re] = k1[i] - k3[i]
                zf[i, im] = k1[i] + k2[i]
            if ft % 4 != 3 and nxt < NP - 1:
                oproj(nxt)
                nxt += 1
        Gm = g_ref[...]
        for i in range(NCH):
            ts = slice(i * C, (i + 1) * C)
            y = dot(Gm, zf[i].astype(BF16)) + ga_s[ts]
            ga_s[ts] = gate_s[ts] * (x_s[ts, cs].astype(F32) * y)
        while nxt < NP:
            oproj(nxt)
            nxt += 1
        o_b[slot] = (ga_s[...] + (1.0 - gate_s[...]) * acc[0]).astype(BF16)
        ocopy(c, slot).start()
        return carry
    lax.fori_loop(0, NT, tile_step, 0)
    ocopy(NT - 2, 0).wait()
    ocopy(NT - 1, 1).wait()

@jax.jit
def pallas_gated_mix__ssm_conv_h3__compressed_kv_cla__prompt_kernel(
        A_q, A_k, A_v, A_shift_k, A_ssm_k, A_ssm_D, B_x, B_c_kv, B_w_q, B_w_uk, B_w_uv, B_w_o, gate_w):
    any_ = pl.BlockSpec(memory_space=pl.ANY)
    vm = pl.BlockSpec(memory_space=pltpu.VMEM)
    out = pl.pallas_call(
        kernel,
        in_specs=[vm] * 5 + [any_] * 9,
        out_specs=any_,
        out_shape=jax.ShapeDtypeStruct((1, S, DM), BF16),
        scratch_shapes=[
            pltpu.VMEM((S, DM), BF16), pltpu.VMEM((S, DC), BF16),
            pltpu.VMEM((2, DM, 128), jnp.uint32), pltpu.VMEM((2, DC, 128), jnp.uint32), pltpu.VMEM((2, DC, 128), jnp.uint32),
            pltpu.VMEM((2, 2, S, 128), BF16), pltpu.VMEM((2, 2, S, 128), BF16), pltpu.VMEM((2, 2, S, 128), BF16),
            pltpu.VMEM((NP, S, 256), BF16),
            pltpu.VMEM((S, 128), F32),
            pltpu.VMEM((2, S, 128), BF16), pltpu.VMEM((2, S, 128), BF16), pltpu.VMEM((2, 128, S), BF16),
            pltpu.VMEM((2, H, HD, 128), BF16), pltpu.VMEM((2, S, 128), BF16),
            pltpu.VMEM((NCH, 2 * C, 128), F32), pltpu.VMEM((NCH, 2 * C, 128), F32), pltpu.VMEM((NCH, 2 * C, 128), F32),
            pltpu.VMEM((S, 128), F32),
            pltpu.SemaphoreType.DMA((2,)), pltpu.SemaphoreType.DMA((3, 2)), pltpu.SemaphoreType.DMA((4, 2)),
            pltpu.SemaphoreType.DMA((2,)),
        ],
        compiler_params=pltpu.CompilerParams(vmem_limit_bytes=110 * 1024 * 1024),
    )(gate_w.reshape(1, DM), A_shift_k.T.reshape(KS, NT, 128).transpose(1, 0, 2), A_ssm_D.reshape(NT, 1, 128), _F, _G,
      A_q, A_k, A_v, A_ssm_k, B_c_kv, B_w_q, B_w_uk, B_w_uv, B_w_o)
    return out
```

```python
import numpy as np
import jax
import jax.numpy as jnp
from jax import lax
import jax.experimental.pallas as pl
import jax.experimental.pallas.tpu as pltpu
import ml_dtypes

S, DM, H, HD, DC, KS = 2048, 1024, 32, 128, 512, 4
C = 128
NCH = S // C
NP = H // 2
NT = DM // 128
HS = S // 2
F32, BF16, U32 = jnp.float32, jnp.bfloat16, jnp.uint32
NTD = (((1,), (1,)), ((), ()))

BQ = 128
NG = HS // BQ
A_TMP = 0
A_CT = A_TMP + S + 4 * BQ
A_END = A_CT + 7 * NP * (HS // 2)
ONLY1 = 0
ONLY2 = 0
OR = 128
GT = 1
LAG = 0
REV = 0
CLAG = 0
TOK0 = 0
SL0 = (1,2,3,4,5,7,9,10,12,13)
SL1 = (0,2,4,16)

def _dft_consts():
    N = 2 * C
    f = np.arange(C, dtype=np.float64)[:, None] + 0.5
    t = np.arange(C, dtype=np.float64)[None, :]
    ang = 2 * np.pi * f * t / N
    Fm = np.concatenate([np.cos(ang), -np.sin(ang)], 0)
    Gm = np.concatenate([np.cos(ang).T, -np.sin(ang).T], 1) * (2.0 / N)
    return Fm.astype(ml_dtypes.bfloat16), Gm.astype(ml_dtypes.bfloat16)
_F, _G = _dft_consts()

def dot(a, b):
    return jnp.dot(a, b, preferred_element_type=F32)

def dot_nt(a, b):
    return lax.dot_general(a, b, NTD, preferred_element_type=F32)

def pack(x):
    return pltpu.bitcast(x.astype(BF16), U32)

def unpack(w):
    return pltpu.bitcast(w, BF16)

def halves(w):
    return pltpu.bitcast(w << 16, F32), pltpu.bitcast(w & jnp.uint32(0xFFFF0000), F32)

def lhs_ops(a11, a12, a21, a22):
    return [lambda: a11() + a22(), lambda: a21() + a22(), a11, a22,
            lambda: a11() + a12(), lambda: a21() - a11(), lambda: a12() - a22()]

def rhs_ops(b11, b12, b21, b22):
    return [lambda: b11() + b22(), b11, lambda: b12() - b22(), lambda: b21() - b11(),
            b22, lambda: b11() + b12(), lambda: b21() + b22()]

PORD = (2, 4, 1, 0, 5, 3, 6)
SKIP = (4, 10, 16)

def strassen_steps(prod, emit, m, dyn):
    def step(i):
        def f():
            v = prod(i)
            if i == 2:
                m[0 + dyn] = v
            elif i == 4:
                emit(0, 1, m[0] + v)
                m[1 + dyn] = v
            elif i == 1:
                m[2 + dyn] = v
            elif i == 0:
                m[3 + dyn] = v
            elif i == 5:
                emit(1, 1, (m[0] - m[2]) + (m[3] + v))
            elif i == 3:
                emit(1, 0, m[2] + v)
                m[0 + dyn] = v
            else:
                emit(0, 0, (m[3] - m[1]) + (m[0] + v))
        return f
    return [step(i) for i in PORD]

def kernel(gw, shk, ssmd, f_ref, g_ref, aq_hbm, ak_hbm, av_hbm, ssmk_hbm, c_hbm, wq_hbm, wk_hbm, wv_hbm, wo_hbm,
           o_hbm,
           x_s, c_s, xab, cab, wq_b, wk_b, wv_b, h0b, h1b, arb, s0, s1, mkv, mq, gate_s, ak_b, av_b, hk_b, wo_b, o_b, uf, hf, zf, ga_s,
           sem_x, sem_w, sem_t, sem_o):

    def wcopies(p, slot):
        return [pltpu.make_async_copy(src.bitcast(U32).at[:, p, :], dst.at[slot], sem_w.at[i, slot])
                for i, (src, dst) in enumerate(((wk_hbm, wk_b), (wv_hbm, wv_b), (wq_hbm, wq_b)))]

    def tcopies(t, slot):
        cs = pl.ds(pl.multiple_of(t * 256, 256), 256)
        return [pltpu.make_async_copy(ak_hbm.at[0, :, cs], ak_b.at[slot], sem_t.at[0, slot]),
                pltpu.make_async_copy(av_hbm.at[0, :, cs], av_b.at[slot], sem_t.at[1, slot]),
                pltpu.make_async_copy(ssmk_hbm.at[cs, :], hk_b.at[slot], sem_t.at[2, slot]),
                pltpu.make_async_copy(wo_hbm.at[:, :, cs], wo_b.at[slot], sem_t.at[3, slot])]

    def ocopy(t, slot):
        cs = pl.ds(pl.multiple_of(t * 256, 256), 256)
        return pltpu.make_async_copy(o_b.at[slot], o_hbm.at[0, :, cs], sem_o.at[slot])

    RB = 256
    def rcopies(src, dst, which, r):
        rows = lambda a: pl.ds(pl.multiple_of(a * HS + r * RB, RB), RB)
        return [pltpu.make_async_copy(src.at[0, rows(a)], dst.at[rows(a)], sem_x.at[which, a, r]) for a in range(2)]
    ccopies = lambda r: rcopies(c_hbm, c_s, 0, r)
    xcopies = lambda r: rcopies(aq_hbm, x_s, 1, r)
    w0 = wcopies(0, 0)
    for cp in w0[:2] + ccopies(0):
        cp.start()

    qscale = float((HD ** -0.5) * np.log2(np.e))

    ar, xa, ca = arb.bitcast(U32), xab.bitcast(U32), cab.bitcast(U32)
    h0, h1 = h0b.bitcast(U32), h1b.bitcast(U32)

    def qkv_load(slot, which, hh, r0, n):
        rs = slice(r0 // 2, (r0 + n) // 2)
        return h0[which, rs] if hh == 0 else h1[slot, which, rs]

    def qkv_store(slot, which, hh, r0, val):
        rs = pl.ds(pl.multiple_of(r0, 128), val.shape[0])
        if hh == 0:
            h0b[which, rs] = val.astype(BF16)
        else:
            h1b[slot, which, rs] = val.astype(BF16)

    def proj_pieces(slot, dyn, r0=0, n=HS):
        def wblk(refs, r, c):
            def f():
                k2 = refs[0].shape[1] // 2
                parts = [halves(ref[slot, r * k2:(r + 1) * k2])[c] for ref in refs]
                return parts[0] if len(parts) == 1 else jnp.concatenate(parts, axis=1)
            return f
        def mk(refs, lhs, emit, m):
            rops = rhs_ops(wblk(refs, 0, 0), wblk(refs, 0, 1), wblk(refs, 1, 0), wblk(refs, 1, 1))
            rs = pl.ds(pl.multiple_of(r0 // 2, 64), n // 2)
            return strassen_steps(lambda i: dot(unpack(lhs[i, rs]), rops[i]().astype(BF16)), emit, m.at[:, 0:n], dyn)
        def emit_kv(r, c, val):
            qkv_store(slot, 1, c, r * HS + r0, val[:, :128])
            for t in range(0, n, 128):
                qkv_store(slot, 2, c, r * HS + r0 + t, val[t:t + 128, 128:].T)
        def emit_q(r, c, val):
            qkv_store(slot, 0, c, r * HS + r0, val * qscale)
        return mk((wk_b, wv_b), ca, emit_kv, mkv), mk((wq_b,), xa, emit_q, mq)

    def scores(slot, hh, i, buf, dyn):
        L = (i + 1) * BQ
        q = unpack(qkv_load(slot, 0, hh, i * BQ, BQ))
        m = None
        n = L // 4
        for a in range(4):
            st = dot_nt(unpack(qkv_load(slot, 1, hh, a * n, n)), q)
            d0 = max(L - BQ - a * n, 0)
            if d0 < n:
                row = lax.broadcasted_iota(jnp.int32, (n - d0, BQ), 0) + (a * n + d0 - (L - BQ))
                col = lax.broadcasted_iota(jnp.int32, (n - d0, BQ), 1)
                dg = jnp.where(row <= col, st[d0:], -1e9)
                st = dg if d0 == 0 else jnp.concatenate([st[:d0], dg], axis=0)
            (s0, s1)[buf][pl.ds(pl.multiple_of(a * n + dyn, 32), n)] = st
            ma = jnp.max(st.reshape(n // 8, 8, BQ), axis=0)
            m = ma if m is None else jnp.maximum(m, ma)
        return jnp.broadcast_to(jnp.max(m, axis=0, keepdims=True), (8, BQ))

    def weighted(slot, hh, i, buf, m, never, dyn2):
        l = ot = None
        for t0 in range(0, i + 1, GT):
            nt = min(GT, i + 1 - t0)
            pj = jnp.exp2((s0, s1)[buf][t0 * BQ:(t0 + nt) * BQ] - jnp.tile(m, (nt * BQ // 8, 1)))
            lj = jnp.sum(pj.reshape(nt * BQ // 8, 8, BQ), axis=0)
            if LAG and l is not None:
                pj = jnp.concatenate([jnp.where(never, l, pj[:8]), pj[8:]], axis=0)
            l = lj if l is None else l + lj
            pt = pj.astype(BF16)
            ns = 1 if nt == 4 else 2 if nt == 2 else 4
            parts = []
            for a in range(ns):
                vt = jnp.concatenate([qkv_load(slot, 2, hh, t * 128 + a * HD // ns, HD // ns)
                                      for t in range(t0, t0 + nt)], axis=1)
                parts.append(dot(unpack(vt), pt))
            d = jnp.concatenate(parts, axis=0)
            ot = d if ot is None else ot + d
        l = jnp.sum(l, axis=0, keepdims=True)
        r = pl.reciprocal(l, approx=True)
        r = r * (2.0 - l * r)
        return (ot * r).T

    def attention(p, slot, pieces):
        pieces = list(pieces)
        dyn = lax.shift_right_logical(p, 8)
        never = jnp.broadcast_to(p, (8, BQ)) < 0
        dyn2 = lax.shift_right_logical(p, 9)
        tmp = lambda i: pl.ds(pl.multiple_of(A_TMP + i * BQ + dyn, 64), BQ)
        gs = lambda hh: range(NG) if not (REV >> hh) & 1 else reversed(range(NG))
        units = [(hh, g + a * NG) for hh in range(2) for g in gs(hh) for a in range(2)]
        slot1 = lambda i: 2 * NG + (i % 2) * 2 + i // NG

        nxt = scores(slot, *units[0], 0, dyn)
        tok = {}
        for u, (hh, i) in enumerate(units):
            cur = nxt
            if u + 1 < len(units):
                nxt = scores(slot, *units[u + 1], (u + 1) % 2, dyn)
            if pieces and (u in SL0 or u - 2 * NG in SL1):
                pieces.pop(0)()
            if u in tok:
                cur = jnp.where(never, tok[u], cur)
            o = weighted(slot, hh, i, u % 2, cur, never, dyn2)
            if hh == 0 or i < NG:
                ar[tmp(i if hh == 0 else slot1(i))] = pltpu.bitcast(o, U32)
            else:
                g = i - NG
                ld = lambda t: (lambda: pltpu.bitcast(ar[tmp(t)], F32))
                for j, op in enumerate(lhs_ops(ld(g), ld(slot1(g)), ld(i), lambda: o)):
                    base = A_CT + (j * NP + p) * (HS // 2) + g * (BQ // 2)
                    arb[pl.ds(pl.multiple_of(base * 2, 64), BQ)] = op().astype(BF16)
            if CLAG and (hh == 1 and i >= NG or TOK0 and u % 2):
                tok[u + CLAG] = pltpu.bitcast(ar[pl.ds(pl.multiple_of(A_TMP + dyn2, 8), 8)], F32)
        while pieces:
            pieces.pop(0)()

    def combos(src, dst, r0, n, gate):
        k2 = src.shape[1] // 2
        top, bot = (src[pl.ds(pl.multiple_of(a * HS + r0, n), n)].astype(F32) for a in range(2))
        ops = lhs_ops(lambda: top[:, :k2], lambda: top[:, k2:], lambda: bot[:, :k2], lambda: bot[:, k2:])
        for j, op in enumerate(ops):
            dst[j, pl.ds(pl.multiple_of(r0, n), n)] = op().astype(BF16)
        if gate:
            for a, v in enumerate((top, bot)):
                gl = jnp.sum(v * gw[...].astype(F32), axis=-1, keepdims=True)
                gate_s[pl.ds(pl.multiple_of(a * HS + r0, n), n)] = jnp.broadcast_to(jax.nn.sigmoid(gl), (n, 128))

    NC = HS // RB
    for cp in w0[:2]:
        cp.wait()
    for cp in xcopies(0) + w0[2:]:
        cp.start()
    def pro_step(r, carry):
        r0 = r * RB
        both = lambda ref: unpack(jnp.concatenate(
            [ref.bitcast(U32)[pl.ds(pl.multiple_of((a * HS + r0) // 2, RB // 2), RB // 2)] for a in range(2)], axis=0))
        for cp in ccopies(r):
            cp.wait()
        @pl.when(r + 1 < NC)
        def _():
            for cp in ccopies(r + 1) + xcopies(r + 1):
                cp.start()
        @pl.when(r + 1 == NC)
        def _():
            for cp in wcopies(1, 1):
                cp.start()
        for which, wb in ((1, wk_b), (2, wv_b)):
            val = dot(both(c_s), jnp.concatenate(halves(wb[0]), axis=1).astype(BF16))
            for hh in range(2):
                for t in range(0, 2 * RB, 128):
                    blk = val[t:t + 128, hh * 128:(hh + 1) * 128]
                    qkv_store(0, which, hh, t // RB * HS + r0 + t % RB, blk if which == 1 else blk.T)
        for a in range(0, RB, 32):
            combos(c_s, cab, r0 + a, 32, False)
        for cp in xcopies(r):
            cp.wait()
        @pl.when(r == 0)
        def _():
            w0[2].wait()
        val = dot(both(x_s), jnp.concatenate(halves(wq_b[0]), axis=1).astype(BF16)) * qscale
        for hh in range(2):
            for a in range(2):
                qkv_store(0, 0, hh, a * HS + r0, val[a * RB:(a + 1) * RB, hh * 128:(hh + 1) * 128])
        for a in range(0, RB, 16):
            combos(x_s, xab, r0 + a, 16, True)
        return carry
    lax.fori_loop(0, NC, pro_step, 0)

    def pair_step(p, carry):
        slot = p % 2
        for cp in wcopies(p + 1, 1 - slot):
            cp.wait()
        @pl.when(p + 2 < NP)
        def _():
            for cp in wcopies(p + 2, slot):
                cp.start()
        @pl.when(p == NP - 2)
        def _():
            for cp in tcopies(0, 0):
                cp.start()
        kvp, qp = proj_pieces(1 - slot, lax.shift_right_logical(p, 8))
        attention(p, slot, [f for pair in zip(kvp, qp) for f in pair])
        return carry + 1
    last = lax.fori_loop(0, NP - 1, pair_step, 0) if not ONLY2 else None
    if ONLY1:
        return
    if not ONLY2:
        attention(last, (NP - 1) % 2, [])

    def tile_step(t, carry):
        slot = t % 2
        for cp in tcopies(t, slot):
            cp.wait()
        @pl.when(t + 1 < NT // 2)
        def _():
            for cp in tcopies(t + 1, 1 - slot):
                cp.start()
        @pl.when(t >= 2)
        def _():
            ocopy(t - 2, slot).wait()

        KC = 4
        def oprod(i):
            acc = None
            for j0 in range(0, NP, KC):
                def wblk(r, c):
                    return lambda: jnp.concatenate(
                        [wo_b[slot, 2 * j + r, :, c * 128:(c + 1) * 128] for j in range(j0, j0 + KC)], axis=0).astype(F32)
                w = rhs_ops(wblk(0, 0), wblk(0, 1), wblk(1, 0), wblk(1, 1))[i]().astype(BF16)
                a = jnp.concatenate([ar[pl.ds(A_CT + (i * NP + j) * (HS // 2), HS // 2)] for j in range(j0, j0 + KC)], axis=1)
                d = dot(unpack(a), w)
                acc = d if acc is None else acc + d
                yield acc
        def emit_o(r, c, val):
            rs = slice(r * HS, (r + 1) * HS)
            cs = slice(c * 128, (c + 1) * 128)
            o_b[slot, rs, cs] = (ga_s[c, rs] + (1.0 - gate_s[rs]) * val).astype(BF16)
        def opieces():
            m = {}
            for i in PORD:
                for acc in oprod(i):
                    m[i] = acc
                    yield
            yield
            emit_o(0, 1, m[2] + m[4])
            emit_o(1, 0, m[1] + m[3])
            emit_o(0, 0, (m[0] + m[6]) + (m[3] - m[4]))
            emit_o(1, 1, (m[0] + m[5]) + (m[2] - m[1]))
            yield
        gen = opieces()
        def piece(n=1):
            for _ in range(n):
                next(gen)

        rows = lax.broadcasted_iota(jnp.int32, (8, 128), 0)
        sgn = (1 - 2 * (rows & 1)).astype(F32)
        Fm = f_ref[...]
        Gm = g_ref[...]
        for c in range(2):
            cs = slice(c * 128, (c + 1) * 128)
            piece()
            kk = ak_b[slot, :, cs].astype(F32)
            sh = shk[2 * t + c].astype(F32)
            ksf = kk * sh[0:1, :]
            for j in range(1, KS):
                kr = pltpu.roll(kk, j, 0)
                kr = jnp.concatenate([jnp.where(rows >= j, kr[:8], 0.0), kr[8:]], axis=0)
                ksf = ksf + kr * sh[j:j + 1, :]
            kv = (ksf * av_b[slot, :, cs].astype(F32)).astype(BF16)
            for j in range(0, NCH, 4):
                r = dot_nt(Fm, jnp.concatenate([hk_b[slot, cs, (j + a) * C:(j + a + 1) * C] for a in range(4)], axis=0))
                for a in range(4):
                    hf[j + a] = r[:, a * 128:(a + 1) * 128]
            piece()
            for j in range(0, NCH, 4):
                r = dot(Fm, jnp.concatenate([kv[(j + a) * C:(j + a + 1) * C] for a in range(4)], axis=1))
                for a in range(4):
                    uf[j + a] = r[:, a * 128:(a + 1) * 128]
            ga_s[c] = kv.astype(F32) * ssmd[2 * t + c].astype(F32)
            piece()
            for ft in range(C // 8):
                re = slice(ft * 8, ft * 8 + 8)
                im = slice(C + ft * 8, C + ft * 8 + 8)
                hc = [hf[0, re]] + [hf[m, re] - sgn * hf[m - 1, im] for m in range(1, NCH)]
                hd = [hf[0, im]] + [hf[m, im] + sgn * hf[m - 1, re] for m in range(1, NCH)]
                ua = [uf[j, re] for j in range(NCH)]
                ub = [uf[j, im] for j in range(NCH)]
                def toep(u, h):
                    out = []
                    for i in range(NCH):
                        a = u[0] * h[i]
                        for j in range(1, i + 1):
                            a = a + u[j] * h[i - j]
                        out.append(a)
                    return out
                k1 = toep([a + b for a, b in zip(ua, ub)], hc)
                k2 = toep(ua, [d - c_ for c_, d in zip(hc, hd)])
                k3 = toep(ub, [d + c_ for c_, d in zip(hc, hd)])
                for i in range(NCH):
                    zf[i, re] = k1[i] - k3[i]
                    zf[i, im] = k1[i] + k2[i]
                if ft % 8 not in (0, 3, 6):
                    piece()
            xcs = pl.ds(pl.multiple_of((2 * t + c) * 128, 128), 128)
            for j in range(0, NCH, 4):
                r = dot(Gm, jnp.concatenate([zf[j + a] for a in range(4)], axis=1).astype(BF16))
                for a in range(4):
                    ts = slice((j + a) * C, (j + a + 1) * C)
                    y = r[:, a * 128:(a + 1) * 128] + ga_s[c, ts]
                    ga_s[c, ts] = gate_s[ts] * (x_s[ts, xcs].astype(F32) * y)
                if j == 4:
                    piece()
        piece(2)
        ocopy(t, slot).start()
        return carry
    lax.fori_loop(0, NT // 2, tile_step, 0)
    ocopy(NT // 2 - 2, 0).wait()
    ocopy(NT // 2 - 1, 1).wait()

@jax.jit
def pallas_gated_mix__ssm_conv_h3__compressed_kv_cla__prompt_kernel(
        A_q, A_k, A_v, A_shift_k, A_ssm_k, A_ssm_D, B_x, B_c_kv, B_w_q, B_w_uk, B_w_uv, B_w_o, gate_w):
    any_ = pl.BlockSpec(memory_space=pl.ANY)
    vm = pl.BlockSpec(memory_space=pltpu.VMEM)
    out = pl.pallas_call(
        kernel,
        in_specs=[vm] * 5 + [any_] * 9,
        out_specs=any_,
        out_shape=jax.ShapeDtypeStruct((1, S, DM), BF16),
        scratch_shapes=[
            pltpu.VMEM((S, DM), BF16), pltpu.VMEM((S, DC), BF16),
            pltpu.VMEM((7, HS, DM // 2), BF16), pltpu.VMEM((7, HS, DC // 2), BF16),
            pltpu.VMEM((2, DM, 128), U32), pltpu.VMEM((2, DC, 128), U32), pltpu.VMEM((2, DC, 128), U32),
            pltpu.VMEM((3, S, 128), BF16), pltpu.VMEM((2, 3, S, 128), BF16), pltpu.VMEM((2 * A_END, 128), BF16),
            pltpu.VMEM((S, 128), F32), pltpu.VMEM((S, 128), F32), pltpu.VMEM((4, HS, 256), F32), pltpu.VMEM((4, HS, 128), F32),
            pltpu.VMEM((S, 128), F32),
            pltpu.VMEM((2, S, 256), BF16), pltpu.VMEM((2, S, 256), BF16), pltpu.VMEM((2, 256, S), BF16),
            pltpu.VMEM((2, H, HD, 256), BF16), pltpu.VMEM((2, S, 256), BF16),
            pltpu.VMEM((NCH, 2 * C, 128), F32), pltpu.VMEM((NCH, 2 * C, 128), F32), pltpu.VMEM((NCH, 2 * C, 128), F32),
            pltpu.VMEM((2, S, 128), F32),
            pltpu.SemaphoreType.DMA((2, 2, 4)), pltpu.SemaphoreType.DMA((3, 2)), pltpu.SemaphoreType.DMA((4, 2)),
            pltpu.SemaphoreType.DMA((2,)),
        ],
        compiler_params=pltpu.CompilerParams(vmem_limit_bytes=120 * 1024 * 1024),
    )(gate_w.reshape(1, DM), A_shift_k.T.reshape(KS, NT, 128).transpose(1, 0, 2), A_ssm_D.reshape(NT, 1, 128), _F, _G,
      A_q, A_k, A_v, A_ssm_k, B_c_kv, B_w_q, B_w_uk, B_w_uv, B_w_o)
    return out
```

```python
import numpy as np
import jax
import jax.numpy as jnp
from jax import lax
import jax.experimental.pallas as pl
import jax.experimental.pallas.tpu as pltpu
import ml_dtypes

S, DM, H, HD, DC, KS = 2048, 1024, 32, 128, 512, 4
C = 128
NCH = S // C
NP = H // 2
NT = DM // 128
HS = S // 2
QS = S // 4
F32, BF16, U32 = jnp.float32, jnp.bfloat16, jnp.uint32
NTD = (((1,), (1,)), ((), ()))

BQ = 128
NG = HS // BQ
A_TMP = 0
A_CT = A_TMP + S + 4 * BQ
A_END = A_CT + 7 * NP * (HS // 2)
ONLY1 = 0
ONLY2 = 0
OR = 128
GT = 1
LAG = 0
REV = 0
CLAG = 0
TOK0 = 0
SPL = 0
CCH = 32
SL0 = (1,2,3,4,5,7,9,10,12,13)
SL1 = (0,2,4,16)

def _dft_consts():
    N = 2 * C
    f = np.arange(C, dtype=np.float64)[:, None] + 0.5
    t = np.arange(C, dtype=np.float64)[None, :]
    ang = 2 * np.pi * f * t / N
    Fm = np.concatenate([np.cos(ang), -np.sin(ang)], 0)
    Gm = np.concatenate([np.cos(ang).T, -np.sin(ang).T], 1) * (2.0 / N)
    return Fm.astype(ml_dtypes.bfloat16), Gm.astype(ml_dtypes.bfloat16)
_F, _G = _dft_consts()

def dot(a, b):
    return jnp.dot(a, b, preferred_element_type=F32)

def dot_nt(a, b):
    return lax.dot_general(a, b, NTD, preferred_element_type=F32)

def pack(x):
    return pltpu.bitcast(x.astype(BF16), U32)

def unpack(w):
    return pltpu.bitcast(w, BF16)

def halves(w):
    return pltpu.bitcast(w << 16, F32), pltpu.bitcast(w & jnp.uint32(0xFFFF0000), F32)

def lhs_ops(a11, a12, a21, a22):
    return [lambda: a11() + a22(), lambda: a21() + a22(), a11, a22,
            lambda: a11() + a12(), lambda: a21() - a11(), lambda: a12() - a22()]

def rhs_ops(b11, b12, b21, b22):
    return [lambda: b11() + b22(), b11, lambda: b12() - b22(), lambda: b21() - b11(),
            b22, lambda: b11() + b12(), lambda: b21() + b22()]

PORD = (2, 4, 1, 0, 5, 3, 6)
SKIP = (4, 10, 16)

def consume(i, v, emit, m, dyn):
    if i == 2:
        m[0 + dyn] = v
    elif i == 4:
        emit(0, 1, m[0] + v)
        m[1 + dyn] = v
    elif i == 1:
        m[2 + dyn] = v
    elif i == 0:
        m[3 + dyn] = v
    elif i == 5:
        emit(1, 1, (m[0] - m[2]) + (m[3] + v))
    elif i == 3:
        emit(1, 0, m[2] + v)
        m[0 + dyn] = v
    else:
        emit(0, 0, (m[3] - m[1]) + (m[0] + v))

def kernel(gw, shk, ssmd, f_ref, g_ref, aq_hbm, ak_hbm, av_hbm, ssmk_hbm, c_hbm, wq_hbm, wk_hbm, wv_hbm, wo_hbm,
           o_hbm,
           x_s, c_s, xab, cab, wq_b, wk_b, wv_b, h0b, h1b, arb, s0, s1, mkv, mi, mq, gate_s, ak_b, av_b, hk_b, wo_b, o_b, uf, hf, zf, ga_s, dd_s,
           sem_x, sem_w, sem_t, sem_o):

    def wcopies(p, slot):
        return [pltpu.make_async_copy(src.bitcast(U32).at[:, p, :], dst.at[slot], sem_w.at[i, slot])
                for i, (src, dst) in enumerate(((wk_hbm, wk_b), (wv_hbm, wv_b), (wq_hbm, wq_b)))]

    def tcopies(t, slot):
        cs = pl.ds(pl.multiple_of(t * 256, 256), 256)
        return [pltpu.make_async_copy(ak_hbm.at[0, :, cs], ak_b.at[slot], sem_t.at[0, slot]),
                pltpu.make_async_copy(av_hbm.at[0, :, cs], av_b.at[slot], sem_t.at[1, slot]),
                pltpu.make_async_copy(ssmk_hbm.at[cs, :], hk_b.at[slot], sem_t.at[2, slot]),
                pltpu.make_async_copy(wo_hbm.at[:, :, cs], wo_b.at[slot], sem_t.at[3, slot])]

    def ocopy(t, slot):
        cs = pl.ds(pl.multiple_of(t * 256, 256), 256)
        return pltpu.make_async_copy(o_b.at[slot], o_hbm.at[0, :, cs], sem_o.at[slot])

    RB = 128
    def rcopies(src, dst, which, r):
        rows = lambda a: pl.ds(pl.multiple_of(a * QS + r * RB, RB), RB)
        return [pltpu.make_async_copy(src.at[0, rows(a)], dst.at[rows(a)], sem_x.at[which, a, r]) for a in range(4)]
    ccopies = lambda r: rcopies(c_hbm, c_s, 0, r)
    xcopies = lambda r: rcopies(aq_hbm, x_s, 1, r)
    w0 = wcopies(0, 0)
    for cp in w0[:2] + ccopies(0):
        cp.start()

    qscale = float((HD ** -0.5) * np.log2(np.e))

    ar, xa, ca = arb.bitcast(U32), xab.bitcast(U32), cab.bitcast(U32)
    h0, h1 = h0b.bitcast(U32), h1b.bitcast(U32)

    def qkv_load(slot, which, hh, r0, n):
        rs = slice(r0 // 2, (r0 + n) // 2)
        return h0[which, rs] if hh == 0 else h1[slot, which, rs]

    def qkv_store(slot, which, hh, r0, val):
        rs = pl.ds(pl.multiple_of(r0, 128), val.shape[0])
        if hh == 0:
            h0b[which, rs] = val.astype(BF16)
        else:
            h1b[slot, which, rs] = val.astype(BF16)

    def proj_pieces(slot, dyn):
        def q_piece(i):
            def f():
                blk = lambda r, c: (lambda: halves(wq_b[slot, r * (DM // 2):(r + 1) * (DM // 2)])[c])
                w = rhs_ops(blk(0, 0), blk(0, 1), blk(1, 0), blk(1, 1))[i]().astype(BF16)
                a = jnp.concatenate([xa[i, b] for b in range(DM // 256)], axis=1)
                emit = lambda r, c, val: qkv_store(slot, 0, c, r * HS, val * qscale)
                consume(i, dot(unpack(a), w), emit, mq, dyn)
            return f
        def kv_piece(i):
            def f():
                def outer(kk, nn):
                    raw = lambda r, c: (lambda: halves((wk_b, wv_b)[nn][slot, (2 * r + kk) * 128:(2 * r + kk + 1) * 128])[c])
                    return rhs_ops(raw(0, 0), raw(0, 1), raw(1, 0), raw(1, 1))[i]
                rops = rhs_ops(outer(0, 0), outer(0, 1), outer(1, 0), outer(1, 1))
                def inner_emit(r2, c2, v):
                    def emit(r, c, val):
                        for t in range(0, QS, 128):
                            blk = val[t:t + 128]
                            qkv_store(slot, 1 + c2, c, r * HS + r2 * QS + t, blk.T if c2 else blk)
                    consume(i, v, emit, mkv.at[:, c2, r2 * QS:(r2 + 1) * QS], dyn)
                for j in PORD:
                    w = rops[j]().astype(BF16)
                    v = jnp.concatenate([dot(unpack(ca[i, j, a * QS // 8:(a + 1) * QS // 8]), w) for a in range(4)], axis=0)
                    consume(j, v, inner_emit, mi, dyn)
            return f
        return [kv_piece(i) for i in PORD], [q_piece(i) for i in PORD]

    def scores(slot, hh, i, buf, dyn):
        L = (i + 1) * BQ
        q = unpack(qkv_load(slot, 0, hh, i * BQ, BQ))
        m = None
        n = L // 4
        for a in range(4):
            st = dot_nt(unpack(qkv_load(slot, 1, hh, a * n, n)), q)
            d0 = max(L - BQ - a * n, 0)
            if d0 < n:
                row = lax.broadcasted_iota(jnp.int32, (n - d0, BQ), 0) + (a * n + d0 - (L - BQ))
                col = lax.broadcasted_iota(jnp.int32, (n - d0, BQ), 1)
                dg = jnp.where(row <= col, st[d0:], -1e9)
                st = dg if d0 == 0 else jnp.concatenate([st[:d0], dg], axis=0)
            (s0, s1)[buf][pl.ds(pl.multiple_of(a * n + dyn, 32), n)] = st
            ma = jnp.max(st.reshape(n // 8, 8, BQ), axis=0)
            m = ma if m is None else jnp.maximum(m, ma)
        return jnp.broadcast_to(jnp.max(m, axis=0, keepdims=True), (8, BQ))

    def weighted(slot, hh, i, buf, m, never, dyn2):
        l = ot = None
        for t0 in range(0, i + 1, GT):
            nt = min(GT, i + 1 - t0)
            pj = jnp.exp2((s0, s1)[buf][t0 * BQ:(t0 + nt) * BQ] - jnp.tile(m, (nt * BQ // 8, 1)))
            lj = jnp.sum(pj.reshape(nt * BQ // 8, 8, BQ), axis=0)
            if LAG and l is not None:
                pj = jnp.concatenate([jnp.where(never, l, pj[:8]), pj[8:]], axis=0)
            l = lj if l is None else l + lj
            pt = pj.astype(BF16)
            ns = 1 if nt == 4 else 2 if nt == 2 else 4
            if SPL and t0 < (i + 1) // SPL * SPL:
                ns = 4 // SPL
            parts = []
            for a in range(ns):
                vt = jnp.concatenate([qkv_load(slot, 2, hh, t * 128 + a * HD // ns, HD // ns)
                                      for t in range(t0, t0 + nt)], axis=1)
                parts.append(dot(unpack(vt), pt))
            d = jnp.concatenate(parts, axis=0)
            ot = d if ot is None else ot + d
        l = jnp.sum(l, axis=0, keepdims=True)
        r = pl.reciprocal(l, approx=True)
        r = r * (2.0 - l * r)
        return (ot * r).T

    def attention(p, slot, pieces):
        pieces = list(pieces)
        dyn = lax.shift_right_logical(p, 8)
        never = jnp.broadcast_to(p, (8, BQ)) < 0
        dyn2 = lax.shift_right_logical(p, 9)
        tmp = lambda i: pl.ds(pl.multiple_of(A_TMP + i * BQ + dyn, 64), BQ)
        gs = lambda hh: range(NG) if not (REV >> hh) & 1 else reversed(range(NG))
        units = [(hh, g + a * NG) for hh in range(2) for g in gs(hh) for a in range(2)]
        slot1 = lambda i: 2 * NG + (i % 2) * 2 + i // NG

        nxt = scores(slot, *units[0], 0, dyn)
        tok = {}
        for u, (hh, i) in enumerate(units):
            cur = nxt
            if u + 1 < len(units):
                nxt = scores(slot, *units[u + 1], (u + 1) % 2, dyn)
            if pieces and (u in SL0 or u - 2 * NG in SL1):
                pieces.pop(0)()
            if u in tok:
                cur = jnp.where(never, tok[u], cur)
            o = weighted(slot, hh, i, u % 2, cur, never, dyn2)
            if hh == 0 or i < NG:
                ar[tmp(i if hh == 0 else slot1(i))] = pltpu.bitcast(o, U32)
            else:
                g = i - NG
                for rc in range(0, BQ, CCH):
                    a11, a12, a21 = (pltpu.bitcast(ar[pl.ds(pl.multiple_of(A_TMP + t * BQ + rc + dyn, 16), CCH)], F32)
                                     for t in (g, slot1(g), i))
                    for j, op in enumerate(lhs_ops(lambda: a11, lambda: a12, lambda: a21, lambda: o[rc:rc + CCH])):
                        base = A_CT + (j * NP + p) * (HS // 2) + g * (BQ // 2)
                        arb[pl.ds(pl.multiple_of(base * 2 + rc, 16), CCH)] = op().astype(BF16)
            if CLAG and (hh == 1 and i >= NG or TOK0 and u % 2):
                tok[u + CLAG] = pltpu.bitcast(ar[pl.ds(pl.multiple_of(A_TMP + dyn2, 8), 8)], F32)
        while pieces:
            pieces.pop(0)()

    def x_combos(r0, n):
        k2 = DM // 2
        top, bot = (x_s[pl.ds(pl.multiple_of(a * HS + r0, n), n)].astype(F32) for a in range(2))
        ops = lhs_ops(lambda: top[:, :k2], lambda: top[:, k2:], lambda: bot[:, :k2], lambda: bot[:, k2:])
        for j, op in enumerate(ops):
            val = op().astype(BF16)
            for b in range(k2 // 128):
                xab[j, b, pl.ds(pl.multiple_of(r0, n), n)] = val[:, b * 128:(b + 1) * 128]
        for a, v in enumerate((top, bot)):
            gwf = gw[...].astype(F32)
            gl = v[:, 0:128] * gwf[0:1]
            for b in range(1, NT):
                gl = gl + v[:, b * 128:(b + 1) * 128] * gwf[b:b + 1]
            gl = jnp.sum(gl, axis=-1, keepdims=True)
            gate_s[pl.ds(pl.multiple_of(a * HS + r0, n), n)] = jnp.broadcast_to(jax.nn.sigmoid(gl), (n, 128))

    def c_combos(r0, n):
        quarter = [c_s[pl.ds(pl.multiple_of(a * QS + r0, n), n)].astype(F32) for a in range(4)]
        for i in range(7):
            def outer(r2, kk):
                raw = lambda r, c: (lambda: quarter[2 * r + r2][:, (2 * c + kk) * 128:(2 * c + kk + 1) * 128])
                val = lhs_ops(raw(0, 0), raw(0, 1), raw(1, 0), raw(1, 1))[i]()
                return lambda: val
            for j, op in enumerate(lhs_ops(outer(0, 0), outer(0, 1), outer(1, 0), outer(1, 1))):
                cab[i, j, pl.ds(pl.multiple_of(r0, n), n)] = op().astype(BF16)

    dd_s[...] = ssmd[...].astype(F32)
    NC = QS // RB
    for cp in w0[:2]:
        cp.wait()
    for cp in xcopies(0) + w0[2:]:
        cp.start()
    def pro_step(r, carry):
        r0 = r * RB
        both = lambda ref: unpack(jnp.concatenate(
            [ref.bitcast(U32)[pl.ds(pl.multiple_of((a * QS + r0) // 2, RB // 2), RB // 2)] for a in range(4)], axis=0))
        for cp in ccopies(r):
            cp.wait()
        @pl.when(r + 1 < NC)
        def _():
            for cp in ccopies(r + 1) + xcopies(r + 1):
                cp.start()
        @pl.when(r + 1 == NC)
        def _():
            for cp in wcopies(1, 1):
                cp.start()
        for which, wb in ((1, wk_b), (2, wv_b)):
            val = dot(both(c_s), jnp.concatenate(halves(wb[0]), axis=1).astype(BF16))
            for hh in range(2):
                for a in range(4):
                    blk = val[a * RB:(a + 1) * RB, hh * 128:(hh + 1) * 128]
                    qkv_store(0, which, hh, a * QS + r0, blk if which == 1 else blk.T)
        for a in range(0, RB, 16):
            c_combos(r0 + a, 16)
        for cp in xcopies(r):
            cp.wait()
        @pl.when(r == 0)
        def _():
            w0[2].wait()
        val = dot(both(x_s), jnp.concatenate(halves(wq_b[0]), axis=1).astype(BF16)) * qscale
        for hh in range(2):
            for a in range(4):
                qkv_store(0, 0, hh, a * QS + r0, val[a * RB:(a + 1) * RB, hh * 128:(hh + 1) * 128])
        for a in range(2):
            for b in range(0, RB, 16):
                x_combos(a * QS + r0 + b, 16)
        return carry
    lax.fori_loop(0, NC, pro_step, 0)

    def pair_step(p, carry):
        slot = p % 2
        for cp in wcopies(p + 1, 1 - slot):
            cp.wait()
        @pl.when(p + 2 < NP)
        def _():
            for cp in wcopies(p + 2, slot):
                cp.start()
        @pl.when(p == NP - 2)
        def _():
            for cp in tcopies(0, 0):
                cp.start()
        kvp, qp = proj_pieces(1 - slot, lax.shift_right_logical(p, 8))
        attention(p, slot, [f for pair in zip(kvp, qp) for f in pair])
        return carry + 1
    last = lax.fori_loop(0, NP - 1, pair_step, 0) if not ONLY2 else None
    if ONLY1:
        return
    if not ONLY2:
        attention(last, (NP - 1) % 2, [])

    def tile_step(t, carry):
        slot = t % 2
        for cp in tcopies(t, slot):
            cp.wait()
        @pl.when(t + 1 < NT // 2)
        def _():
            for cp in tcopies(t + 1, 1 - slot):
                cp.start()
        @pl.when(t >= 2)
        def _():
            ocopy(t - 2, slot).wait()

        KC = 4
        def oprod(i):
            acc = None
            for j0 in range(0, NP, KC):
                def wblk(r, c):
                    return lambda: jnp.concatenate(
                        [wo_b[slot, 2 * j + r, :, c * 128:(c + 1) * 128] for j in range(j0, j0 + KC)], axis=0).astype(F32)
                w = rhs_ops(wblk(0, 0), wblk(0, 1), wblk(1, 0), wblk(1, 1))[i]().astype(BF16)
                a = jnp.concatenate([ar[pl.ds(A_CT + (i * NP + j) * (HS // 2), HS // 2)] for j in range(j0, j0 + KC)], axis=1)
                d = dot(unpack(a), w)
                acc = d if acc is None else acc + d
                yield acc
        def emit_o(r, c, val):
            rs = slice(r * HS, (r + 1) * HS)
            cs = slice(c * 128, (c + 1) * 128)
            o_b[slot, rs, cs] = (ga_s[c, rs] + (1.0 - gate_s[rs]) * val).astype(BF16)
        def opieces():
            m = {}
            for i in PORD:
                for acc in oprod(i):
                    m[i] = acc
                    yield
            yield
            emit_o(0, 1, m[2] + m[4])
            emit_o(1, 0, m[1] + m[3])
            emit_o(0, 0, (m[0] + m[6]) + (m[3] - m[4]))
            emit_o(1, 1, (m[0] + m[5]) + (m[2] - m[1]))
            yield
        gen = opieces()
        def piece(n=1):
            for _ in range(n):
                next(gen)

        rows = lax.broadcasted_iota(jnp.int32, (8, 128), 0)
        sgn = (1 - 2 * (rows & 1)).astype(F32)
        Fm = f_ref[...]
        Gm = g_ref[...]
        for c in range(2):
            cs = slice(c * 128, (c + 1) * 128)
            piece()
            kk = ak_b[slot, :, cs].astype(F32)
            sh = shk[2 * t + c].astype(F32)
            ksf = kk * sh[0:1, :]
            for j in range(1, KS):
                kr = pltpu.roll(kk, j, 0)
                kr = jnp.concatenate([jnp.where(rows >= j, kr[:8], 0.0), kr[8:]], axis=0)
                ksf = ksf + kr * sh[j:j + 1, :]
            kv = (ksf * av_b[slot, :, cs].astype(F32)).astype(BF16)
            for j in range(0, NCH, 4):
                r = dot_nt(Fm, jnp.concatenate([hk_b[slot, cs, (j + a) * C:(j + a + 1) * C] for a in range(4)], axis=0))
                for a in range(4):
                    hf[j + a] = r[:, a * 128:(a + 1) * 128]
            piece()
            for j in range(0, NCH, 4):
                r = dot(Fm, jnp.concatenate([kv[(j + a) * C:(j + a + 1) * C] for a in range(4)], axis=1))
                for a in range(4):
                    uf[j + a] = r[:, a * 128:(a + 1) * 128]
            ga_s[c] = kv.astype(F32) * dd_s[pl.ds(2 * t + c, 1)]
            piece()
            for ft in range(C // 8):
                re = slice(ft * 8, ft * 8 + 8)
                im = slice(C + ft * 8, C + ft * 8 + 8)
                hc = [hf[0, re]] + [hf[m, re] - sgn * hf[m - 1, im] for m in range(1, NCH)]
                hd = [hf[0, im]] + [hf[m, im] + sgn * hf[m - 1, re] for m in range(1, NCH)]
                ua = [uf[j, re] for j in range(NCH)]
                ub = [uf[j, im] for j in range(NCH)]
                def toep(u, h):
                    out = []
                    for i in range(NCH):
                        a = u[0] * h[i]
                        for j in range(1, i + 1):
                            a = a + u[j] * h[i - j]
                        out.append(a)
                    return out
                k1 = toep([a + b for a, b in zip(ua, ub)], hc)
                k2 = toep(ua, [d - c_ for c_, d in zip(hc, hd)])
                k3 = toep(ub, [d + c_ for c_, d in zip(hc, hd)])
                for i in range(NCH):
                    zf[i, re] = k1[i] - k3[i]
                    zf[i, im] = k1[i] + k2[i]
                if ft % 8 not in (0, 3, 6):
                    piece()
            xcs = pl.ds(pl.multiple_of((2 * t + c) * 128, 128), 128)
            for j in range(0, NCH, 4):
                r = dot(Gm, jnp.concatenate([zf[j + a] for a in range(4)], axis=1).astype(BF16))
                for a in range(4):
                    ts = slice((j + a) * C, (j + a + 1) * C)
                    y = r[:, a * 128:(a + 1) * 128] + ga_s[c, ts]
                    ga_s[c, ts] = gate_s[ts] * (x_s[ts, xcs].astype(F32) * y)
                if j == 4:
                    piece()
        piece(2)
        ocopy(t, slot).start()
        return carry
    lax.fori_loop(0, NT // 2, tile_step, 0)
    ocopy(NT // 2 - 2, 0).wait()
    ocopy(NT // 2 - 1, 1).wait()

@jax.jit
def pallas_gated_mix__ssm_conv_h3__compressed_kv_cla__prompt_kernel(
        A_q, A_k, A_v, A_shift_k, A_ssm_k, A_ssm_D, B_x, B_c_kv, B_w_q, B_w_uk, B_w_uv, B_w_o, gate_w):
    any_ = pl.BlockSpec(memory_space=pl.ANY)
    vm = pl.BlockSpec(memory_space=pltpu.VMEM)
    out = pl.pallas_call(
        kernel,
        in_specs=[vm] * 5 + [any_] * 9,
        out_specs=any_,
        out_shape=jax.ShapeDtypeStruct((1, S, DM), BF16),
        scratch_shapes=[
            pltpu.VMEM((S, DM), BF16), pltpu.VMEM((S, DC), BF16),
            pltpu.VMEM((7, DM // 256, HS, 128), BF16), pltpu.VMEM((7, 7, QS, 128), BF16),
            pltpu.VMEM((2, DM, 128), U32), pltpu.VMEM((2, DC, 128), U32), pltpu.VMEM((2, DC, 128), U32),
            pltpu.VMEM((3, S, 128), BF16), pltpu.VMEM((2, 3, S, 128), BF16), pltpu.VMEM((2 * A_END, 128), BF16),
            pltpu.VMEM((S, 128), F32), pltpu.VMEM((S, 128), F32), pltpu.VMEM((4, 2, HS, 128), F32), pltpu.VMEM((4, QS, 128), F32), pltpu.VMEM((4, HS, 128), F32),
            pltpu.VMEM((S, 128), F32),
            pltpu.VMEM((2, S, 256), BF16), pltpu.VMEM((2, S, 256), BF16), pltpu.VMEM((2, 256, S), BF16),
            pltpu.VMEM((2, H, HD, 256), BF16), pltpu.VMEM((2, S, 256), BF16),
            pltpu.VMEM((NCH, 2 * C, 128), F32), pltpu.VMEM((NCH, 2 * C, 128), F32), pltpu.VMEM((NCH, 2 * C, 128), F32),
            pltpu.VMEM((2, S, 128), F32), pltpu.VMEM((NT, 128), F32),
            pltpu.SemaphoreType.DMA((2, 4, 4)), pltpu.SemaphoreType.DMA((3, 2)), pltpu.SemaphoreType.DMA((4, 2)),
            pltpu.SemaphoreType.DMA((2,)),
        ],
        compiler_params=pltpu.CompilerParams(vmem_limit_bytes=120 * 1024 * 1024),
    )(gate_w.reshape(NT, 128), A_shift_k.T.reshape(KS, NT, 128).transpose(1, 0, 2), A_ssm_D.reshape(NT, 128), _F, _G,
      A_q, A_k, A_v, A_ssm_k, B_c_kv, B_w_q, B_w_uk, B_w_uv, B_w_o)
    return out
```

```python
import numpy as np
import jax
import jax.numpy as jnp
from jax import lax
import jax.experimental.pallas as pl
import jax.experimental.pallas.tpu as pltpu
import ml_dtypes

S, DM, H, HD, DC, KS = 2048, 1024, 32, 128, 512, 4
C = 128
NCH = S // C
NP = H // 2
NT = DM // 128
HS = S // 2
QS = S // 4
F32, BF16, U32 = jnp.float32, jnp.bfloat16, jnp.uint32
NTD = (((1,), (1,)), ((), ()))

BQ = 128
NG = HS // BQ
A_TMP = 0
A_CT = A_TMP + S + 4 * BQ
A_END = A_CT + 7 * NP * (HS // 2)
ONLY1 = 0
ONLY2 = 0
OR = 128
GT = 1
LAG = 0
REV = 3
CLAG = 3
TOK0 = 0
SPL = 0
CH = 0
PP = ((1,2,2,0,(1,3,5,7,9,11,13,15)),(1,1,2,1,(0,2,3,5,6,8,10,11,13,14)))
NOPRO = 0
PO = 0
UO = 3
PQ = ((0,), (1,), (2,), (3,))
CCH = 32
SL0 = (0,1,2,3,4,7,9,12,13,15)
SL1 = (0,13,14,16)

def _dft_consts():
    N = 2 * C
    f = np.arange(C, dtype=np.float64)[:, None] + 0.5
    t = np.arange(C, dtype=np.float64)[None, :]
    ang = 2 * np.pi * f * t / N
    Fm = np.concatenate([np.cos(ang), -np.sin(ang)], 0)
    Gm = np.concatenate([np.cos(ang).T, -np.sin(ang).T], 1) * (2.0 / N)
    return Fm.astype(ml_dtypes.bfloat16), Gm.astype(ml_dtypes.bfloat16)
_F, _G = _dft_consts()

def dot(a, b):
    return jnp.dot(a, b, preferred_element_type=F32)

def dot_nt(a, b):
    return lax.dot_general(a, b, NTD, preferred_element_type=F32)

def pack(x):
    return pltpu.bitcast(x.astype(BF16), U32)

def unpack(w):
    return pltpu.bitcast(w, BF16)

def halves(w):
    return pltpu.bitcast(w << 16, F32), pltpu.bitcast(w & jnp.uint32(0xFFFF0000), F32)

def lhs_ops(a11, a12, a21, a22):
    return [lambda: a11() + a22(), lambda: a21() + a22(), a11, a22,
            lambda: a11() + a12(), lambda: a21() - a11(), lambda: a12() - a22()]

def rhs_ops(b11, b12, b21, b22):
    return [lambda: b11() + b22(), b11, lambda: b12() - b22(), lambda: b21() - b11(),
            b22, lambda: b11() + b12(), lambda: b21() + b22()]

PORD = (2, 4, 1, 0, 5, 3, 6)
SKIP = (4, 10, 16)

def consume(i, v, emit, m, dyn):
    if i == 2:
        m[0 + dyn] = v
    elif i == 4:
        emit(0, 1, m[0] + v)
        m[1 + dyn] = v
    elif i == 1:
        m[2 + dyn] = v
    elif i == 0:
        m[3 + dyn] = v
    elif i == 5:
        emit(1, 1, (m[0] - m[2]) + (m[3] + v))
    elif i == 3:
        emit(1, 0, m[2] + v)
        m[0 + dyn] = v
    else:
        emit(0, 0, (m[3] - m[1]) + (m[0] + v))

def kernel(gw, shk, ssmd, f_ref, g_ref, aq_hbm, ak_hbm, av_hbm, ssmk_hbm, c_hbm, wq_hbm, wk_hbm, wv_hbm, wo_hbm,
           o_hbm,
           x_s, c_s, xab, cab, wq_b, wk_b, wv_b, h0b, h1b, arb, s0, s1, mkv, mi, mq, gate_s, ak_b, av_b, hk_b, wo_b, o_b, uf, hf, zf, ga_s, dd_s, gw_s,
           sem_x, sem_w, sem_t, sem_o):

    def wcopies(p, slot):
        return [pltpu.make_async_copy(src.bitcast(U32).at[:, p, :], dst.at[slot], sem_w.at[i, slot])
                for i, (src, dst) in enumerate(((wk_hbm, wk_b), (wv_hbm, wv_b), (wq_hbm, wq_b)))]

    def tcopies(t, slot):
        cs = pl.ds(pl.multiple_of(t * 256, 256), 256)
        return [pltpu.make_async_copy(ak_hbm.at[0, :, cs], ak_b.at[slot], sem_t.at[0, slot]),
                pltpu.make_async_copy(av_hbm.at[0, :, cs], av_b.at[slot], sem_t.at[1, slot]),
                pltpu.make_async_copy(ssmk_hbm.at[cs, :], hk_b.at[slot], sem_t.at[2, slot]),
                pltpu.make_async_copy(wo_hbm.at[:, :, cs], wo_b.at[slot], sem_t.at[3, slot])]

    def ocopy(t, slot):
        cs = pl.ds(pl.multiple_of(t * 256, 256), 256)
        return pltpu.make_async_copy(o_b.at[slot], o_hbm.at[0, :, cs], sem_o.at[slot])

    RB = 128
    def ccopies(r):
        rows = lambda a: pl.ds(pl.multiple_of(a * QS + r * RB, RB), RB)
        return [pltpu.make_async_copy(c_hbm.at[0, rows(a)], c_s.at[rows(a)], sem_x.at[a, r]) for a in range(4)]
    w0 = wcopies(0, 0)
    for cp in w0[:2] + ccopies(0):
        cp.start()

    qscale = float((HD ** -0.5) * np.log2(np.e))

    ar, xa, ca = arb.bitcast(U32), xab.bitcast(U32), cab.bitcast(U32)
    h0, h1 = h0b.bitcast(U32), h1b.bitcast(U32)

    def qkv_load(slot, which, hh, r0, n):
        rs = slice(r0 // 2, (r0 + n) // 2)
        return h0[which, rs] if hh == 0 else h1[slot, which, rs]

    def qkv_store(slot, which, hh, r0, val):
        rs = pl.ds(pl.multiple_of(r0, 128), val.shape[0])
        if hh == 0:
            h0b[which, rs] = val.astype(BF16)
        else:
            h1b[slot, which, rs] = val.astype(BF16)

    def proj_pieces(slot, dyn):
        def q_piece(i):
            def f():
                blk = lambda r, c: (lambda: halves(wq_b[slot, r * (DM // 2):(r + 1) * (DM // 2)])[c])
                w = rhs_ops(blk(0, 0), blk(0, 1), blk(1, 0), blk(1, 1))[i]().astype(BF16)
                a = jnp.concatenate([xa[i, b] for b in range(DM // 256)], axis=1)
                emit = lambda r, c, val: qkv_store(slot, 0, c, r * HS, val * qscale)
                consume(i, dot(unpack(a), w), emit, mq, dyn)
            return f
        def kv_piece(i):
            def f():
                def outer(kk, nn):
                    raw = lambda r, c: (lambda: halves((wk_b, wv_b)[nn][slot, (2 * r + kk) * 128:(2 * r + kk + 1) * 128])[c])
                    return rhs_ops(raw(0, 0), raw(0, 1), raw(1, 0), raw(1, 1))[i]
                rops = rhs_ops(outer(0, 0), outer(0, 1), outer(1, 0), outer(1, 1))
                def inner_emit(r2, c2, v):
                    def emit(r, c, val):
                        for t in range(0, QS, 128):
                            blk = val[t:t + 128]
                            qkv_store(slot, 1 + c2, c, r * HS + r2 * QS + t, blk.T if c2 else blk)
                    consume(i, v, emit, mkv.at[:, c2, r2 * QS:(r2 + 1) * QS], dyn)
                for j in PORD:
                    w = rops[j]().astype(BF16)
                    v = jnp.concatenate([dot(unpack(ca[i, j, a * QS // 8:(a + 1) * QS // 8]), w) for a in range(4)], axis=0)
                    consume(j, v, inner_emit, mi, dyn)
            return f
        return [kv_piece(i) for i in PORD], [q_piece(i) for i in PORD]

    def scores(slot, hh, i, buf, dyn):
        L = (i + 1) * BQ
        q = unpack(qkv_load(slot, 0, hh, i * BQ, BQ))
        m = None
        n = L // 4
        for a in range(4):
            st = dot_nt(unpack(qkv_load(slot, 1, hh, a * n, n)), q)
            d0 = max(L - BQ - a * n, 0)
            if d0 < n:
                row = lax.broadcasted_iota(jnp.int32, (n - d0, BQ), 0) + (a * n + d0 - (L - BQ))
                col = lax.broadcasted_iota(jnp.int32, (n - d0, BQ), 1)
                dg = jnp.where(row <= col, st[d0:], -1e9)
                st = dg if d0 == 0 else jnp.concatenate([st[:d0], dg], axis=0)
            (s0, s1)[buf][pl.ds(pl.multiple_of(a * n + dyn, 32), n)] = st
            ma = jnp.max(st.reshape(n // 8, 8, BQ), axis=0)
            m = ma if m is None else jnp.maximum(m, ma)
        return jnp.broadcast_to(jnp.max(m, axis=0, keepdims=True), (8, BQ))

    def weighted(slot, hh, i, buf, m, never, dyn2):
        l = ot = None
        for t0 in range(0, i + 1, GT):
            nt = min(GT, i + 1 - t0)
            pj = jnp.exp2((s0, s1)[buf][t0 * BQ:(t0 + nt) * BQ] - jnp.tile(m, (nt * BQ // 8, 1)))
            lj = jnp.sum(pj.reshape(nt * BQ // 8, 8, BQ), axis=0)
            if LAG and l is not None:
                pj = jnp.concatenate([jnp.where(never, l, pj[:8]), pj[8:]], axis=0)
            l = lj if l is None else l + lj
            pt = pj.astype(BF16)
            ns = 1 if nt == 4 else 2 if nt == 2 else 4
            if SPL and t0 < (i + 1) // SPL * SPL:
                ns = 4 // SPL
            parts = []
            for a in range(ns):
                vt = jnp.concatenate([qkv_load(slot, 2, hh, t * 128 + a * HD // ns, HD // ns)
                                      for t in range(t0, t0 + nt)], axis=1)
                parts.append(dot(unpack(vt), pt))
            d = jnp.concatenate(parts, axis=0)
            ot = d if ot is None else ot + d
        l = jnp.sum(l, axis=0, keepdims=True)
        r = pl.reciprocal(l, approx=True)
        r = r * (2.0 - l * r)
        return (ot * r).T

    def attention(p, slot, pieces):
        pieces = list(pieces)
        dyn = lax.shift_right_logical(p, 8)
        never = jnp.broadcast_to(p, (8, BQ)) < 0
        dyn2 = lax.shift_right_logical(p, 9)
        tmp = lambda i: pl.ds(pl.multiple_of(A_TMP + i * BQ + dyn, 64), BQ)
        gs = lambda hh: range(NG) if not (REV >> hh) & 1 else reversed(range(NG))
        units = [(hh, g + a * NG) for hh in range(2) for g in gs(hh) for a in range(2)]
        if UO == 1:
            units[:2 * NG] = [(0, i) for g in range(NG) for i in (g, 2 * NG - 1 - g)]
        elif UO == 2:
            units[:2 * NG] = [(0, i) for i in range(2 * NG)]
        elif UO == 3:
            units[:2 * NG] = [(0, i) for g in range(NG) for i in (2 * NG - 1 - g, g)]
        slot1 = lambda i: 2 * NG + (i % 2) * 2 + i // NG

        nxt = scores(slot, *units[0], 0, dyn)
        tok = {}
        for u, (hh, i) in enumerate(units):
            cur = nxt
            if u + 1 < len(units):
                nxt = scores(slot, *units[u + 1], (u + 1) % 2, dyn)
            if pieces and (u in SL0 or u - 2 * NG in SL1):
                pieces.pop(0)()
            if u in tok:
                cur = jnp.where(never, tok[u], cur)
            o = weighted(slot, hh, i, u % 2, cur, never, dyn2)
            if hh == 0 or i < NG:
                ar[tmp(i if hh == 0 else slot1(i))] = pltpu.bitcast(o, U32)
            else:
                g = i - NG
                for rc in range(0, BQ, CCH):
                    a11, a12, a21 = (pltpu.bitcast(ar[pl.ds(pl.multiple_of(A_TMP + t * BQ + rc + dyn, 16), CCH)], F32)
                                     for t in (g, slot1(g), i))
                    for j, op in enumerate(lhs_ops(lambda: a11, lambda: a12, lambda: a21, lambda: o[rc:rc + CCH])):
                        base = A_CT + (j * NP + p) * (HS // 2) + g * (BQ // 2)
                        arb[pl.ds(pl.multiple_of(base * 2 + rc, 16), CCH)] = op().astype(BF16)
            if CLAG and (hh == 1 and i >= NG or TOK0 and u % 2):
                tok[u + CLAG] = pltpu.bitcast(ar[pl.ds(pl.multiple_of(A_TMP + dyn2, 8), 8)], F32)
        while pieces:
            pieces.pop(0)()

    def x_combos(r0, n):
        rows = [pl.ds(pl.multiple_of(a * HS + r0, n), n) for a in range(2)]
        gl = [None, None]
        for b in range(NT // 2):
            blk = [[x_s[rows[a], (c * NT // 2 + b) * 128:(c * NT // 2 + b + 1) * 128].astype(F32) for c in range(2)]
                   for a in range(2)]
            ops = lhs_ops(lambda: blk[0][0], lambda: blk[0][1], lambda: blk[1][0], lambda: blk[1][1])
            for j, op in enumerate(ops):
                xab[j, b, rows[0]] = op().astype(BF16)
            for a in range(2):
                for c in range(2):
                    term = blk[a][c] * gw_s[c * NT // 2 + b, 0:n]
                    gl[a] = term if gl[a] is None else gl[a] + term
        for a in range(2):
            gate_s[rows[a]] = jnp.broadcast_to(jax.nn.sigmoid(jnp.sum(gl[a], axis=-1, keepdims=True)), (n, 128))

    def c_combos(r0, n):
        quarter = [c_s[pl.ds(pl.multiple_of(a * QS + r0, n), n)].astype(F32) for a in range(4)]
        for i in range(7):
            def outer(r2, kk):
                raw = lambda r, c: (lambda: quarter[2 * r + r2][:, (2 * c + kk) * 128:(2 * c + kk + 1) * 128])
                val = lhs_ops(raw(0, 0), raw(0, 1), raw(1, 0), raw(1, 1))[i]()
                return lambda: val
            for j, op in enumerate(lhs_ops(outer(0, 0), outer(0, 1), outer(1, 0), outer(1, 1))):
                cab[i, j, pl.ds(pl.multiple_of(r0, n), n)] = op().astype(BF16)

    dd_s[...] = ssmd[...].astype(F32)
    for b in range(NT):
        gw_s[b] = jnp.broadcast_to(gw[...].astype(F32)[b:b + 1], (16, 128))
    NC = QS // RB
    for cp in w0[:2] + ccopies(0):
        cp.wait()
    cp_x = pltpu.make_async_copy(aq_hbm.at[0], x_s, sem_x.at[0, NC])
    rest = [cp for r in range(1, NC) for cp in ccopies(r)]
    for cp in rest + w0[2:] + [cp_x]:
        cp.start()
    rows_of = lambda ref, r: unpack(ref.bitcast(U32)[pl.ds(pl.multiple_of(r // 2, RB // 2), RB // 2)])
    def pro_kv(r, carry):
        r0 = r * RB
        @pl.when(r == 1)
        def _():
            for cp in rest:
                cp.wait()
        w = jnp.concatenate(halves(wk_b[0]) + halves(wv_b[0]), axis=1).astype(BF16)
        for a in range(4):
            val = dot(rows_of(c_s, a * QS + r0), w)
            for n in range(4):
                blk = val[:, n * 128:(n + 1) * 128]
                qkv_store(0, 1 + n // 2, n % 2, a * QS + r0, blk.T if n // 2 else blk)
            for b in range(a * RB // 4, (a + 1) * RB // 4, 16):
                c_combos(r0 + b, 16)
        return carry
    def pro_q(r, carry):
        r0 = r * RB
        w = jnp.concatenate(halves(wq_b[0]), axis=1).astype(BF16)
        for a in range(4):
            val = dot(rows_of(x_s, a * QS + r0), w) * qscale
            for hh in range(2):
                qkv_store(0, 0, hh, a * QS + r0, val[:, hh * 128:(hh + 1) * 128])
            for b in range(a % 2 * RB // 2, (a % 2 + 1) * RB // 2, 16):
                x_combos(a // 2 * QS + r0 + b, 16)
        return carry
    lax.fori_loop(0, NC, pro_kv, 0) if not NOPRO else None
    cp_x.wait()
    w0[2].wait()
    for cp in wcopies(1, 1):
        cp.start()
    lax.fori_loop(0, NC, pro_q, 0) if not NOPRO else None

    def pair_step(p, carry):
        slot = p % 2
        for cp in wcopies(p + 1, 1 - slot):
            cp.wait()
        @pl.when(p + 2 < NP)
        def _():
            for cp in wcopies(p + 2, slot):
                cp.start()
        @pl.when(p == NP - 2)
        def _():
            for cp in tcopies(0, 0):
                cp.start()
        kvp, qp = proj_pieces(1 - slot, lax.shift_right_logical(p, 8))
        attention(p, slot, [f for pair in (zip(kvp, qp) if PO == 0 else zip(qp, kvp)) for f in pair])
        return carry + 1
    last = lax.fori_loop(0, NP - 1, pair_step, 0) if not ONLY2 else None
    if ONLY1:
        return
    if not ONLY2:
        attention(last, (NP - 1) % 2, [])

    def tile_step(t, carry):
        slot = t % 2
        for cp in tcopies(t, slot):
            cp.wait()
        @pl.when(t + 1 < NT // 2)
        def _():
            for cp in tcopies(t + 1, 1 - slot):
                cp.start()
        @pl.when(t >= 2)
        def _():
            ocopy(t - 2, slot).wait()

        KC = 4
        def oprod(i):
            acc = None
            for j0 in range(0, NP, KC):
                def wblk(r, c):
                    return lambda: jnp.concatenate(
                        [wo_b[slot, 2 * j + r, :, c * 128:(c + 1) * 128] for j in range(j0, j0 + KC)], axis=0).astype(F32)
                w = rhs_ops(wblk(0, 0), wblk(0, 1), wblk(1, 0), wblk(1, 1))[i]().astype(BF16)
                a = jnp.concatenate([ar[pl.ds(A_CT + (i * NP + j) * (HS // 2), HS // 2)] for j in range(j0, j0 + KC)], axis=1)
                d = dot(unpack(a), w)
                acc = d if acc is None else acc + d
                yield acc
        def emit_o(r, c, val):
            rs = slice(r * HS, (r + 1) * HS)
            cs = slice(c * 128, (c + 1) * 128)
            o_b[slot, rs, cs] = (ga_s[c, rs] + (1.0 - gate_s[rs]) * val).astype(BF16)
        def opieces():
            m = {}
            for i in PORD:
                for acc in oprod(i):
                    m[i] = acc
                    yield
            yield
            emit_o(0, 1, m[2] + m[4])
            emit_o(1, 0, m[1] + m[3])
            emit_o(0, 0, (m[0] + m[6]) + (m[3] - m[4]))
            emit_o(1, 1, (m[0] + m[5]) + (m[2] - m[1]))
            yield
        gen = opieces()
        def piece(n=1):
            for _ in range(n):
                next(gen)

        rows = lax.broadcasted_iota(jnp.int32, (8, 128), 0)
        sgn = (1 - 2 * (rows & 1)).astype(F32)
        Fm = f_ref[...]
        Gm = g_ref[...]
        for c in range(2):
            cs = slice(c * 128, (c + 1) * 128)
            n0, n1, n2, n3, fts = PP[c]
            piece(n0)
            kk = ak_b[slot, :, cs].astype(F32)
            sh = shk[2 * t + c].astype(F32)
            ksf = kk * sh[0:1, :]
            for j in range(1, KS):
                kr = pltpu.roll(kk, j, 0)
                kr = jnp.concatenate([jnp.where(rows >= j, kr[:8], 0.0), kr[8:]], axis=0)
                ksf = ksf + kr * sh[j:j + 1, :]
            kv = (ksf * av_b[slot, :, cs].astype(F32)).astype(BF16)
            for j in range(0, NCH, 4):
                r = dot_nt(Fm, jnp.concatenate([hk_b[slot, cs, (j + a) * C:(j + a + 1) * C] for a in range(4)], axis=0))
                for a in range(4):
                    hf[j + a] = r[:, a * 128:(a + 1) * 128]
            piece(n1)
            for j in range(0, NCH, 4):
                r = dot(Fm, jnp.concatenate([kv[(j + a) * C:(j + a + 1) * C] for a in range(4)], axis=1))
                for a in range(4):
                    uf[j + a] = r[:, a * 128:(a + 1) * 128]
            ga_s[c] = kv.astype(F32) * dd_s[pl.ds(2 * t + c, 1)]
            piece(n2)
            for ft in range(C // 8):
                re = slice(ft * 8, ft * 8 + 8)
                im = slice(C + ft * 8, C + ft * 8 + 8)
                hc = [hf[0, re]] + [hf[m, re] - sgn * hf[m - 1, im] for m in range(1, NCH)]
                hd = [hf[0, im]] + [hf[m, im] + sgn * hf[m - 1, re] for m in range(1, NCH)]
                ua = [uf[j, re] for j in range(NCH)]
                ub = [uf[j, im] for j in range(NCH)]
                def toep(u, h):
                    out = []
                    for i in range(NCH):
                        a = u[0] * h[i]
                        for j in range(1, i + 1):
                            a = a + u[j] * h[i - j]
                        out.append(a)
                    return out
                k1 = toep([a + b for a, b in zip(ua, ub)], hc)
                k2 = toep(ua, [d - c_ for c_, d in zip(hc, hd)])
                k3 = toep(ub, [d + c_ for c_, d in zip(hc, hd)])
                for i in range(NCH):
                    zf[i, re] = k1[i] - k3[i]
                    zf[i, im] = k1[i] + k2[i]
                if ft in fts:
                    piece()
            xcs = pl.ds(pl.multiple_of((2 * t + c) * 128, 128), 128)
            for j in range(0, NCH, 4):
                r = dot(Gm, jnp.concatenate([zf[j + a] for a in range(4)], axis=1).astype(BF16))
                for a in range(4):
                    ts = slice((j + a) * C, (j + a + 1) * C)
                    y = r[:, a * 128:(a + 1) * 128] + ga_s[c, ts]
                    ga_s[c, ts] = gate_s[ts] * (x_s[ts, xcs].astype(F32) * y)
                if j == 4:
                    piece(n3)
        for _ in gen:
            pass
        ocopy(t, slot).start()
        return carry
    lax.fori_loop(0, NT // 2, tile_step, 0)
    ocopy(NT // 2 - 2, 0).wait()
    ocopy(NT // 2 - 1, 1).wait()

@jax.jit
def pallas_gated_mix__ssm_conv_h3__compressed_kv_cla__prompt_kernel(
        A_q, A_k, A_v, A_shift_k, A_ssm_k, A_ssm_D, B_x, B_c_kv, B_w_q, B_w_uk, B_w_uv, B_w_o, gate_w):
    any_ = pl.BlockSpec(memory_space=pl.ANY)
    vm = pl.BlockSpec(memory_space=pltpu.VMEM)
    out = pl.pallas_call(
        kernel,
        in_specs=[vm] * 5 + [any_] * 9,
        out_specs=any_,
        out_shape=jax.ShapeDtypeStruct((1, S, DM), BF16),
        scratch_shapes=[
            pltpu.VMEM((S, DM), BF16), pltpu.VMEM((S, DC), BF16),
            pltpu.VMEM((7, DM // 256, HS, 128), BF16), pltpu.VMEM((7, 7, QS, 128), BF16),
            pltpu.VMEM((2, DM, 128), U32), pltpu.VMEM((2, DC, 128), U32), pltpu.VMEM((2, DC, 128), U32),
            pltpu.VMEM((3, S, 128), BF16), pltpu.VMEM((2, 3, S, 128), BF16), pltpu.VMEM((2 * A_END, 128), BF16),
            pltpu.VMEM((S, 128), F32), pltpu.VMEM((S, 128), F32), pltpu.VMEM((4, 2, HS, 128), F32), pltpu.VMEM((4, QS, 128), F32), pltpu.VMEM((4, HS, 128), F32),
            pltpu.VMEM((S, 128), F32),
            pltpu.VMEM((2, S, 256), BF16), pltpu.VMEM((2, S, 256), BF16), pltpu.VMEM((2, 256, S), BF16),
            pltpu.VMEM((2, H, HD, 256), BF16), pltpu.VMEM((2, S, 256), BF16),
            pltpu.VMEM((NCH, 2 * C, 128), F32), pltpu.VMEM((NCH, 2 * C, 128), F32), pltpu.VMEM((NCH, 2 * C, 128), F32),
            pltpu.VMEM((2, S, 128), F32), pltpu.VMEM((NT, 128), F32), pltpu.VMEM((NT, 16, 128), F32),
            pltpu.SemaphoreType.DMA((4, 5)), pltpu.SemaphoreType.DMA((3, 2)), pltpu.SemaphoreType.DMA((4, 2)),
            pltpu.SemaphoreType.DMA((2,)),
        ],
        compiler_params=pltpu.CompilerParams(vmem_limit_bytes=120 * 1024 * 1024),
    )(gate_w.reshape(NT, 128), A_shift_k.T.reshape(KS, NT, 128).transpose(1, 0, 2), A_ssm_D.reshape(NT, 128), _F, _G,
      A_q, A_k, A_v, A_ssm_k, B_c_kv, B_w_q, B_w_uk, B_w_uv, B_w_o)
    return out
```

```python
import numpy as np
import jax
import jax.numpy as jnp
from jax import lax
import jax.experimental.pallas as pl
import jax.experimental.pallas.tpu as pltpu
import ml_dtypes

S, DM, H, HD, DC, KS = 2048, 1024, 32, 128, 512, 4
C = 128
NCH = S // C
NP = H // 2
NT = DM // 128
HS = S // 2
QS = S // 4
F32, BF16, U32 = jnp.float32, jnp.bfloat16, jnp.uint32
NTD = (((1,), (1,)), ((), ()))

BQ = 128
NG = HS // BQ
A_TMP = 0
A_CT = A_TMP + S + 4 * BQ
A_END = A_CT + 7 * NP * (HS // 2)
ONLY1 = 0
ONLY2 = 0
OR = 128
GT = 1
LAG = 0
REV = 3
CLAG = 2
TOK0 = 0
SPL = 0
CH = 0
PP = ((1,2,2,0,(1,3,5,7,9,11,13,15)),(1,1,2,1,(0,2,3,5,6,8,10,11,13,14)))
NOPRO = 0
PF = -1
CO = (1, 0)
EE = 1
AQ = 0
AO = 0
AI = 0
PB = (2,10,15,16)
PO = 0
UO = 3
PQ = ((0,), (1,), (2,), (3,))
CCH = 32
SL0 = (0,1,2,3,4,9,10,12,13,15)
SL1 = (0,13,14,16)

def _dft_consts():
    N = 2 * C
    f = np.arange(C, dtype=np.float64)[:, None] + 0.5
    t = np.arange(C, dtype=np.float64)[None, :]
    ang = 2 * np.pi * f * t / N
    Fm = np.concatenate([np.cos(ang), -np.sin(ang)], 0)
    Gm = np.concatenate([np.cos(ang).T, -np.sin(ang).T], 1) * (2.0 / N)
    return Fm.astype(ml_dtypes.bfloat16), Gm.astype(ml_dtypes.bfloat16)
_F, _G = _dft_consts()

def dot(a, b):
    return jnp.dot(a, b, preferred_element_type=F32)

def dot_nt(a, b):
    return lax.dot_general(a, b, NTD, preferred_element_type=F32)

def pack(x):
    return pltpu.bitcast(x.astype(BF16), U32)

def unpack(w):
    return pltpu.bitcast(w, BF16)

def halves(w):
    return pltpu.bitcast(w << 16, F32), pltpu.bitcast(w & jnp.uint32(0xFFFF0000), F32)

def lhs_ops(a11, a12, a21, a22):
    return [lambda: a11() + a22(), lambda: a21() + a22(), a11, a22,
            lambda: a11() + a12(), lambda: a21() - a11(), lambda: a12() - a22()]

def rhs_ops(b11, b12, b21, b22):
    return [lambda: b11() + b22(), b11, lambda: b12() - b22(), lambda: b21() - b11(),
            b22, lambda: b11() + b12(), lambda: b21() + b22()]

PORD = (2, 4, 1, 0, 5, 3, 6)
SKIP = (4, 10, 16)

def consume(i, v, emit, m, dyn, acc=0):
    if i == 2:
        m[0 + dyn] = v
    elif i == 4:
        emit(0, 1, m[0] + v)
        m[1 + dyn] = v
    elif i == 1:
        m[2 + dyn] = v
        if acc & 1:
            m[0 + dyn] = m[0] - v
    elif i == 0:
        m[3 + dyn] = v
        if acc & 2:
            m[1 + dyn] = v - m[1]
    elif i == 5:
        emit(1, 1, (m[0] if acc & 1 else m[0] - m[2]) + (m[3] + v))
    elif i == 3:
        emit(1, 0, m[2] + v)
        m[0 + dyn] = v
    else:
        emit(0, 0, (m[1] if acc & 2 else m[3] - m[1]) + (m[0] + v))

def kernel(gw, shk, ssmd, f_ref, g_ref, aq_hbm, ak_hbm, av_hbm, ssmk_hbm, c_hbm, wq_hbm, wk_hbm, wv_hbm, wo_hbm,
           o_hbm,
           x_s, c_s, xab, cab, wq_b, wk_b, wv_b, h0b, h1b, arb, s0, s1, mkv, mi, mq, gate_s, ak_b, av_b, hk_b, wo_b, o_b, uf, hf, zf, ga_s, dd_s, gw_s,
           sem_x, sem_w, sem_t, sem_o):

    def wcopies(p, slot):
        return [pltpu.make_async_copy(src.bitcast(U32).at[:, p, :], dst.at[slot], sem_w.at[i, slot])
                for i, (src, dst) in enumerate(((wk_hbm, wk_b), (wv_hbm, wv_b), (wq_hbm, wq_b)))]

    def tcopies(t, slot):
        cps = [pltpu.make_async_copy(ssmk_hbm.at[pl.ds(pl.multiple_of(t * 256, 256), 256), :], hk_b.at[slot], sem_t.at[0, slot])]
        for c in range(2):
            cs = pl.ds(pl.multiple_of((2 * t + c) * 128, 128), 128)
            cps += [pltpu.make_async_copy(ak_hbm.at[0, :, cs], ak_b.at[slot, c], sem_t.at[1 + c, slot]),
                    pltpu.make_async_copy(av_hbm.at[0, :, cs], av_b.at[slot, c], sem_t.at[3 + c, slot]),
                    pltpu.make_async_copy(wo_hbm.at[:, :, cs], wo_b.at[slot, c], sem_t.at[5 + c, slot])]
        return cps

    def ocopy(t, slot, c):
        cs = pl.ds(pl.multiple_of((2 * t + c) * 128, 128), 128)
        return pltpu.make_async_copy(o_b.at[slot, c], o_hbm.at[0, :, cs], sem_o.at[c, slot])

    RB = 128
    def ccopies(r):
        rows = lambda a: pl.ds(pl.multiple_of(a * QS + r * RB, RB), RB)
        return [pltpu.make_async_copy(c_hbm.at[0, rows(a)], c_s.at[rows(a)], sem_x.at[a, r]) for a in range(4)]
    w0 = wcopies(0, 0)
    for cp in w0[:2] + ccopies(0):
        cp.start()

    qscale = float((HD ** -0.5) * np.log2(np.e))

    ar, xa, ca = arb.bitcast(U32), xab.bitcast(U32), cab.bitcast(U32)
    h0, h1 = h0b.bitcast(U32), h1b.bitcast(U32)

    def qkv_load(slot, which, hh, r0, n):
        rs = slice(r0 // 2, (r0 + n) // 2)
        return h0[which, rs] if hh == 0 else h1[slot, which, rs]

    def qkv_store(slot, which, hh, r0, val):
        rs = pl.ds(pl.multiple_of(r0, 128), val.shape[0])
        if hh == 0:
            h0b[which, rs] = val.astype(BF16)
        else:
            h1b[slot, which, rs] = val.astype(BF16)

    def proj_pieces(slot, dyn):
        def q_piece(i):
            def f():
                blk = lambda r, c: (lambda: halves(wq_b[slot, r * (DM // 2):(r + 1) * (DM // 2)])[c])
                w = rhs_ops(blk(0, 0), blk(0, 1), blk(1, 0), blk(1, 1))[i]().astype(BF16)
                a = jnp.concatenate([xa[i, b] for b in range(DM // 256)], axis=1)
                emit = lambda r, c, val: qkv_store(slot, 0, c, r * HS, val * qscale)
                consume(i, dot(unpack(a), w), emit, mq, dyn, AQ)
            return f
        def kv_piece(i):
            def f():
                def outer(kk, nn):
                    raw = lambda r, c: (lambda: halves((wk_b, wv_b)[nn][slot, (2 * r + kk) * 128:(2 * r + kk + 1) * 128])[c])
                    return rhs_ops(raw(0, 0), raw(0, 1), raw(1, 0), raw(1, 1))[i]
                rops = rhs_ops(outer(0, 0), outer(0, 1), outer(1, 0), outer(1, 1))
                def inner_emit(r2, c2, v):
                    def emit(r, c, val):
                        for t in range(0, QS, 128):
                            blk = val[t:t + 128]
                            qkv_store(slot, 1 + c2, c, r * HS + r2 * QS + t, blk.T if c2 else blk)
                    consume(i, v, emit, mkv.at[:, c2, r2 * QS:(r2 + 1) * QS], dyn, AO)
                for j in PORD:
                    w = rops[j]().astype(BF16)
                    v = jnp.concatenate([dot(unpack(ca[i, j, a * QS // 8:(a + 1) * QS // 8]), w) for a in range(4)], axis=0)
                    consume(j, v, inner_emit, mi, dyn, AI)
            return f
        return [kv_piece(i) for i in PORD], [q_piece(i) for i in PORD]

    def scores(slot, hh, i, buf, dyn):
        L = (i + 1) * BQ
        q = unpack(qkv_load(slot, 0, hh, i * BQ, BQ))
        m = None
        n = L // 4
        for a in range(4):
            st = dot_nt(unpack(qkv_load(slot, 1, hh, a * n, n)), q)
            d0 = max(L - BQ - a * n, 0)
            if d0 < n:
                row = lax.broadcasted_iota(jnp.int32, (n - d0, BQ), 0) + (a * n + d0 - (L - BQ))
                col = lax.broadcasted_iota(jnp.int32, (n - d0, BQ), 1)
                dg = jnp.where(row <= col, st[d0:], -1e9)
                st = dg if d0 == 0 else jnp.concatenate([st[:d0], dg], axis=0)
            (s0, s1)[buf][pl.ds(pl.multiple_of(a * n + dyn, 32), n)] = st
            ma = jnp.max(st.reshape(n // 8, 8, BQ), axis=0)
            m = ma if m is None else jnp.maximum(m, ma)
        return jnp.broadcast_to(jnp.max(m, axis=0, keepdims=True), (8, BQ))

    def weighted(slot, hh, i, buf, m, never, dyn2):
        l = ot = None
        for t0 in range(0, i + 1, GT):
            nt = min(GT, i + 1 - t0)
            pj = jnp.exp2((s0, s1)[buf][t0 * BQ:(t0 + nt) * BQ] - jnp.tile(m, (nt * BQ // 8, 1)))
            lj = jnp.sum(pj.reshape(nt * BQ // 8, 8, BQ), axis=0)
            if LAG and l is not None:
                pj = jnp.concatenate([jnp.where(never, l, pj[:8]), pj[8:]], axis=0)
            l = lj if l is None else l + lj
            pt = pj.astype(BF16)
            ns = 1 if nt == 4 else 2 if nt == 2 else 4
            if SPL and t0 < (i + 1) // SPL * SPL:
                ns = 4 // SPL
            parts = []
            for a in range(ns):
                vt = jnp.concatenate([qkv_load(slot, 2, hh, t * 128 + a * HD // ns, HD // ns)
                                      for t in range(t0, t0 + nt)], axis=1)
                parts.append(dot(unpack(vt), pt))
            d = jnp.concatenate(parts, axis=0)
            ot = d if ot is None else ot + d
        l = jnp.sum(l, axis=0, keepdims=True)
        r = pl.reciprocal(l, approx=True)
        r = r * (2.0 - l * r)
        return (ot * r).T

    def attention(p, slot, pieces):
        pieces = list(pieces)
        dyn = lax.shift_right_logical(p, 8)
        never = jnp.broadcast_to(p, (8, BQ)) < 0
        dyn2 = lax.shift_right_logical(p, 9)
        tmp = lambda i: pl.ds(pl.multiple_of(A_TMP + i * BQ + dyn, 64), BQ)
        gs = lambda hh: range(NG) if not (REV >> hh) & 1 else reversed(range(NG))
        units = [(hh, g + a * NG) for hh in range(2) for g in gs(hh) for a in range(2)]
        if UO == 1:
            units[:2 * NG] = [(0, i) for g in range(NG) for i in (g, 2 * NG - 1 - g)]
        elif UO == 2:
            units[:2 * NG] = [(0, i) for i in range(2 * NG)]
        elif UO == 3:
            units[:2 * NG] = [(0, i) for g in range(NG) for i in (2 * NG - 1 - g, g)]
        slot1 = lambda i: 2 * NG + (i % 2) * 2 + i // NG

        nxt = scores(slot, *units[0], 0, dyn)
        tok = {}
        for u, (hh, i) in enumerate(units):
            cur = nxt
            here = pieces and (u in SL0 or u - 2 * NG in SL1)
            if here and u in PB:
                pieces.pop(0)()
            if u + 1 < len(units):
                nxt = scores(slot, *units[u + 1], (u + 1) % 2, dyn)
            if here and u not in PB:
                pieces.pop(0)()
            if u in tok:
                cur = jnp.where(never, tok[u], cur)
            o = weighted(slot, hh, i, u % 2, cur, never, dyn2)
            if hh == 0 or i < NG:
                ar[tmp(i if hh == 0 else slot1(i))] = pltpu.bitcast(o, U32)
            else:
                g = i - NG
                for rc in range(0, BQ, CCH):
                    a11, a12, a21 = (pltpu.bitcast(ar[pl.ds(pl.multiple_of(A_TMP + t * BQ + rc + dyn, 16), CCH)], F32)
                                     for t in (g, slot1(g), i))
                    for j, op in enumerate(lhs_ops(lambda: a11, lambda: a12, lambda: a21, lambda: o[rc:rc + CCH])):
                        base = A_CT + (j * NP + p) * (HS // 2) + g * (BQ // 2)
                        arb[pl.ds(pl.multiple_of(base * 2 + rc, 16), CCH)] = op().astype(BF16)
            if CLAG and (hh == 1 and i >= NG or TOK0 and u % 2):
                tok[u + CLAG] = pltpu.bitcast(ar[pl.ds(pl.multiple_of(A_TMP + dyn2, 8), 8)], F32)
        while pieces:
            pieces.pop(0)()

    def x_combos(r0, n):
        rows = [pl.ds(pl.multiple_of(a * HS + r0, n), n) for a in range(2)]
        gl = [None, None]
        for b in range(NT // 2):
            blk = [[x_s[rows[a], (c * NT // 2 + b) * 128:(c * NT // 2 + b + 1) * 128].astype(F32) for c in range(2)]
                   for a in range(2)]
            ops = lhs_ops(lambda: blk[0][0], lambda: blk[0][1], lambda: blk[1][0], lambda: blk[1][1])
            for j, op in enumerate(ops):
                xab[j, b, rows[0]] = op().astype(BF16)
            for a in range(2):
                for c in range(2):
                    term = blk[a][c] * gw_s[c * NT // 2 + b, 0:n]
                    gl[a] = term if gl[a] is None else gl[a] + term
        for a in range(2):
            gate_s[rows[a]] = jnp.broadcast_to(jax.nn.sigmoid(jnp.sum(gl[a], axis=-1, keepdims=True)), (n, 128))

    def c_combos(r0, n):
        quarter = [c_s[pl.ds(pl.multiple_of(a * QS + r0, n), n)].astype(F32) for a in range(4)]
        for i in range(7):
            def outer(r2, kk):
                raw = lambda r, c: (lambda: quarter[2 * r + r2][:, (2 * c + kk) * 128:(2 * c + kk + 1) * 128])
                val = lhs_ops(raw(0, 0), raw(0, 1), raw(1, 0), raw(1, 1))[i]()
                return lambda: val
            for j, op in enumerate(lhs_ops(outer(0, 0), outer(0, 1), outer(1, 0), outer(1, 1))):
                cab[i, j, pl.ds(pl.multiple_of(r0, n), n)] = op().astype(BF16)

    dd_s[...] = ssmd[...].astype(F32)
    for b in range(NT):
        gw_s[b] = jnp.broadcast_to(gw[...].astype(F32)[b:b + 1], (16, 128))
    NC = QS // RB
    for cp in w0[:2] + ccopies(0):
        cp.wait()
    cp_x = pltpu.make_async_copy(aq_hbm.at[0], x_s, sem_x.at[0, NC])
    rest = [cp for r in range(1, NC) for cp in ccopies(r)]
    for cp in rest + w0[2:] + [cp_x]:
        cp.start()
    rows_of = lambda ref, r: unpack(ref.bitcast(U32)[pl.ds(pl.multiple_of(r // 2, RB // 2), RB // 2)])
    def pro_kv(r, carry):
        r0 = r * RB
        @pl.when(r == 1)
        def _():
            for cp in rest:
                cp.wait()
        w = jnp.concatenate(halves(wk_b[0]) + halves(wv_b[0]), axis=1).astype(BF16)
        for a in range(4):
            val = dot(rows_of(c_s, a * QS + r0), w)
            for n in range(4):
                blk = val[:, n * 128:(n + 1) * 128]
                qkv_store(0, 1 + n // 2, n % 2, a * QS + r0, blk.T if n // 2 else blk)
            for b in range(a * RB // 4, (a + 1) * RB // 4, 16):
                c_combos(r0 + b, 16)
        return carry
    def pro_q(r, carry):
        r0 = r * RB
        w = jnp.concatenate(halves(wq_b[0]), axis=1).astype(BF16)
        for a in range(4):
            val = dot(rows_of(x_s, a * QS + r0), w) * qscale
            for hh in range(2):
                qkv_store(0, 0, hh, a * QS + r0, val[:, hh * 128:(hh + 1) * 128])
            for b in range(a % 2 * RB // 2, (a % 2 + 1) * RB // 2, 16):
                x_combos(a // 2 * QS + r0 + b, 16)
        return carry
    lax.fori_loop(0, NC, pro_kv, 0) if not NOPRO else None
    cp_x.wait()
    w0[2].wait()
    for cp in wcopies(1, 1):
        cp.start()
    lax.fori_loop(0, NC, pro_q, 0) if not NOPRO else None

    def pair_step(p, carry):
        slot = p % 2
        for cp in wcopies(p + 1, 1 - slot):
            cp.wait()
        @pl.when(p + 2 < NP)
        def _():
            for cp in wcopies(p + 2, slot):
                cp.start()
        @pl.when(p == NP - 2)
        def _():
            for cp in tcopies(0, 0):
                cp.start()
        kvp, qp = proj_pieces(1 - slot, lax.shift_right_logical(p, 8))
        attention(p, slot, [f for pair in (zip(kvp, qp) if PO == 0 else zip(qp, kvp)) for f in pair])
        return carry + 1
    last = lax.fori_loop(0, NP - 1, pair_step, 0) if not ONLY2 else None
    if ONLY1:
        return
    if not ONLY2:
        attention(last, (NP - 1) % 2, [])

    def tile_step(t, carry):
        slot = t % 2
        for cp in tcopies(t, slot):
            cp.wait()
        def prefetch():
            @pl.when(t + 1 < NT // 2)
            def _():
                for cp in tcopies(t + 1, 1 - slot):
                    cp.start()
            @pl.when(t >= 2)
            def _():
                for c in range(2):
                    ocopy(t - 2, slot, c).wait()
        if PF < 0:
            prefetch()

        KC = 4
        def oprod(i):
            acc = None
            for j0 in range(0, NP, KC):
                def wblk(r, c):
                    return lambda: jnp.concatenate(
                        [unpack(wo_b.bitcast(U32)[slot, c, 2 * j + r]) for j in range(j0, j0 + KC)], axis=0).astype(F32)
                w = rhs_ops(wblk(0, 0), wblk(0, 1), wblk(1, 0), wblk(1, 1))[i]().astype(BF16)
                a = jnp.concatenate([ar[pl.ds(A_CT + (i * NP + j) * (HS // 2), HS // 2)] for j in range(j0, j0 + KC)], axis=1)
                d = dot(unpack(a), w)
                acc = d if acc is None else acc + d
                yield acc
        def emit_o(r, c, val):
            rs = slice(r * HS, (r + 1) * HS)
            o_b[slot, c, rs] = (ga_s[c, rs] + (1.0 - gate_s[rs]) * val).astype(BF16)
        def opieces():
            m = {}
            def second_tile():
                emit_o(0, 1, m[2] + m[4])
                emit_o(1, 1, (m[0] + m[5]) + (m[2] - m[1]))
                ocopy(t, slot, 1).start()
            for i in PORD:
                for acc in oprod(i):
                    m[i] = acc
                    yield
                if EE and i == PORD[3 + EE]:
                    second_tile()
            yield
            if not EE:
                second_tile()
            emit_o(1, 0, m[1] + m[3])
            emit_o(0, 0, (m[0] + m[6]) + (m[3] - m[4]))
            ocopy(t, slot, 0).start()
        gen = opieces()
        def piece(n=1):
            for _ in range(n):
                next(gen)

        rows = lax.broadcasted_iota(jnp.int32, (8, 128), 0)
        sgn = (1 - 2 * (rows & 1)).astype(F32)
        Fm = f_ref[...]
        Gm = g_ref[...]
        for c, (n0, n1, n2, n3, fts) in zip(CO, PP):
            cs = slice(c * 128, (c + 1) * 128)
            piece(n0)
            if c == PF:
                prefetch()
            kk = unpack(ak_b.bitcast(U32)[slot, c]).astype(F32)
            sh = shk[2 * t + c].astype(F32)
            ksf = kk * sh[0:1, :]
            for j in range(1, KS):
                kr = pltpu.roll(kk, j, 0)
                kr = jnp.concatenate([jnp.where(rows >= j, kr[:8], 0.0), kr[8:]], axis=0)
                ksf = ksf + kr * sh[j:j + 1, :]
            kv = (ksf * unpack(av_b.bitcast(U32)[slot, c]).astype(F32)).astype(BF16)
            for j in range(0, NCH, 4):
                r = dot_nt(Fm, jnp.concatenate([hk_b[slot, cs, (j + a) * C:(j + a + 1) * C] for a in range(4)], axis=0))
                for a in range(4):
                    hf[j + a] = r[:, a * 128:(a + 1) * 128]
            piece(n1)
            for j in range(0, NCH, 4):
                r = dot(Fm, jnp.concatenate([kv[(j + a) * C:(j + a + 1) * C] for a in range(4)], axis=1))
                for a in range(4):
                    uf[j + a] = r[:, a * 128:(a + 1) * 128]
            ga_s[c] = kv.astype(F32) * dd_s[pl.ds(2 * t + c, 1)]
            piece(n2)
            for ft in range(C // 8):
                re = slice(ft * 8, ft * 8 + 8)
                im = slice(C + ft * 8, C + ft * 8 + 8)
                hc = [hf[0, re]] + [hf[m, re] - sgn * hf[m - 1, im] for m in range(1, NCH)]
                hd = [hf[0, im]] + [hf[m, im] + sgn * hf[m - 1, re] for m in range(1, NCH)]
                ua = [uf[j, re] for j in range(NCH)]
                ub = [uf[j, im] for j in range(NCH)]
                def toep(u, h):
                    out = []
                    for i in range(NCH):
                        a = u[0] * h[i]
                        for j in range(1, i + 1):
                            a = a + u[j] * h[i - j]
                        out.append(a)
                    return out
                k1 = toep([a + b for a, b in zip(ua, ub)], hc)
                k2 = toep(ua, [d - c_ for c_, d in zip(hc, hd)])
                k3 = toep(ub, [d + c_ for c_, d in zip(hc, hd)])
                for i in range(NCH):
                    zf[i, re] = k1[i] - k3[i]
                    zf[i, im] = k1[i] + k2[i]
                if ft in fts:
                    piece()
            xcs = pl.ds(pl.multiple_of((2 * t + c) * 128, 128), 128)
            for j in range(0, NCH, 4):
                r = dot(Gm, jnp.concatenate([zf[j + a] for a in range(4)], axis=1).astype(BF16))
                for a in range(4):
                    ts = slice((j + a) * C, (j + a + 1) * C)
                    y = r[:, a * 128:(a + 1) * 128] + ga_s[c, ts]
                    ga_s[c, ts] = gate_s[ts] * (x_s[ts, xcs].astype(F32) * y)
                if j == 4:
                    piece(n3)
        for _ in gen:
            pass
        return carry
    lax.fori_loop(0, NT // 2, tile_step, 0)
    for t in range(NT // 2 - 2, NT // 2):
        for c in range(2):
            ocopy(t, t % 2, c).wait()

@jax.jit
def pallas_gated_mix__ssm_conv_h3__compressed_kv_cla__prompt_kernel(
        A_q, A_k, A_v, A_shift_k, A_ssm_k, A_ssm_D, B_x, B_c_kv, B_w_q, B_w_uk, B_w_uv, B_w_o, gate_w):
    any_ = pl.BlockSpec(memory_space=pl.ANY)
    vm = pl.BlockSpec(memory_space=pltpu.VMEM)
    out = pl.pallas_call(
        kernel,
        in_specs=[vm] * 5 + [any_] * 9,
        out_specs=any_,
        out_shape=jax.ShapeDtypeStruct((1, S, DM), BF16),
        scratch_shapes=[
            pltpu.VMEM((S, DM), BF16), pltpu.VMEM((S, DC), BF16),
            pltpu.VMEM((7, DM // 256, HS, 128), BF16), pltpu.VMEM((7, 7, QS, 128), BF16),
            pltpu.VMEM((2, DM, 128), U32), pltpu.VMEM((2, DC, 128), U32), pltpu.VMEM((2, DC, 128), U32),
            pltpu.VMEM((3, S, 128), BF16), pltpu.VMEM((2, 3, S, 128), BF16), pltpu.VMEM((2 * A_END, 128), BF16),
            pltpu.VMEM((S, 128), F32), pltpu.VMEM((S, 128), F32), pltpu.VMEM((4, 2, HS, 128), F32), pltpu.VMEM((4, QS, 128), F32), pltpu.VMEM((4, HS, 128), F32),
            pltpu.VMEM((S, 128), F32),
            pltpu.VMEM((2, 2, S, 128), BF16), pltpu.VMEM((2, 2, S, 128), BF16), pltpu.VMEM((2, 256, S), BF16),
            pltpu.VMEM((2, 2, H, HD, 128), BF16), pltpu.VMEM((2, 2, S, 128), BF16),
            pltpu.VMEM((NCH, 2 * C, 128), F32), pltpu.VMEM((NCH, 2 * C, 128), F32), pltpu.VMEM((NCH, 2 * C, 128), F32),
            pltpu.VMEM((2, S, 128), F32), pltpu.VMEM((NT, 128), F32), pltpu.VMEM((NT, 16, 128), F32),
            pltpu.SemaphoreType.DMA((4, 5)), pltpu.SemaphoreType.DMA((3, 2)), pltpu.SemaphoreType.DMA((7, 2)),
            pltpu.SemaphoreType.DMA((2, 2)),
        ],
        compiler_params=pltpu.CompilerParams(vmem_limit_bytes=120 * 1024 * 1024),
    )(gate_w.reshape(NT, 128), A_shift_k.T.reshape(KS, NT, 128).transpose(1, 0, 2), A_ssm_D.reshape(NT, 128), _F, _G,
      A_q, A_k, A_v, A_ssm_k, B_c_kv, B_w_q, B_w_uk, B_w_uv, B_w_o)
    return out
```

```python
import numpy as np
import jax
import jax.numpy as jnp
from jax import lax
import jax.experimental.pallas as pl
import jax.experimental.pallas.tpu as pltpu
import ml_dtypes

S, DM, H, HD, DC, KS = 2048, 1024, 32, 128, 512, 4
C = 128
NCH = S // C
NP = H // 2
NT = DM // 128
HS = S // 2
QS = S // 4
F32, BF16, U32 = jnp.float32, jnp.bfloat16, jnp.uint32
NTD = (((1,), (1,)), ((), ()))

BQ = 128
NG = HS // BQ
A_TMP = 0
A_CT = A_TMP + S + 4 * BQ
A_END = A_CT + 7 * NP * (HS // 2)
ONLY1 = 0
ONLY2 = 0
OR = 128
GT = 1
LAG = 0
REV = 3
CLAG = 2
TOK0 = 0
SPL = 0
CH = 0
PP = ((1,1,2,3,(1,3,5,7,9,11,13,15)),(2,1,2,1,(0,2,3,4,5,6,8)))
NOPRO = 0
PF = -1
CO = (1, 0)
EE = 1
AQ = 0
AO = 0
AI = 0
PB = (2,10,15,16)
PO = 0
UO = 3
PQ = ((0,), (1,), (2,), (3,))
CCH = 32
SL0 = (0,1,2,3,4,9,10,12,13,15)
SL1 = (0,13,14,16)

def _dft_consts():
    N = 2 * C
    f = np.arange(C, dtype=np.float64)[:, None] + 0.5
    t = np.arange(C, dtype=np.float64)[None, :]
    ang = 2 * np.pi * f * t / N
    Fm = np.concatenate([np.cos(ang), -np.sin(ang)], 0)
    Gm = np.concatenate([np.cos(ang).T, -np.sin(ang).T], 1) * (2.0 / N)
    return Fm.astype(ml_dtypes.bfloat16), Gm.astype(ml_dtypes.bfloat16)
_F, _G = _dft_consts()

def dot(a, b):
    return jnp.dot(a, b, preferred_element_type=F32)

def dot_nt(a, b):
    return lax.dot_general(a, b, NTD, preferred_element_type=F32)

def pack(x):
    return pltpu.bitcast(x.astype(BF16), U32)

def unpack(w):
    return pltpu.bitcast(w, BF16)

def halves(w):
    return pltpu.bitcast(w << 16, F32), pltpu.bitcast(w & jnp.uint32(0xFFFF0000), F32)

def lhs_ops(a11, a12, a21, a22):
    return [lambda: a11() + a22(), lambda: a21() + a22(), a11, a22,
            lambda: a11() + a12(), lambda: a21() - a11(), lambda: a12() - a22()]

def rhs_ops(b11, b12, b21, b22):
    return [lambda: b11() + b22(), b11, lambda: b12() - b22(), lambda: b21() - b11(),
            b22, lambda: b11() + b12(), lambda: b21() + b22()]

PORD = (2, 4, 1, 0, 5, 3, 6)
SKIP = (4, 10, 16)

def consume(i, v, emit, m, dyn, acc=0):
    if i == 2:
        m[0 + dyn] = v
    elif i == 4:
        emit(0, 1, m[0] + v)
        m[1 + dyn] = v
    elif i == 1:
        m[2 + dyn] = v
        if acc & 1:
            m[0 + dyn] = m[0] - v
    elif i == 0:
        m[3 + dyn] = v
        if acc & 2:
            m[1 + dyn] = v - m[1]
    elif i == 5:
        emit(1, 1, (m[0] if acc & 1 else m[0] - m[2]) + (m[3] + v))
    elif i == 3:
        emit(1, 0, m[2] + v)
        m[0 + dyn] = v
    else:
        emit(0, 0, (m[1] if acc & 2 else m[3] - m[1]) + (m[0] + v))

def kernel(gw, shk, ssmd, f_ref, g_ref, aq_hbm, ak_hbm, av_hbm, ssmk_hbm, c_hbm, wq_hbm, wk_hbm, wv_hbm, wo_hbm,
           o_hbm,
           x_s, c_s, xab, cab, wq_b, wk_b, wv_b, h0b, h1b, arb, s0, s1, mkv, mi, mq, gate_s, ak_b, av_b, hk_b, wo_b, o_b, uf, hf, zf, ga_s, dd_s, gw_s, wp,
           sem_x, sem_w, sem_t, sem_o):

    def wcopies(p, slot):
        return [pltpu.make_async_copy(src.bitcast(U32).at[:, p, :], dst.at[slot], sem_w.at[i, slot])
                for i, (src, dst) in enumerate(((wk_hbm, wk_b), (wv_hbm, wv_b), (wq_hbm, wq_b)))]

    def tcopies(t, slot):
        cps = [pltpu.make_async_copy(ssmk_hbm.at[pl.ds(pl.multiple_of(t * 256, 256), 256), :], hk_b.at[slot], sem_t.at[0, slot])]
        for c in range(2):
            cs = pl.ds(pl.multiple_of((2 * t + c) * 128, 128), 128)
            cps += [pltpu.make_async_copy(ak_hbm.at[0, :, cs], ak_b.at[slot, c], sem_t.at[1 + c, slot]),
                    pltpu.make_async_copy(av_hbm.at[0, :, cs], av_b.at[slot, c], sem_t.at[3 + c, slot]),
                    pltpu.make_async_copy(wo_hbm.at[:, :, cs], wo_b.at[slot, c], sem_t.at[5 + c, slot])]
        return cps

    def ocopy(t, slot, c):
        cs = pl.ds(pl.multiple_of((2 * t + c) * 128, 128), 128)
        return pltpu.make_async_copy(o_b.at[slot, c], o_hbm.at[0, :, cs], sem_o.at[c, slot])

    RB = 128
    def rcopies(src, dst, which, r):
        rows = lambda a: pl.ds(pl.multiple_of(a * QS + r * RB, RB), RB)
        return [pltpu.make_async_copy(src.at[0, rows(a)], dst.at[rows(a)], sem_x.at[which, a, r]) for a in range(4)]
    ccopies = lambda r: rcopies(c_hbm, c_s, 0, r)
    xcopies = lambda r: rcopies(aq_hbm, x_s, 1, r)
    w0 = wcopies(0, 0)
    for cp in w0[:2] + ccopies(0):
        cp.start()

    qscale = float((HD ** -0.5) * np.log2(np.e))

    ar, xa, ca = arb.bitcast(U32), xab.bitcast(U32), cab.bitcast(U32)
    h0, h1 = h0b.bitcast(U32), h1b.bitcast(U32)

    def qkv_load(slot, which, hh, r0, n):
        rs = slice(r0 // 2, (r0 + n) // 2)
        return h0[which, rs] if hh == 0 else h1[slot, which, rs]

    def qkv_store(slot, which, hh, r0, val):
        rs = pl.ds(pl.multiple_of(r0, 128), val.shape[0])
        if hh == 0:
            h0b[which, rs] = val.astype(BF16)
        else:
            h1b[slot, which, rs] = val.astype(BF16)

    def proj_pieces(slot, dyn):
        def q_piece(i):
            def f():
                blk = lambda r, c: (lambda: halves(wq_b[slot, r * (DM // 2):(r + 1) * (DM // 2)])[c])
                w = rhs_ops(blk(0, 0), blk(0, 1), blk(1, 0), blk(1, 1))[i]().astype(BF16)
                a = jnp.concatenate([xa[i, b] for b in range(DM // 256)], axis=1)
                emit = lambda r, c, val: qkv_store(slot, 0, c, r * HS, val * qscale)
                consume(i, dot(unpack(a), w), emit, mq, dyn, AQ)
            return f
        def kv_piece(i):
            def f():
                def outer(kk, nn):
                    raw = lambda r, c: (lambda: halves((wk_b, wv_b)[nn][slot, (2 * r + kk) * 128:(2 * r + kk + 1) * 128])[c])
                    return rhs_ops(raw(0, 0), raw(0, 1), raw(1, 0), raw(1, 1))[i]
                rops = rhs_ops(outer(0, 0), outer(0, 1), outer(1, 0), outer(1, 1))
                def inner_emit(r2, c2, v):
                    def emit(r, c, val):
                        for t in range(0, QS, 128):
                            blk = val[t:t + 128]
                            qkv_store(slot, 1 + c2, c, r * HS + r2 * QS + t, blk.T if c2 else blk)
                    consume(i, v, emit, mkv.at[:, c2, r2 * QS:(r2 + 1) * QS], dyn, AO)
                for j in PORD:
                    w = rops[j]().astype(BF16)
                    v = jnp.concatenate([dot(unpack(ca[i, j, a * QS // 8:(a + 1) * QS // 8]), w) for a in range(4)], axis=0)
                    consume(j, v, inner_emit, mi, dyn, AI)
            return f
        return [kv_piece(i) for i in PORD], [q_piece(i) for i in PORD]

    def scores(slot, hh, i, buf, dyn):
        L = (i + 1) * BQ
        q = unpack(qkv_load(slot, 0, hh, i * BQ, BQ))
        m = None
        n = L // 4
        for a in range(4):
            st = dot_nt(unpack(qkv_load(slot, 1, hh, a * n, n)), q)
            d0 = max(L - BQ - a * n, 0)
            if d0 < n:
                row = lax.broadcasted_iota(jnp.int32, (n - d0, BQ), 0) + (a * n + d0 - (L - BQ))
                col = lax.broadcasted_iota(jnp.int32, (n - d0, BQ), 1)
                dg = jnp.where(row <= col, st[d0:], -1e9)
                st = dg if d0 == 0 else jnp.concatenate([st[:d0], dg], axis=0)
            (s0, s1)[buf][pl.ds(pl.multiple_of(a * n + dyn, 32), n)] = st
            ma = jnp.max(st.reshape(n // 8, 8, BQ), axis=0)
            m = ma if m is None else jnp.maximum(m, ma)
        return jnp.broadcast_to(jnp.max(m, axis=0, keepdims=True), (8, BQ))

    def weighted(slot, hh, i, buf, m, never, dyn2):
        l = ot = None
        for t0 in range(0, i + 1, GT):
            nt = min(GT, i + 1 - t0)
            pj = jnp.exp2((s0, s1)[buf][t0 * BQ:(t0 + nt) * BQ] - jnp.tile(m, (nt * BQ // 8, 1)))
            lj = jnp.sum(pj.reshape(nt * BQ // 8, 8, BQ), axis=0)
            if LAG and l is not None:
                pj = jnp.concatenate([jnp.where(never, l, pj[:8]), pj[8:]], axis=0)
            l = lj if l is None else l + lj
            pt = pj.astype(BF16)
            ns = 1 if nt == 4 else 2 if nt == 2 else 4
            if SPL and t0 < (i + 1) // SPL * SPL:
                ns = 4 // SPL
            parts = []
            for a in range(ns):
                vt = jnp.concatenate([qkv_load(slot, 2, hh, t * 128 + a * HD // ns, HD // ns)
                                      for t in range(t0, t0 + nt)], axis=1)
                parts.append(dot(unpack(vt), pt))
            d = jnp.concatenate(parts, axis=0)
            ot = d if ot is None else ot + d
        l = jnp.sum(l, axis=0, keepdims=True)
        r = pl.reciprocal(l, approx=True)
        r = r * (2.0 - l * r)
        return (ot * r).T

    def attention(p, slot, pieces):
        pieces = list(pieces)
        dyn = lax.shift_right_logical(p, 8)
        never = jnp.broadcast_to(p, (8, BQ)) < 0
        dyn2 = lax.shift_right_logical(p, 9)
        tmp = lambda i: pl.ds(pl.multiple_of(A_TMP + i * BQ + dyn, 64), BQ)
        gs = lambda hh: range(NG) if not (REV >> hh) & 1 else reversed(range(NG))
        units = [(hh, g + a * NG) for hh in range(2) for g in gs(hh) for a in range(2)]
        if UO == 1:
            units[:2 * NG] = [(0, i) for g in range(NG) for i in (g, 2 * NG - 1 - g)]
        elif UO == 2:
            units[:2 * NG] = [(0, i) for i in range(2 * NG)]
        elif UO == 3:
            units[:2 * NG] = [(0, i) for g in range(NG) for i in (2 * NG - 1 - g, g)]
        slot1 = lambda i: 2 * NG + (i % 2) * 2 + i // NG

        nxt = scores(slot, *units[0], 0, dyn)
        tok = {}
        for u, (hh, i) in enumerate(units):
            cur = nxt
            here = pieces and (u in SL0 or u - 2 * NG in SL1)
            if here and u in PB:
                pieces.pop(0)()
            if u + 1 < len(units):
                nxt = scores(slot, *units[u + 1], (u + 1) % 2, dyn)
            if here and u not in PB:
                pieces.pop(0)()
            if u in tok:
                cur = jnp.where(never, tok[u], cur)
            o = weighted(slot, hh, i, u % 2, cur, never, dyn2)
            if hh == 0 or i < NG:
                ar[tmp(i if hh == 0 else slot1(i))] = pltpu.bitcast(o, U32)
            else:
                g = i - NG
                for rc in range(0, BQ, CCH):
                    a11, a12, a21 = (pltpu.bitcast(ar[pl.ds(pl.multiple_of(A_TMP + t * BQ + rc + dyn, 16), CCH)], F32)
                                     for t in (g, slot1(g), i))
                    for j, op in enumerate(lhs_ops(lambda: a11, lambda: a12, lambda: a21, lambda: o[rc:rc + CCH])):
                        base = A_CT + (j * NP + p) * (HS // 2) + g * (BQ // 2)
                        arb[pl.ds(pl.multiple_of(base * 2 + rc, 16), CCH)] = op().astype(BF16)
            if CLAG and (hh == 1 and i >= NG or TOK0 and u % 2):
                tok[u + CLAG] = pltpu.bitcast(ar[pl.ds(pl.multiple_of(A_TMP + dyn2, 8), 8)], F32)
        while pieces:
            pieces.pop(0)()

    def x_combos(r0, n):
        rows = [pl.ds(pl.multiple_of(a * HS + r0, n), n) for a in range(2)]
        gl = [None, None]
        for b in range(NT // 2):
            blk = [[x_s[rows[a], (c * NT // 2 + b) * 128:(c * NT // 2 + b + 1) * 128].astype(F32) for c in range(2)]
                   for a in range(2)]
            ops = lhs_ops(lambda: blk[0][0], lambda: blk[0][1], lambda: blk[1][0], lambda: blk[1][1])
            for j, op in enumerate(ops):
                xab[j, b, rows[0]] = op().astype(BF16)
            for a in range(2):
                for c in range(2):
                    term = blk[a][c] * gw_s[c * NT // 2 + b, 0:n]
                    gl[a] = term if gl[a] is None else gl[a] + term
        for a in range(2):
            gate_s[rows[a]] = jnp.broadcast_to(jax.nn.sigmoid(jnp.sum(gl[a], axis=-1, keepdims=True)), (n, 128))

    def c_combos(r0, n):
        quarter = [c_s[pl.ds(pl.multiple_of(a * QS + r0, n), n)].astype(F32) for a in range(4)]
        for i in range(7):
            def outer(r2, kk):
                raw = lambda r, c: (lambda: quarter[2 * r + r2][:, (2 * c + kk) * 128:(2 * c + kk + 1) * 128])
                val = lhs_ops(raw(0, 0), raw(0, 1), raw(1, 0), raw(1, 1))[i]()
                return lambda: val
            for j, op in enumerate(lhs_ops(outer(0, 0), outer(0, 1), outer(1, 0), outer(1, 1))):
                cab[i, j, pl.ds(pl.multiple_of(r0, n), n)] = op().astype(BF16)

    dd_s[...] = ssmd[...].astype(F32)
    for b in range(NT):
        gw_s[b] = jnp.broadcast_to(gw[...].astype(F32)[b:b + 1], (16, 128))
    NC = QS // RB
    for cp in w0[:2] + ccopies(0):
        cp.wait()
    for cp in w0[2:] + [cp for r in range(1, NC) for cp in ccopies(r)]:
        cp.start()
    rows_of = lambda ref, r: unpack(ref.bitcast(U32)[pl.ds(pl.multiple_of(r // 2, RB // 2), RB // 2)])
    def pro_kv(r, carry):
        r0 = r * RB
        @pl.when(r > 0)
        def _():
            for cp in ccopies(r):
                cp.wait()
            for cp in xcopies(r - 1):
                cp.start()
        w = unpack(jnp.concatenate([wp.bitcast(U32)[n, 0:DC // 2] for n in range(4)], axis=1))
        for a in range(4):
            val = dot(rows_of(c_s, a * QS + r0), w)
            for n in range(4):
                blk = val[:, n * 128:(n + 1) * 128]
                qkv_store(0, 1 + n // 2, n % 2, a * QS + r0, blk.T if n // 2 else blk)
            for b in range(a * RB // 4, (a + 1) * RB // 4, 16):
                c_combos(r0 + b, 16)
        return carry
    def pro_q(r, carry):
        r0 = r * RB
        for cp in xcopies(r):
            cp.wait()
        w = unpack(jnp.concatenate([wp.bitcast(U32)[n] for n in range(2)], axis=1))
        for a in range(4):
            val = dot(rows_of(x_s, a * QS + r0), w) * qscale
            for hh in range(2):
                qkv_store(0, 0, hh, a * QS + r0, val[:, hh * 128:(hh + 1) * 128])
            for b in range(a % 2 * RB // 2, (a % 2 + 1) * RB // 2, 16):
                x_combos(a // 2 * QS + r0 + b, 16)
        return carry
    for n, w in enumerate(halves(wk_b[0]) + halves(wv_b[0])):
        wp[n, 0:DC] = w.astype(BF16)
    lax.fori_loop(0, NC, pro_kv, 0) if not NOPRO else None
    w0[2].wait()
    for cp in xcopies(NC - 1):
        cp.start()
    for cp in wcopies(1, 1):
        cp.start()
    for n, w in enumerate(halves(wq_b[0])):
        wp[n] = w.astype(BF16)
    lax.fori_loop(0, NC, pro_q, 0) if not NOPRO else None

    def pair_step(p, carry):
        slot = p % 2
        for cp in wcopies(p + 1, 1 - slot):
            cp.wait()
        @pl.when(p + 2 < NP)
        def _():
            for cp in wcopies(p + 2, slot):
                cp.start()
        @pl.when(p == NP - 2)
        def _():
            for cp in tcopies(0, 0):
                cp.start()
        kvp, qp = proj_pieces(1 - slot, lax.shift_right_logical(p, 8))
        attention(p, slot, [f for pair in (zip(kvp, qp) if PO == 0 else zip(qp, kvp)) for f in pair])
        return carry + 1
    last = lax.fori_loop(0, NP - 1, pair_step, 0) if not ONLY2 else None
    if ONLY1:
        return
    if not ONLY2:
        attention(last, (NP - 1) % 2, [])

    def tile_step(t, carry):
        slot = t % 2
        for cp in tcopies(t, slot):
            cp.wait()
        def prefetch():
            @pl.when(t + 1 < NT // 2)
            def _():
                for cp in tcopies(t + 1, 1 - slot):
                    cp.start()
            @pl.when(t >= 2)
            def _():
                for c in range(2):
                    ocopy(t - 2, slot, c).wait()
        if PF < 0:
            prefetch()

        KC = 4
        def oprod(i):
            acc = None
            for j0 in range(0, NP, KC):
                def wblk(r, c):
                    return lambda: jnp.concatenate(
                        [unpack(wo_b.bitcast(U32)[slot, c, 2 * j + r]) for j in range(j0, j0 + KC)], axis=0).astype(F32)
                w = rhs_ops(wblk(0, 0), wblk(0, 1), wblk(1, 0), wblk(1, 1))[i]().astype(BF16)
                a = jnp.concatenate([ar[pl.ds(A_CT + (i * NP + j) * (HS // 2), HS // 2)] for j in range(j0, j0 + KC)], axis=1)
                d = dot(unpack(a), w)
                acc = d if acc is None else acc + d
                yield acc
        def emit_o(r, c, val):
            rs = slice(r * HS, (r + 1) * HS)
            o_b[slot, c, rs] = (ga_s[c, rs] + (1.0 - gate_s[rs]) * val).astype(BF16)
        def opieces():
            m = {}
            def second_tile():
                emit_o(0, 1, m[2] + m[4])
                emit_o(1, 1, (m[0] + m[5]) + (m[2] - m[1]))
                ocopy(t, slot, 1).start()
            for i in PORD:
                for acc in oprod(i):
                    m[i] = acc
                    yield
                if EE and i == PORD[3 + EE]:
                    second_tile()
            yield
            if not EE:
                second_tile()
            emit_o(1, 0, m[1] + m[3])
            emit_o(0, 0, (m[0] + m[6]) + (m[3] - m[4]))
            ocopy(t, slot, 0).start()
        gen = opieces()
        def piece(n=1):
            for _ in range(n):
                next(gen)

        rows = lax.broadcasted_iota(jnp.int32, (8, 128), 0)
        sgn = (1 - 2 * (rows & 1)).astype(F32)
        Fm = f_ref[...]
        Gm = g_ref[...]
        for c, (n0, n1, n2, n3, fts) in zip(CO, PP):
            cs = slice(c * 128, (c + 1) * 128)
            piece(n0)
            if c == PF:
                prefetch()
            kk = unpack(ak_b.bitcast(U32)[slot, c]).astype(F32)
            sh = shk[2 * t + c].astype(F32)
            ksf = kk * sh[0:1, :]
            for j in range(1, KS):
                kr = pltpu.roll(kk, j, 0)
                kr = jnp.concatenate([jnp.where(rows >= j, kr[:8], 0.0), kr[8:]], axis=0)
                ksf = ksf + kr * sh[j:j + 1, :]
            kv = (ksf * unpack(av_b.bitcast(U32)[slot, c]).astype(F32)).astype(BF16)
            for j in range(0, NCH, 4):
                r = dot_nt(Fm, jnp.concatenate([hk_b[slot, cs, (j + a) * C:(j + a + 1) * C] for a in range(4)], axis=0))
                for a in range(4):
                    hf[j + a] = r[:, a * 128:(a + 1) * 128]
            piece(n1)
            for j in range(0, NCH, 4):
                r = dot(Fm, jnp.concatenate([kv[(j + a) * C:(j + a + 1) * C] for a in range(4)], axis=1))
                for a in range(4):
                    uf[j + a] = r[:, a * 128:(a + 1) * 128]
            ga_s[c] = kv.astype(F32) * dd_s[pl.ds(2 * t + c, 1)]
            piece(n2)
            for ft in range(C // 8):
                re = slice(ft * 8, ft * 8 + 8)
                im = slice(C + ft * 8, C + ft * 8 + 8)
                hc = [hf[0, re]] + [hf[m, re] - sgn * hf[m - 1, im] for m in range(1, NCH)]
                hd = [hf[0, im]] + [hf[m, im] + sgn * hf[m - 1, re] for m in range(1, NCH)]
                ua = [uf[j, re] for j in range(NCH)]
                ub = [uf[j, im] for j in range(NCH)]
                def toep(u, h):
                    out = []
                    for i in range(NCH):
                        a = u[0] * h[i]
                        for j in range(1, i + 1):
                            a = a + u[j] * h[i - j]
                        out.append(a)
                    return out
                k1 = toep([a + b for a, b in zip(ua, ub)], hc)
                k2 = toep(ua, [d - c_ for c_, d in zip(hc, hd)])
                k3 = toep(ub, [d + c_ for c_, d in zip(hc, hd)])
                for i in range(NCH):
                    zf[i, re] = k1[i] - k3[i]
                    zf[i, im] = k1[i] + k2[i]
                if ft in fts:
                    piece()
            xcs = pl.ds(pl.multiple_of((2 * t + c) * 128, 128), 128)
            for j in range(0, NCH, 4):
                r = dot(Gm, jnp.concatenate([zf[j + a] for a in range(4)], axis=1).astype(BF16))
                for a in range(4):
                    ts = slice((j + a) * C, (j + a + 1) * C)
                    y = r[:, a * 128:(a + 1) * 128] + ga_s[c, ts]
                    ga_s[c, ts] = gate_s[ts] * (x_s[ts, xcs].astype(F32) * y)
                if j == 4:
                    piece(n3)
        for _ in gen:
            pass
        return carry
    lax.fori_loop(0, NT // 2, tile_step, 0)
    for t in range(NT // 2 - 2, NT // 2):
        for c in range(2):
            ocopy(t, t % 2, c).wait()

@jax.jit
def pallas_gated_mix__ssm_conv_h3__compressed_kv_cla__prompt_kernel(
        A_q, A_k, A_v, A_shift_k, A_ssm_k, A_ssm_D, B_x, B_c_kv, B_w_q, B_w_uk, B_w_uv, B_w_o, gate_w):
    any_ = pl.BlockSpec(memory_space=pl.ANY)
    vm = pl.BlockSpec(memory_space=pltpu.VMEM)
    out = pl.pallas_call(
        kernel,
        in_specs=[vm] * 5 + [any_] * 9,
        out_specs=any_,
        out_shape=jax.ShapeDtypeStruct((1, S, DM), BF16),
        scratch_shapes=[
            pltpu.VMEM((S, DM), BF16), pltpu.VMEM((S, DC), BF16),
            pltpu.VMEM((7, DM // 256, HS, 128), BF16), pltpu.VMEM((7, 7, QS, 128), BF16),
            pltpu.VMEM((2, DM, 128), U32), pltpu.VMEM((2, DC, 128), U32), pltpu.VMEM((2, DC, 128), U32),
            pltpu.VMEM((3, S, 128), BF16), pltpu.VMEM((2, 3, S, 128), BF16), pltpu.VMEM((2 * A_END, 128), BF16),
            pltpu.VMEM((S, 128), F32), pltpu.VMEM((S, 128), F32), pltpu.VMEM((4, 2, HS, 128), F32), pltpu.VMEM((4, QS, 128), F32), pltpu.VMEM((4, HS, 128), F32),
            pltpu.VMEM((S, 128), F32),
            pltpu.VMEM((2, 2, S, 128), BF16), pltpu.VMEM((2, 2, S, 128), BF16), pltpu.VMEM((2, 256, S), BF16),
            pltpu.VMEM((2, 2, H, HD, 128), BF16), pltpu.VMEM((2, 2, S, 128), BF16),
            pltpu.VMEM((NCH, 2 * C, 128), F32), pltpu.VMEM((NCH, 2 * C, 128), F32), pltpu.VMEM((NCH, 2 * C, 128), F32),
            pltpu.VMEM((2, S, 128), F32), pltpu.VMEM((NT, 128), F32), pltpu.VMEM((NT, 16, 128), F32), pltpu.VMEM((4, DM, 128), BF16),
            pltpu.SemaphoreType.DMA((2, 4, 4)), pltpu.SemaphoreType.DMA((3, 2)), pltpu.SemaphoreType.DMA((7, 2)),
            pltpu.SemaphoreType.DMA((2, 2)),
        ],
        compiler_params=pltpu.CompilerParams(vmem_limit_bytes=120 * 1024 * 1024),
    )(gate_w.reshape(NT, 128), A_shift_k.T.reshape(KS, NT, 128).transpose(1, 0, 2), A_ssm_D.reshape(NT, 128), _F, _G,
      A_q, A_k, A_v, A_ssm_k, B_c_kv, B_w_q, B_w_uk, B_w_uv, B_w_o)
    return out
```

```python
import numpy as np
import jax
import jax.numpy as jnp
from jax import lax
import jax.experimental.pallas as pl
import jax.experimental.pallas.tpu as pltpu
import ml_dtypes

S, DM, H, HD, DC, KS = 2048, 1024, 32, 128, 512, 4
C = 128
NCH = S // C
NP = H // 2
NT = DM // 128
HS = S // 2
QS = S // 4
F32, BF16, U32 = jnp.float32, jnp.bfloat16, jnp.uint32
NTD = (((1,), (1,)), ((), ()))

BQ = 128
NG = HS // BQ
A_TMP = 0
A_CT = A_TMP + S + 4 * BQ
A_END = A_CT + 7 * NP * (HS // 2)
ONLY1 = 0
ONLY2 = 0
OR = 128
GT = 1
LAG = 0
REV = 3
CLAG = 2
TOK0 = 0
SPL = 0
CH = 0
PP = ((1,1,2,3,(1,3,5,7,9,11,13,15)),(2,1,2,1,(0,2,3,4,5,6,8)))
NOPRO = 0
RC = 64
PF = -1
CO = (1, 0)
EE = 1
AQ = 0
AO = 0
AI = 0
PB = (2,10,12,15,16)
PO = 0
UO = 1
PQ = ((0,), (1,), (2,), (3,))
CCH = 32
SL0 = (0,1,2,3,4,8,9,13,14,15)
SL1 = (4,13,14,16)

def _dft_consts():
    N = 2 * C
    f = np.arange(C, dtype=np.float64)[:, None] + 0.5
    t = np.arange(C, dtype=np.float64)[None, :]
    ang = 2 * np.pi * f * t / N
    Fm = np.concatenate([np.cos(ang), -np.sin(ang)], 0)
    Gm = np.concatenate([np.cos(ang).T, -np.sin(ang).T], 1) * (2.0 / N)
    return Fm.astype(ml_dtypes.bfloat16), Gm.astype(ml_dtypes.bfloat16)
_F, _G = _dft_consts()

def dot(a, b):
    return jnp.dot(a, b, preferred_element_type=F32)

def dot_nt(a, b):
    return lax.dot_general(a, b, NTD, preferred_element_type=F32)

def pack(x):
    return pltpu.bitcast(x.astype(BF16), U32)

def unpack(w):
    return pltpu.bitcast(w, BF16)

def halves(w):
    return pltpu.bitcast(w << 16, F32), pltpu.bitcast(w & jnp.uint32(0xFFFF0000), F32)

def lhs_ops(a11, a12, a21, a22):
    return [lambda: a11() + a22(), lambda: a21() + a22(), a11, a22,
            lambda: a11() + a12(), lambda: a21() - a11(), lambda: a12() - a22()]

def rhs_ops(b11, b12, b21, b22):
    return [lambda: b11() + b22(), b11, lambda: b12() - b22(), lambda: b21() - b11(),
            b22, lambda: b11() + b12(), lambda: b21() + b22()]

PORD = (2, 4, 1, 0, 5, 3, 6)
SKIP = (4, 10, 16)

def consume(i, v, emit, m, dyn, acc=0):
    if i == 2:
        m[0 + dyn] = v
    elif i == 4:
        emit(0, 1, m[0] + v)
        m[1 + dyn] = v
    elif i == 1:
        m[2 + dyn] = v
        if acc & 1:
            m[0 + dyn] = m[0] - v
    elif i == 0:
        m[3 + dyn] = v
        if acc & 2:
            m[1 + dyn] = v - m[1]
    elif i == 5:
        emit(1, 1, (m[0] if acc & 1 else m[0] - m[2]) + (m[3] + v))
    elif i == 3:
        emit(1, 0, m[2] + v)
        m[0 + dyn] = v
    else:
        emit(0, 0, (m[1] if acc & 2 else m[3] - m[1]) + (m[0] + v))

def kernel(gw, shk, ssmd, f_ref, g_ref, aq_hbm, ak_hbm, av_hbm, ssmk_hbm, c_hbm, wq_hbm, wk_hbm, wv_hbm, wo_hbm,
           o_hbm,
           x_s, c_s, xab, cab, wq_b, wk_b, wv_b, h0b, h1b, arb, s0, s1, mkv, mi, mq, gate_s, ak_b, av_b, hk_b, wo_b, o_b, uf, hf, zf, ga_s, dd_s, gw_s, wp,
           sem_x, sem_w, sem_t, sem_o):

    def wcopies(p, slot):
        return [pltpu.make_async_copy(src.bitcast(U32).at[:, p, :], dst.at[slot], sem_w.at[i, slot])
                for i, (src, dst) in enumerate(((wk_hbm, wk_b), (wv_hbm, wv_b), (wq_hbm, wq_b)))]

    def tcopies(t, slot):
        cps = [pltpu.make_async_copy(ssmk_hbm.at[pl.ds(pl.multiple_of(t * 256, 256), 256), :], hk_b.at[slot], sem_t.at[0, slot])]
        for c in range(2):
            cs = pl.ds(pl.multiple_of((2 * t + c) * 128, 128), 128)
            cps += [pltpu.make_async_copy(ak_hbm.at[0, :, cs], ak_b.at[slot, c], sem_t.at[1 + c, slot]),
                    pltpu.make_async_copy(av_hbm.at[0, :, cs], av_b.at[slot, c], sem_t.at[3 + c, slot]),
                    pltpu.make_async_copy(wo_hbm.at[:, :, cs], wo_b.at[slot, c], sem_t.at[5 + c, slot])]
        return cps

    def ocopy(t, slot, c):
        cs = pl.ds(pl.multiple_of((2 * t + c) * 128, 128), 128)
        return pltpu.make_async_copy(o_b.at[slot, c], o_hbm.at[0, :, cs], sem_o.at[c, slot])

    RB = 128
    def rcopies(src, dst, which, r):
        rows = lambda a: pl.ds(pl.multiple_of(a * QS + r * RB, RB), RB)
        return [pltpu.make_async_copy(src.at[0, rows(a)], dst.at[rows(a)], sem_x.at[which, a, r]) for a in range(4)]
    ccopies = lambda r: rcopies(c_hbm, c_s, 0, r)
    xcopies = lambda r: rcopies(aq_hbm, x_s, 1, r)
    w0 = wcopies(0, 0)
    for cp in w0[:2] + ccopies(0):
        cp.start()

    qscale = float((HD ** -0.5) * np.log2(np.e))

    ar, xa, ca = arb.bitcast(U32), xab.bitcast(U32), cab.bitcast(U32)
    h0, h1 = h0b.bitcast(U32), h1b.bitcast(U32)

    def qkv_load(slot, which, hh, r0, n):
        rs = slice(r0 // 2, (r0 + n) // 2)
        return h0[which, rs] if hh == 0 else h1[slot, which, rs]

    def qkv_store(slot, which, hh, r0, val):
        rs = pl.ds(pl.multiple_of(r0, 32), val.shape[0])
        if hh == 0:
            h0b[which, rs] = val.astype(BF16)
        else:
            h1b[slot, which, rs] = val.astype(BF16)

    def proj_pieces(slot, dyn):
        def q_piece(i):
            def f():
                blk = lambda r, c: (lambda: halves(wq_b[slot, r * (DM // 2):(r + 1) * (DM // 2)])[c])
                w = rhs_ops(blk(0, 0), blk(0, 1), blk(1, 0), blk(1, 1))[i]().astype(BF16)
                a = jnp.concatenate([xa[i, b] for b in range(DM // 256)], axis=1)
                emit = lambda r, c, val: qkv_store(slot, 0, c, r * HS, val * qscale)
                consume(i, dot(unpack(a), w), emit, mq, dyn, AQ)
            return f
        def kv_piece(i):
            def f():
                def outer(kk, nn):
                    raw = lambda r, c: (lambda: halves((wk_b, wv_b)[nn][slot, (2 * r + kk) * 128:(2 * r + kk + 1) * 128])[c])
                    return rhs_ops(raw(0, 0), raw(0, 1), raw(1, 0), raw(1, 1))[i]
                rops = rhs_ops(outer(0, 0), outer(0, 1), outer(1, 0), outer(1, 1))
                def inner_emit(r2, c2, v):
                    def emit(r, c, val):
                        for t in range(0, QS, 128):
                            blk = val[t:t + 128]
                            qkv_store(slot, 1 + c2, c, r * HS + r2 * QS + t, blk.T if c2 else blk)
                    consume(i, v, emit, mkv.at[:, c2, r2 * QS:(r2 + 1) * QS], dyn, AO)
                if RC == 0:
                    for j in PORD:
                        w = rops[j]().astype(BF16)
                        v = jnp.concatenate([dot(unpack(ca[i, j, a * QS // 8:(a + 1) * QS // 8]), w) for a in range(4)], axis=0)
                        consume(j, v, inner_emit, mi, dyn, AI)
                    return
                for j in PORD:
                    wp[dyn, j * 128:(j + 1) * 128] = rops[j]().astype(BF16)
                for t0 in range(0, QS, 128):
                    blocks = {}
                    for a in range(t0, t0 + 128, RC):
                        v = {j: dot(unpack(ca[i, j, a // 2:(a + RC) // 2]), unpack(wp.bitcast(U32)[0, j * 64:(j + 1) * 64]))
                             for j in PORD}
                        for key, val in (((0, 1), v[2] + v[4]), ((1, 1), (v[2] - v[1]) + (v[0] + v[5])),
                                         ((1, 0), v[1] + v[3]), ((0, 0), (v[0] - v[4]) + (v[3] + v[6]))):
                            r2, c2 = key
                            def emit(r, c, val, r2=r2, c2=c2, a=a):
                                if c2 == 0:
                                    qkv_store(slot, 1, c, r * HS + r2 * QS + a, val)
                                else:
                                    blocks.setdefault((r, c, r2), []).append(val)
                            consume(i, val, emit, mkv.at[:, c2, r2 * QS + a:r2 * QS + a + RC], dyn, AO)
                    for (r, c, r2), vals in blocks.items():
                        qkv_store(slot, 2, c, r * HS + r2 * QS + t0, jnp.concatenate(vals, axis=0).T)
            return f
        return [kv_piece(i) for i in PORD], [q_piece(i) for i in PORD]

    def scores(slot, hh, i, buf, dyn):
        L = (i + 1) * BQ
        q = unpack(qkv_load(slot, 0, hh, i * BQ, BQ))
        m = None
        n = L // 4
        for a in range(4):
            st = dot_nt(unpack(qkv_load(slot, 1, hh, a * n, n)), q)
            d0 = max(L - BQ - a * n, 0)
            if d0 < n:
                row = lax.broadcasted_iota(jnp.int32, (n - d0, BQ), 0) + (a * n + d0 - (L - BQ))
                col = lax.broadcasted_iota(jnp.int32, (n - d0, BQ), 1)
                dg = jnp.where(row <= col, st[d0:], -1e9)
                st = dg if d0 == 0 else jnp.concatenate([st[:d0], dg], axis=0)
            (s0, s1)[buf][pl.ds(pl.multiple_of(a * n + dyn, 32), n)] = st
            ma = jnp.max(st.reshape(n // 8, 8, BQ), axis=0)
            m = ma if m is None else jnp.maximum(m, ma)
        return jnp.broadcast_to(jnp.max(m, axis=0, keepdims=True), (8, BQ))

    def weighted(slot, hh, i, buf, m, never, dyn2):
        l = ot = None
        for t0 in range(0, i + 1, GT):
            nt = min(GT, i + 1 - t0)
            pj = jnp.exp2((s0, s1)[buf][t0 * BQ:(t0 + nt) * BQ] - jnp.tile(m, (nt * BQ // 8, 1)))
            lj = jnp.sum(pj.reshape(nt * BQ // 8, 8, BQ), axis=0)
            if LAG and l is not None:
                pj = jnp.concatenate([jnp.where(never, l, pj[:8]), pj[8:]], axis=0)
            l = lj if l is None else l + lj
            pt = pj.astype(BF16)
            ns = 1 if nt == 4 else 2 if nt == 2 else 4
            if SPL and t0 < (i + 1) // SPL * SPL:
                ns = 4 // SPL
            parts = []
            for a in range(ns):
                vt = jnp.concatenate([qkv_load(slot, 2, hh, t * 128 + a * HD // ns, HD // ns)
                                      for t in range(t0, t0 + nt)], axis=1)
                parts.append(dot(unpack(vt), pt))
            d = jnp.concatenate(parts, axis=0)
            ot = d if ot is None else ot + d
        l = jnp.sum(l, axis=0, keepdims=True)
        r = pl.reciprocal(l, approx=True)
        r = r * (2.0 - l * r)
        return (ot * r).T

    def attention(p, slot, pieces):
        pieces = list(pieces)
        dyn = lax.shift_right_logical(p, 8)
        never = jnp.broadcast_to(p, (8, BQ)) < 0
        dyn2 = lax.shift_right_logical(p, 9)
        tmp = lambda i: pl.ds(pl.multiple_of(A_TMP + i * BQ + dyn, 64), BQ)
        gs = lambda hh: range(NG) if not (REV >> hh) & 1 else reversed(range(NG))
        units = [(hh, g + a * NG) for hh in range(2) for g in gs(hh) for a in range(2)]
        if UO == 1:
            units[:2 * NG] = [(0, i) for g in range(NG) for i in (g, 2 * NG - 1 - g)]
        elif UO == 2:
            units[:2 * NG] = [(0, i) for i in range(2 * NG)]
        elif UO == 3:
            units[:2 * NG] = [(0, i) for g in range(NG) for i in (2 * NG - 1 - g, g)]
        slot1 = lambda i: 2 * NG + (i % 2) * 2 + i // NG

        nxt = scores(slot, *units[0], 0, dyn)
        tok = {}
        for u, (hh, i) in enumerate(units):
            cur = nxt
            here = pieces and (u in SL0 or u - 2 * NG in SL1)
            if here and u in PB:
                pieces.pop(0)()
            if u + 1 < len(units):
                nxt = scores(slot, *units[u + 1], (u + 1) % 2, dyn)
            if here and u not in PB:
                pieces.pop(0)()
            if u in tok:
                cur = jnp.where(never, tok[u], cur)
            o = weighted(slot, hh, i, u % 2, cur, never, dyn2)
            if hh == 0 or i < NG:
                ar[tmp(i if hh == 0 else slot1(i))] = pltpu.bitcast(o, U32)
            else:
                g = i - NG
                for rc in range(0, BQ, CCH):
                    a11, a12, a21 = (pltpu.bitcast(ar[pl.ds(pl.multiple_of(A_TMP + t * BQ + rc + dyn, 16), CCH)], F32)
                                     for t in (g, slot1(g), i))
                    for j, op in enumerate(lhs_ops(lambda: a11, lambda: a12, lambda: a21, lambda: o[rc:rc + CCH])):
                        base = A_CT + (j * NP + p) * (HS // 2) + g * (BQ // 2)
                        arb[pl.ds(pl.multiple_of(base * 2 + rc, 16), CCH)] = op().astype(BF16)
            if CLAG and (hh == 1 and i >= NG or TOK0 and u % 2):
                tok[u + CLAG] = pltpu.bitcast(ar[pl.ds(pl.multiple_of(A_TMP + dyn2, 8), 8)], F32)
        while pieces:
            pieces.pop(0)()

    def x_combos(r0, n):
        rows = [pl.ds(pl.multiple_of(a * HS + r0, n), n) for a in range(2)]
        gl = [None, None]
        for b in range(NT // 2):
            blk = [[x_s[rows[a], (c * NT // 2 + b) * 128:(c * NT // 2 + b + 1) * 128].astype(F32) for c in range(2)]
                   for a in range(2)]
            ops = lhs_ops(lambda: blk[0][0], lambda: blk[0][1], lambda: blk[1][0], lambda: blk[1][1])
            for j, op in enumerate(ops):
                xab[j, b, rows[0]] = op().astype(BF16)
            for a in range(2):
                for c in range(2):
                    term = blk[a][c] * gw_s[c * NT // 2 + b, 0:n]
                    gl[a] = term if gl[a] is None else gl[a] + term
        for a in range(2):
            gate_s[rows[a]] = jnp.broadcast_to(jax.nn.sigmoid(jnp.sum(gl[a], axis=-1, keepdims=True)), (n, 128))

    def c_combos(r0, n):
        quarter = [c_s[pl.ds(pl.multiple_of(a * QS + r0, n), n)].astype(F32) for a in range(4)]
        for i in range(7):
            def outer(r2, kk):
                raw = lambda r, c: (lambda: quarter[2 * r + r2][:, (2 * c + kk) * 128:(2 * c + kk + 1) * 128])
                val = lhs_ops(raw(0, 0), raw(0, 1), raw(1, 0), raw(1, 1))[i]()
                return lambda: val
            for j, op in enumerate(lhs_ops(outer(0, 0), outer(0, 1), outer(1, 0), outer(1, 1))):
                cab[i, j, pl.ds(pl.multiple_of(r0, n), n)] = op().astype(BF16)

    dd_s[...] = ssmd[...].astype(F32)
    for b in range(NT):
        gw_s[b] = jnp.broadcast_to(gw[...].astype(F32)[b:b + 1], (16, 128))
    NC = QS // RB
    for cp in w0[:2] + ccopies(0):
        cp.wait()
    for cp in w0[2:] + [cp for r in range(1, NC) for cp in ccopies(r)]:
        cp.start()
    rows_of = lambda ref, r: unpack(ref.bitcast(U32)[pl.ds(pl.multiple_of(r // 2, RB // 2), RB // 2)])
    def pro_kv(r, carry):
        r0 = r * RB
        @pl.when(r > 0)
        def _():
            for cp in ccopies(r):
                cp.wait()
            for cp in xcopies(r - 1):
                cp.start()
        w = unpack(jnp.concatenate([wp.bitcast(U32)[n, 0:DC // 2] for n in range(4)], axis=1))
        for a in range(4):
            val = dot(rows_of(c_s, a * QS + r0), w)
            for n in range(4):
                blk = val[:, n * 128:(n + 1) * 128]
                qkv_store(0, 1 + n // 2, n % 2, a * QS + r0, blk.T if n // 2 else blk)
            for b in range(a * RB // 4, (a + 1) * RB // 4, 16):
                c_combos(r0 + b, 16)
        return carry
    def pro_q(r, carry):
        r0 = r * RB
        for cp in xcopies(r):
            cp.wait()
        w = unpack(jnp.concatenate([wp.bitcast(U32)[n] for n in range(2)], axis=1))
        for a in range(4):
            val = dot(rows_of(x_s, a * QS + r0), w) * qscale
            for hh in range(2):
                qkv_store(0, 0, hh, a * QS + r0, val[:, hh * 128:(hh + 1) * 128])
            for b in range(a % 2 * RB // 2, (a % 2 + 1) * RB // 2, 16):
                x_combos(a // 2 * QS + r0 + b, 16)
        return carry
    for n, w in enumerate(halves(wk_b[0]) + halves(wv_b[0])):
        wp[n, 0:DC] = w.astype(BF16)
    lax.fori_loop(0, NC, pro_kv, 0) if not NOPRO else None
    w0[2].wait()
    for cp in xcopies(NC - 1):
        cp.start()
    for cp in wcopies(1, 1):
        cp.start()
    for n, w in enumerate(halves(wq_b[0])):
        wp[n] = w.astype(BF16)
    lax.fori_loop(0, NC, pro_q, 0) if not NOPRO else None

    def pair_step(p, carry):
        slot = p % 2
        for cp in wcopies(p + 1, 1 - slot):
            cp.wait()
        @pl.when(p + 2 < NP)
        def _():
            for cp in wcopies(p + 2, slot):
                cp.start()
        @pl.when(p == NP - 2)
        def _():
            for cp in tcopies(0, 0):
                cp.start()
        kvp, qp = proj_pieces(1 - slot, lax.shift_right_logical(p, 8))
        attention(p, slot, [f for pair in (zip(kvp, qp) if PO == 0 else zip(qp, kvp)) for f in pair])
        return carry + 1
    last = lax.fori_loop(0, NP - 1, pair_step, 0) if not ONLY2 else None
    if ONLY1:
        return
    if not ONLY2:
        attention(last, (NP - 1) % 2, [])

    def tile_step(t, carry):
        slot = t % 2
        for cp in tcopies(t, slot):
            cp.wait()
        def prefetch():
            @pl.when(t + 1 < NT // 2)
            def _():
                for cp in tcopies(t + 1, 1 - slot):
                    cp.start()
            @pl.when(t >= 2)
            def _():
                for c in range(2):
                    ocopy(t - 2, slot, c).wait()
        if PF < 0:
            prefetch()

        KC = 4
        def oprod(i):
            acc = None
            for j0 in range(0, NP, KC):
                def wblk(r, c):
                    return lambda: jnp.concatenate(
                        [unpack(wo_b.bitcast(U32)[slot, c, 2 * j + r]) for j in range(j0, j0 + KC)], axis=0).astype(F32)
                w = rhs_ops(wblk(0, 0), wblk(0, 1), wblk(1, 0), wblk(1, 1))[i]().astype(BF16)
                a = jnp.concatenate([ar[pl.ds(A_CT + (i * NP + j) * (HS // 2), HS // 2)] for j in range(j0, j0 + KC)], axis=1)
                d = dot(unpack(a), w)
                acc = d if acc is None else acc + d
                yield acc
        def emit_o(r, c, val):
            rs = slice(r * HS, (r + 1) * HS)
            o_b[slot, c, rs] = (ga_s[c, rs] + (1.0 - gate_s[rs]) * val).astype(BF16)
        def opieces():
            m = {}
            def second_tile():
                emit_o(0, 1, m[2] + m[4])
                emit_o(1, 1, (m[0] + m[5]) + (m[2] - m[1]))
                ocopy(t, slot, 1).start()
            for i in PORD:
                for acc in oprod(i):
                    m[i] = acc
                    yield
                if EE and i == PORD[3 + EE]:
                    second_tile()
            yield
            if not EE:
                second_tile()
            emit_o(1, 0, m[1] + m[3])
            emit_o(0, 0, (m[0] + m[6]) + (m[3] - m[4]))
            ocopy(t, slot, 0).start()
        gen = opieces()
        def piece(n=1):
            for _ in range(n):
                next(gen)

        rows = lax.broadcasted_iota(jnp.int32, (8, 128), 0)
        sgn = (1 - 2 * (rows & 1)).astype(F32)
        Fm = f_ref[...]
        Gm = g_ref[...]
        for c, (n0, n1, n2, n3, fts) in zip(CO, PP):
            cs = slice(c * 128, (c + 1) * 128)
            piece(n0)
            if c == PF:
                prefetch()
            kk = unpack(ak_b.bitcast(U32)[slot, c]).astype(F32)
            sh = shk[2 * t + c].astype(F32)
            ksf = kk * sh[0:1, :]
            for j in range(1, KS):
                kr = pltpu.roll(kk, j, 0)
                kr = jnp.concatenate([jnp.where(rows >= j, kr[:8], 0.0), kr[8:]], axis=0)
                ksf = ksf + kr * sh[j:j + 1, :]
            kv = (ksf * unpack(av_b.bitcast(U32)[slot, c]).astype(F32)).astype(BF16)
            for j in range(0, NCH, 4):
                r = dot_nt(Fm, jnp.concatenate([hk_b[slot, cs, (j + a) * C:(j + a + 1) * C] for a in range(4)], axis=0))
                for a in range(4):
                    hf[j + a] = r[:, a * 128:(a + 1) * 128]
            piece(n1)
            for j in range(0, NCH, 4):
                r = dot(Fm, jnp.concatenate([kv[(j + a) * C:(j + a + 1) * C] for a in range(4)], axis=1))
                for a in range(4):
                    uf[j + a] = r[:, a * 128:(a + 1) * 128]
            ga_s[c] = kv.astype(F32) * dd_s[pl.ds(2 * t + c, 1)]
            piece(n2)
            for ft in range(C // 8):
                re = slice(ft * 8, ft * 8 + 8)
                im = slice(C + ft * 8, C + ft * 8 + 8)
                hc = [hf[0, re]] + [hf[m, re] - sgn * hf[m - 1, im] for m in range(1, NCH)]
                hd = [hf[0, im]] + [hf[m, im] + sgn * hf[m - 1, re] for m in range(1, NCH)]
                ua = [uf[j, re] for j in range(NCH)]
                ub = [uf[j, im] for j in range(NCH)]
                def toep(u, h):
                    out = []
                    for i in range(NCH):
                        a = u[0] * h[i]
                        for j in range(1, i + 1):
                            a = a + u[j] * h[i - j]
                        out.append(a)
                    return out
                k1 = toep([a + b for a, b in zip(ua, ub)], hc)
                k2 = toep(ua, [d - c_ for c_, d in zip(hc, hd)])
                k3 = toep(ub, [d + c_ for c_, d in zip(hc, hd)])
                for i in range(NCH):
                    zf[i, re] = k1[i] - k3[i]
                    zf[i, im] = k1[i] + k2[i]
                if ft in fts:
                    piece()
            xcs = pl.ds(pl.multiple_of((2 * t + c) * 128, 128), 128)
            for j in range(0, NCH, 4):
                r = dot(Gm, jnp.concatenate([zf[j + a] for a in range(4)], axis=1).astype(BF16))
                for a in range(4):
                    ts = slice((j + a) * C, (j + a + 1) * C)
                    y = r[:, a * 128:(a + 1) * 128] + ga_s[c, ts]
                    ga_s[c, ts] = gate_s[ts] * (x_s[ts, xcs].astype(F32) * y)
                if j == 4:
                    piece(n3)
        for _ in gen:
            pass
        return carry
    lax.fori_loop(0, NT // 2, tile_step, 0)
    for t in range(NT // 2 - 2, NT // 2):
        for c in range(2):
            ocopy(t, t % 2, c).wait()

@jax.jit
def pallas_gated_mix__ssm_conv_h3__compressed_kv_cla__prompt_kernel(
        A_q, A_k, A_v, A_shift_k, A_ssm_k, A_ssm_D, B_x, B_c_kv, B_w_q, B_w_uk, B_w_uv, B_w_o, gate_w):
    any_ = pl.BlockSpec(memory_space=pl.ANY)
    vm = pl.BlockSpec(memory_space=pltpu.VMEM)
    out = pl.pallas_call(
        kernel,
        in_specs=[vm] * 5 + [any_] * 9,
        out_specs=any_,
        out_shape=jax.ShapeDtypeStruct((1, S, DM), BF16),
        scratch_shapes=[
            pltpu.VMEM((S, DM), BF16), pltpu.VMEM((S, DC), BF16),
            pltpu.VMEM((7, DM // 256, HS, 128), BF16), pltpu.VMEM((7, 7, QS, 128), BF16),
            pltpu.VMEM((2, DM, 128), U32), pltpu.VMEM((2, DC, 128), U32), pltpu.VMEM((2, DC, 128), U32),
            pltpu.VMEM((3, S, 128), BF16), pltpu.VMEM((2, 3, S, 128), BF16), pltpu.VMEM((2 * A_END, 128), BF16),
            pltpu.VMEM((S, 128), F32), pltpu.VMEM((S, 128), F32), pltpu.VMEM((4, 2, HS, 128), F32), pltpu.VMEM((4, QS, 128), F32), pltpu.VMEM((4, HS, 128), F32),
            pltpu.VMEM((S, 128), F32),
            pltpu.VMEM((2, 2, S, 128), BF16), pltpu.VMEM((2, 2, S, 128), BF16), pltpu.VMEM((2, 256, S), BF16),
            pltpu.VMEM((2, 2, H, HD, 128), BF16), pltpu.VMEM((2, 2, S, 128), BF16),
            pltpu.VMEM((NCH, 2 * C, 128), F32), pltpu.VMEM((NCH, 2 * C, 128), F32), pltpu.VMEM((NCH, 2 * C, 128), F32),
            pltpu.VMEM((2, S, 128), F32), pltpu.VMEM((NT, 128), F32), pltpu.VMEM((NT, 16, 128), F32), pltpu.VMEM((4, DM, 128), BF16),
            pltpu.SemaphoreType.DMA((2, 4, 4)), pltpu.SemaphoreType.DMA((3, 2)), pltpu.SemaphoreType.DMA((7, 2)),
            pltpu.SemaphoreType.DMA((2, 2)),
        ],
        compiler_params=pltpu.CompilerParams(vmem_limit_bytes=120 * 1024 * 1024),
    )(gate_w.reshape(NT, 128), A_shift_k.T.reshape(KS, NT, 128).transpose(1, 0, 2), A_ssm_D.reshape(NT, 128), _F, _G,
      A_q, A_k, A_v, A_ssm_k, B_c_kv, B_w_q, B_w_uk, B_w_uv, B_w_o)
    return out
```

```python
import numpy as np
import jax
import jax.numpy as jnp
from jax import lax
import jax.experimental.pallas as pl
import jax.experimental.pallas.tpu as pltpu
import ml_dtypes

S, DM, H, HD, DC, KS = 2048, 1024, 32, 128, 512, 4
C = 128
NCH = S // C
NP = H // 2
NT = DM // 128
HS = S // 2
QS = S // 4
F32, BF16, U32 = jnp.float32, jnp.bfloat16, jnp.uint32
NTD = (((1,), (1,)), ((), ()))

BQ = 128
NG = HS // BQ
A_TMP = 0
A_CT = A_TMP + S + 4 * BQ
A_END = A_CT + 7 * NP * (HS // 2)
ONLY1 = 0
ONLY2 = 0
OR = 128
GT = 1
LAG = 0
REV = 3
CLAG = 2
TOK0 = 0
SPL = 0
CH = 0
PP = ((1,1,2,3,(1,3,5,7,9,11,13,15)),(2,1,2,1,(0,2,3,4,5,6,8)))
NOPRO = 0
ONLYL = 0
U1 = 1
LK = (2, 3, 2, 1)
RC = 64
PF = -1
CO = (1, 0)
EE = 1
AQ = 0
AO = 0
AI = 0
PB = (2,10,11,12,15,16,26)
PO = 0
UO = 1
PQ = ((0,), (1,), (2,), (3,))
CCH = 32
SL0 = (0,1,2,3,4,6,8,9,11,13)
SL1 = (10,12,14,16)

def _dft_consts():
    N = 2 * C
    f = np.arange(C, dtype=np.float64)[:, None] + 0.5
    t = np.arange(C, dtype=np.float64)[None, :]
    ang = 2 * np.pi * f * t / N
    Fm = np.concatenate([np.cos(ang), -np.sin(ang)], 0)
    Gm = np.concatenate([np.cos(ang).T, -np.sin(ang).T], 1) * (2.0 / N)
    return Fm.astype(ml_dtypes.bfloat16), Gm.astype(ml_dtypes.bfloat16)
_F, _G = _dft_consts()

def dot(a, b):
    return jnp.dot(a, b, preferred_element_type=F32)

def dot_nt(a, b):
    return lax.dot_general(a, b, NTD, preferred_element_type=F32)

def pack(x):
    return pltpu.bitcast(x.astype(BF16), U32)

def unpack(w):
    return pltpu.bitcast(w, BF16)

def halves(w):
    return pltpu.bitcast(w << 16, F32), pltpu.bitcast(w & jnp.uint32(0xFFFF0000), F32)

def lhs_ops(a11, a12, a21, a22):
    return [lambda: a11() + a22(), lambda: a21() + a22(), a11, a22,
            lambda: a11() + a12(), lambda: a21() - a11(), lambda: a12() - a22()]

def rhs_ops(b11, b12, b21, b22):
    return [lambda: b11() + b22(), b11, lambda: b12() - b22(), lambda: b21() - b11(),
            b22, lambda: b11() + b12(), lambda: b21() + b22()]

PORD = (2, 4, 1, 0, 5, 3, 6)
SKIP = (4, 10, 16)

def consume(i, v, emit, m, dyn, acc=0):
    if i == 2:
        m[0 + dyn] = v
    elif i == 4:
        emit(0, 1, m[0] + v)
        m[1 + dyn] = v
    elif i == 1:
        m[2 + dyn] = v
        if acc & 1:
            m[0 + dyn] = m[0] - v
    elif i == 0:
        m[3 + dyn] = v
        if acc & 2:
            m[1 + dyn] = v - m[1]
    elif i == 5:
        emit(1, 1, (m[0] if acc & 1 else m[0] - m[2]) + (m[3] + v))
    elif i == 3:
        emit(1, 0, m[2] + v)
        m[0 + dyn] = v
    else:
        emit(0, 0, (m[1] if acc & 2 else m[3] - m[1]) + (m[0] + v))

def kernel(gw, shk, ssmd, f_ref, g_ref, aq_hbm, ak_hbm, av_hbm, ssmk_hbm, c_hbm, wq_hbm, wk_hbm, wv_hbm, wo_hbm,
           o_hbm,
           x_s, c_s, xab, cab, wq_b, wk_b, wv_b, h0b, h1b, arb, s0, s1, mkv, mi, mq, gate_s, ak_b, av_b, hk_b, wo_b, o_b, uf, hf, zf, ga_s, dd_s, gw_s, wp,
           sem_x, sem_w, sem_t, sem_o):

    def wcopies(p, slot):
        return [pltpu.make_async_copy(src.bitcast(U32).at[:, p, :], dst.at[slot], sem_w.at[i, slot])
                for i, (src, dst) in enumerate(((wk_hbm, wk_b), (wv_hbm, wv_b), (wq_hbm, wq_b)))]

    def tcopies(t, slot):
        cps = [pltpu.make_async_copy(ssmk_hbm.at[pl.ds(pl.multiple_of(t * 256, 256), 256), :], hk_b.at[slot], sem_t.at[0, slot])]
        for c in range(2):
            cs = pl.ds(pl.multiple_of((2 * t + c) * 128, 128), 128)
            cps += [pltpu.make_async_copy(ak_hbm.at[0, :, cs], ak_b.at[slot, c], sem_t.at[1 + c, slot]),
                    pltpu.make_async_copy(av_hbm.at[0, :, cs], av_b.at[slot, c], sem_t.at[3 + c, slot]),
                    pltpu.make_async_copy(wo_hbm.at[:, :, cs], wo_b.at[slot, c], sem_t.at[5 + c, slot])]
        return cps

    def ocopy(t, slot, c):
        cs = pl.ds(pl.multiple_of((2 * t + c) * 128, 128), 128)
        return pltpu.make_async_copy(o_b.at[slot, c], o_hbm.at[0, :, cs], sem_o.at[c, slot])

    RB = 128
    def rcopies(src, dst, which, r):
        rows = lambda a: pl.ds(pl.multiple_of(a * QS + r * RB, RB), RB)
        return [pltpu.make_async_copy(src.at[0, rows(a)], dst.at[rows(a)], sem_x.at[which, a, r]) for a in range(4)]
    ccopies = lambda r: rcopies(c_hbm, c_s, 0, r)
    xcopies = lambda r: rcopies(aq_hbm, x_s, 1, r)
    w0 = wcopies(0, 0)
    for cp in w0[:2] + ccopies(0):
        cp.start()

    qscale = float((HD ** -0.5) * np.log2(np.e))

    ar, xa, ca = arb.bitcast(U32), xab.bitcast(U32), cab.bitcast(U32)
    h0, h1 = h0b.bitcast(U32), h1b.bitcast(U32)

    def qkv_load(slot, which, hh, r0, n):
        rs = slice(r0 // 2, (r0 + n) // 2)
        return h0[which, rs] if hh == 0 else h1[slot, which, rs]

    def qkv_store(slot, which, hh, r0, val):
        rs = pl.ds(pl.multiple_of(r0, 32), val.shape[0])
        if hh == 0:
            h0b[which, rs] = val.astype(BF16)
        else:
            h1b[slot, which, rs] = val.astype(BF16)

    def proj_pieces(slot, dyn):
        def q_piece(i):
            def f():
                blk = lambda r, c: (lambda: halves(wq_b[slot, r * (DM // 2):(r + 1) * (DM // 2)])[c])
                w = rhs_ops(blk(0, 0), blk(0, 1), blk(1, 0), blk(1, 1))[i]().astype(BF16)
                a = jnp.concatenate([xa[i, b] for b in range(DM // 256)], axis=1)
                emit = lambda r, c, val: qkv_store(slot, 0, c, r * HS, val * qscale)
                consume(i, dot(unpack(a), w), emit, mq, dyn, AQ)
            return f
        def kv_piece(i):
            def f():
                def outer(kk, nn):
                    raw = lambda r, c: (lambda: halves((wk_b, wv_b)[nn][slot, (2 * r + kk) * 128:(2 * r + kk + 1) * 128])[c])
                    return rhs_ops(raw(0, 0), raw(0, 1), raw(1, 0), raw(1, 1))[i]
                rops = rhs_ops(outer(0, 0), outer(0, 1), outer(1, 0), outer(1, 1))
                def inner_emit(r2, c2, v):
                    def emit(r, c, val):
                        for t in range(0, QS, 128):
                            blk = val[t:t + 128]
                            qkv_store(slot, 1 + c2, c, r * HS + r2 * QS + t, blk.T if c2 else blk)
                    consume(i, v, emit, mkv.at[:, c2, r2 * QS:(r2 + 1) * QS], dyn, AO)
                if RC == 0:
                    for j in PORD:
                        w = rops[j]().astype(BF16)
                        v = jnp.concatenate([dot(unpack(ca[i, j, a * QS // 8:(a + 1) * QS // 8]), w) for a in range(4)], axis=0)
                        consume(j, v, inner_emit, mi, dyn, AI)
                    return
                for j in PORD:
                    wp[dyn, j * 128:(j + 1) * 128] = rops[j]().astype(BF16)
                for t0 in range(0, QS, 128):
                    blocks = {}
                    for a in range(t0, t0 + 128, RC):
                        v = {j: dot(unpack(ca[i, j, a // 2:(a + RC) // 2]), unpack(wp.bitcast(U32)[0, j * 64:(j + 1) * 64]))
                             for j in PORD}
                        for key, val in (((0, 1), v[2] + v[4]), ((1, 1), (v[2] - v[1]) + (v[0] + v[5])),
                                         ((1, 0), v[1] + v[3]), ((0, 0), (v[0] - v[4]) + (v[3] + v[6]))):
                            r2, c2 = key
                            def emit(r, c, val, r2=r2, c2=c2, a=a):
                                if c2 == 0:
                                    qkv_store(slot, 1, c, r * HS + r2 * QS + a, val)
                                else:
                                    blocks.setdefault((r, c, r2), []).append(val)
                            consume(i, val, emit, mkv.at[:, c2, r2 * QS + a:r2 * QS + a + RC], dyn, AO)
                    for (r, c, r2), vals in blocks.items():
                        qkv_store(slot, 2, c, r * HS + r2 * QS + t0, jnp.concatenate(vals, axis=0).T)
            return f
        return [kv_piece(i) for i in PORD], [q_piece(i) for i in PORD]

    def scores(slot, hh, i, buf, dyn):
        L = (i + 1) * BQ
        q = unpack(qkv_load(slot, 0, hh, i * BQ, BQ))
        m = None
        n = L // 4
        for a in range(4):
            st = dot_nt(unpack(qkv_load(slot, 1, hh, a * n, n)), q)
            d0 = max(L - BQ - a * n, 0)
            if d0 < n:
                row = lax.broadcasted_iota(jnp.int32, (n - d0, BQ), 0) + (a * n + d0 - (L - BQ))
                col = lax.broadcasted_iota(jnp.int32, (n - d0, BQ), 1)
                dg = jnp.where(row <= col, st[d0:], -1e9)
                st = dg if d0 == 0 else jnp.concatenate([st[:d0], dg], axis=0)
            (s0, s1)[buf][pl.ds(pl.multiple_of(a * n + dyn, 32), n)] = st
            ma = jnp.max(st.reshape(n // 8, 8, BQ), axis=0)
            m = ma if m is None else jnp.maximum(m, ma)
        return jnp.broadcast_to(jnp.max(m, axis=0, keepdims=True), (8, BQ))

    def weighted(slot, hh, i, buf, m, never, dyn2):
        l = ot = None
        for t0 in range(0, i + 1, GT):
            nt = min(GT, i + 1 - t0)
            pj = jnp.exp2((s0, s1)[buf][t0 * BQ:(t0 + nt) * BQ] - jnp.tile(m, (nt * BQ // 8, 1)))
            lj = jnp.sum(pj.reshape(nt * BQ // 8, 8, BQ), axis=0)
            if LAG and l is not None:
                pj = jnp.concatenate([jnp.where(never, l, pj[:8]), pj[8:]], axis=0)
            l = lj if l is None else l + lj
            pt = pj.astype(BF16)
            ns = 1 if nt == 4 else 2 if nt == 2 else 4
            if SPL and t0 < (i + 1) // SPL * SPL:
                ns = 4 // SPL
            parts = []
            for a in range(ns):
                vt = jnp.concatenate([qkv_load(slot, 2, hh, t * 128 + a * HD // ns, HD // ns)
                                      for t in range(t0, t0 + nt)], axis=1)
                parts.append(dot(unpack(vt), pt))
            d = jnp.concatenate(parts, axis=0)
            ot = d if ot is None else ot + d
        l = jnp.sum(l, axis=0, keepdims=True)
        r = pl.reciprocal(l, approx=True)
        r = r * (2.0 - l * r)
        return (ot * r).T

    def attention(p, slot, pieces, UO=UO, REV=REV, CLAG=CLAG, U1=0):
        pieces = list(pieces)
        dyn = lax.shift_right_logical(p, 8)
        never = jnp.broadcast_to(p, (8, BQ)) < 0
        dyn2 = lax.shift_right_logical(p, 9)
        tmp = lambda i: pl.ds(pl.multiple_of(A_TMP + i * BQ + dyn, 64), BQ)
        gs = lambda hh: range(NG) if not (REV >> hh) & 1 else reversed(range(NG))
        units = [(hh, g + a * NG) for hh in range(2) for g in gs(hh) for a in range(2)]
        if UO == 1:
            units[:2 * NG] = [(0, i) for g in range(NG) for i in (g, 2 * NG - 1 - g)]
        elif UO == 2:
            units[:2 * NG] = [(0, i) for i in range(2 * NG)]
        elif UO == 3:
            units[:2 * NG] = [(0, i) for g in range(NG) for i in (2 * NG - 1 - g, g)]
        if U1 == 1:
            units[2 * NG:] = [(1, g + a * NG) for g in gs(1) for a in (1, 0)]
        slot1 = lambda i: 2 * NG + (i % 2) * 2 + i // NG

        nxt = scores(slot, *units[0], 0, dyn)
        tok = {}
        for u, (hh, i) in enumerate(units):
            cur = nxt
            here = pieces and (u in SL0 or u - 2 * NG in SL1)
            if here and u in PB:
                pieces.pop(0)()
            if u + 1 < len(units):
                nxt = scores(slot, *units[u + 1], (u + 1) % 2, dyn)
            if here and u not in PB:
                pieces.pop(0)()
            if u in tok:
                cur = jnp.where(never, tok[u], cur)
            o = weighted(slot, hh, i, u % 2, cur, never, dyn2)
            if hh == 0 or u % 2 == 0:
                ar[tmp(i if hh == 0 else slot1(i))] = pltpu.bitcast(o, U32)
            else:
                g = i % NG
                for rc in range(0, BQ, CCH):
                    a11, a12, a21 = (pltpu.bitcast(ar[pl.ds(pl.multiple_of(A_TMP + t * BQ + rc + dyn, 16), CCH)], F32)
                                     for t in (g, slot1(units[u - 1][1]), g + NG))
                    a12, a22 = (a12, o[rc:rc + CCH]) if i >= NG else (o[rc:rc + CCH], a12)
                    for j, op in enumerate(lhs_ops(lambda: a11, lambda: a12, lambda: a21, lambda: a22)):
                        base = A_CT + (j * NP + p) * (HS // 2) + g * (BQ // 2)
                        arb[pl.ds(pl.multiple_of(base * 2 + rc, 16), CCH)] = op().astype(BF16)
            if CLAG and hh == 1 and u % 2:
                tok[u + CLAG] = pltpu.bitcast(ar[pl.ds(pl.multiple_of(A_TMP + dyn2, 8), 8)], F32)
        while pieces:
            pieces.pop(0)()

    def x_combos(r0, n):
        rows = [pl.ds(pl.multiple_of(a * HS + r0, n), n) for a in range(2)]
        gl = [None, None]
        for b in range(NT // 2):
            blk = [[x_s[rows[a], (c * NT // 2 + b) * 128:(c * NT // 2 + b + 1) * 128].astype(F32) for c in range(2)]
                   for a in range(2)]
            ops = lhs_ops(lambda: blk[0][0], lambda: blk[0][1], lambda: blk[1][0], lambda: blk[1][1])
            for j, op in enumerate(ops):
                xab[j, b, rows[0]] = op().astype(BF16)
            for a in range(2):
                for c in range(2):
                    term = blk[a][c] * gw_s[c * NT // 2 + b, 0:n]
                    gl[a] = term if gl[a] is None else gl[a] + term
        for a in range(2):
            gate_s[rows[a]] = jnp.broadcast_to(jax.nn.sigmoid(jnp.sum(gl[a], axis=-1, keepdims=True)), (n, 128))

    def c_combos(r0, n):
        quarter = [c_s[pl.ds(pl.multiple_of(a * QS + r0, n), n)].astype(F32) for a in range(4)]
        for i in range(7):
            def outer(r2, kk):
                raw = lambda r, c: (lambda: quarter[2 * r + r2][:, (2 * c + kk) * 128:(2 * c + kk + 1) * 128])
                val = lhs_ops(raw(0, 0), raw(0, 1), raw(1, 0), raw(1, 1))[i]()
                return lambda: val
            for j, op in enumerate(lhs_ops(outer(0, 0), outer(0, 1), outer(1, 0), outer(1, 1))):
                cab[i, j, pl.ds(pl.multiple_of(r0, n), n)] = op().astype(BF16)

    dd_s[...] = ssmd[...].astype(F32)
    for b in range(NT):
        gw_s[b] = jnp.broadcast_to(gw[...].astype(F32)[b:b + 1], (16, 128))
    NC = QS // RB
    for cp in w0[:2] + ccopies(0):
        cp.wait()
    for cp in w0[2:] + [cp for r in range(1, NC) for cp in ccopies(r)]:
        cp.start()
    rows_of = lambda ref, r: unpack(ref.bitcast(U32)[pl.ds(pl.multiple_of(r // 2, RB // 2), RB // 2)])
    def pro_kv(r, carry):
        r0 = r * RB
        @pl.when(r > 0)
        def _():
            for cp in ccopies(r):
                cp.wait()
            for cp in xcopies(r - 1):
                cp.start()
        w = unpack(jnp.concatenate([wp.bitcast(U32)[n, 0:DC // 2] for n in range(4)], axis=1))
        for a in range(4):
            val = dot(rows_of(c_s, a * QS + r0), w)
            for n in range(4):
                blk = val[:, n * 128:(n + 1) * 128]
                qkv_store(0, 1 + n // 2, n % 2, a * QS + r0, blk.T if n // 2 else blk)
            for b in range(a * RB // 4, (a + 1) * RB // 4, 16):
                c_combos(r0 + b, 16)
        return carry
    def pro_q(r, carry):
        r0 = r * RB
        for cp in xcopies(r):
            cp.wait()
        w = unpack(jnp.concatenate([wp.bitcast(U32)[n] for n in range(2)], axis=1))
        for a in range(4):
            val = dot(rows_of(x_s, a * QS + r0), w) * qscale
            for hh in range(2):
                qkv_store(0, 0, hh, a * QS + r0, val[:, hh * 128:(hh + 1) * 128])
            for b in range(a % 2 * RB // 2, (a % 2 + 1) * RB // 2, 16):
                x_combos(a // 2 * QS + r0 + b, 16)
        return carry
    for n, w in enumerate(halves(wk_b[0]) + halves(wv_b[0])):
        wp[n, 0:DC] = w.astype(BF16)
    lax.fori_loop(0, NC, pro_kv, 0) if not NOPRO else None
    w0[2].wait()
    for cp in xcopies(NC - 1):
        cp.start()
    for cp in wcopies(1, 1):
        cp.start()
    for n, w in enumerate(halves(wq_b[0])):
        wp[n] = w.astype(BF16)
    lax.fori_loop(0, NC, pro_q, 0) if not NOPRO else None

    def pair_step(p, carry):
        slot = p % 2
        for cp in wcopies(p + 1, 1 - slot):
            cp.wait()
        @pl.when(p + 2 < NP)
        def _():
            for cp in wcopies(p + 2, slot):
                cp.start()
        @pl.when(p == NP - 2)
        def _():
            for cp in tcopies(0, 0):
                cp.start()
        kvp, qp = proj_pieces(1 - slot, lax.shift_right_logical(p, 8))
        attention(p, slot, [f for pair in (zip(kvp, qp) if PO == 0 else zip(qp, kvp)) for f in pair], U1=U1)
        return carry + 1
    last = lax.fori_loop(0, NP - 1, pair_step if not ONLYL else (lambda p, c: c + pl.program_id(0) if 0 else c + 1), 0) if not ONLY2 else None
    if ONLY1:
        return
    if not ONLY2:
        attention(last, (NP - 1) % 2, [], *LK)

    if ONLYL:
        return
    def tile_step(t, carry):
        slot = t % 2
        for cp in tcopies(t, slot):
            cp.wait()
        def prefetch():
            @pl.when(t + 1 < NT // 2)
            def _():
                for cp in tcopies(t + 1, 1 - slot):
                    cp.start()
            @pl.when(t >= 2)
            def _():
                for c in range(2):
                    ocopy(t - 2, slot, c).wait()
        if PF < 0:
            prefetch()

        KC = 4
        def oprod(i):
            acc = None
            for j0 in range(0, NP, KC):
                def wblk(r, c):
                    return lambda: jnp.concatenate(
                        [unpack(wo_b.bitcast(U32)[slot, c, 2 * j + r]) for j in range(j0, j0 + KC)], axis=0).astype(F32)
                w = rhs_ops(wblk(0, 0), wblk(0, 1), wblk(1, 0), wblk(1, 1))[i]().astype(BF16)
                a = jnp.concatenate([ar[pl.ds(A_CT + (i * NP + j) * (HS // 2), HS // 2)] for j in range(j0, j0 + KC)], axis=1)
                d = dot(unpack(a), w)
                acc = d if acc is None else acc + d
                yield acc
        def emit_o(r, c, val):
            rs = slice(r * HS, (r + 1) * HS)
            o_b[slot, c, rs] = (ga_s[c, rs] + (1.0 - gate_s[rs]) * val).astype(BF16)
        def opieces():
            m = {}
            def second_tile():
                emit_o(0, 1, m[2] + m[4])
                emit_o(1, 1, (m[0] + m[5]) + (m[2] - m[1]))
                ocopy(t, slot, 1).start()
            for i in PORD:
                for acc in oprod(i):
                    m[i] = acc
                    yield
                if EE and i == PORD[3 + EE]:
                    second_tile()
            yield
            if not EE:
                second_tile()
            emit_o(1, 0, m[1] + m[3])
            emit_o(0, 0, (m[0] + m[6]) + (m[3] - m[4]))
            ocopy(t, slot, 0).start()
        gen = opieces()
        def piece(n=1):
            for _ in range(n):
                next(gen)

        rows = lax.broadcasted_iota(jnp.int32, (8, 128), 0)
        sgn = (1 - 2 * (rows & 1)).astype(F32)
        Fm = f_ref[...]
        Gm = g_ref[...]
        for c, (n0, n1, n2, n3, fts) in zip(CO, PP):
            cs = slice(c * 128, (c + 1) * 128)
            piece(n0)
            if c == PF:
                prefetch()
            kk = unpack(ak_b.bitcast(U32)[slot, c]).astype(F32)
            sh = shk[2 * t + c].astype(F32)
            ksf = kk * sh[0:1, :]
            for j in range(1, KS):
                kr = pltpu.roll(kk, j, 0)
                kr = jnp.concatenate([jnp.where(rows >= j, kr[:8], 0.0), kr[8:]], axis=0)
                ksf = ksf + kr * sh[j:j + 1, :]
            kv = (ksf * unpack(av_b.bitcast(U32)[slot, c]).astype(F32)).astype(BF16)
            for j in range(0, NCH, 4):
                r = dot_nt(Fm, jnp.concatenate([hk_b[slot, cs, (j + a) * C:(j + a + 1) * C] for a in range(4)], axis=0))
                for a in range(4):
                    hf[j + a] = r[:, a * 128:(a + 1) * 128]
            piece(n1)
            for j in range(0, NCH, 4):
                r = dot(Fm, jnp.concatenate([kv[(j + a) * C:(j + a + 1) * C] for a in range(4)], axis=1))
                for a in range(4):
                    uf[j + a] = r[:, a * 128:(a + 1) * 128]
            ga_s[c] = kv.astype(F32) * dd_s[pl.ds(2 * t + c, 1)]
            piece(n2)
            for ft in range(C // 8):
                re = slice(ft * 8, ft * 8 + 8)
                im = slice(C + ft * 8, C + ft * 8 + 8)
                hc = [hf[0, re]] + [hf[m, re] - sgn * hf[m - 1, im] for m in range(1, NCH)]
                hd = [hf[0, im]] + [hf[m, im] + sgn * hf[m - 1, re] for m in range(1, NCH)]
                ua = [uf[j, re] for j in range(NCH)]
                ub = [uf[j, im] for j in range(NCH)]
                def toep(u, h):
                    out = []
                    for i in range(NCH):
                        a = u[0] * h[i]
                        for j in range(1, i + 1):
                            a = a + u[j] * h[i - j]
                        out.append(a)
                    return out
                k1 = toep([a + b for a, b in zip(ua, ub)], hc)
                k2 = toep(ua, [d - c_ for c_, d in zip(hc, hd)])
                k3 = toep(ub, [d + c_ for c_, d in zip(hc, hd)])
                for i in range(NCH):
                    zf[i, re] = k1[i] - k3[i]
                    zf[i, im] = k1[i] + k2[i]
                if ft in fts:
                    piece()
            xcs = pl.ds(pl.multiple_of((2 * t + c) * 128, 128), 128)
            for j in range(0, NCH, 4):
                r = dot(Gm, jnp.concatenate([zf[j + a] for a in range(4)], axis=1).astype(BF16))
                for a in range(4):
                    ts = slice((j + a) * C, (j + a + 1) * C)
                    y = r[:, a * 128:(a + 1) * 128] + ga_s[c, ts]
                    ga_s[c, ts] = gate_s[ts] * (x_s[ts, xcs].astype(F32) * y)
                if j == 4:
                    piece(n3)
        for _ in gen:
            pass
        return carry
    lax.fori_loop(0, NT // 2, tile_step, 0)
    for t in range(NT // 2 - 2, NT // 2):
        for c in range(2):
            ocopy(t, t % 2, c).wait()

@jax.jit
def pallas_gated_mix__ssm_conv_h3__compressed_kv_cla__prompt_kernel(
        A_q, A_k, A_v, A_shift_k, A_ssm_k, A_ssm_D, B_x, B_c_kv, B_w_q, B_w_uk, B_w_uv, B_w_o, gate_w):
    any_ = pl.BlockSpec(memory_space=pl.ANY)
    vm = pl.BlockSpec(memory_space=pltpu.VMEM)
    out = pl.pallas_call(
        kernel,
        in_specs=[vm] * 5 + [any_] * 9,
        out_specs=any_,
        out_shape=jax.ShapeDtypeStruct((1, S, DM), BF16),
        scratch_shapes=[
            pltpu.VMEM((S, DM), BF16), pltpu.VMEM((S, DC), BF16),
            pltpu.VMEM((7, DM // 256, HS, 128), BF16), pltpu.VMEM((7, 7, QS, 128), BF16),
            pltpu.VMEM((2, DM, 128), U32), pltpu.VMEM((2, DC, 128), U32), pltpu.VMEM((2, DC, 128), U32),
            pltpu.VMEM((3, S, 128), BF16), pltpu.VMEM((2, 3, S, 128), BF16), pltpu.VMEM((2 * A_END, 128), BF16),
            pltpu.VMEM((S, 128), F32), pltpu.VMEM((S, 128), F32), pltpu.VMEM((4, 2, HS, 128), F32), pltpu.VMEM((4, QS, 128), F32), pltpu.VMEM((4, HS, 128), F32),
            pltpu.VMEM((S, 128), F32),
            pltpu.VMEM((2, 2, S, 128), BF16), pltpu.VMEM((2, 2, S, 128), BF16), pltpu.VMEM((2, 256, S), BF16),
            pltpu.VMEM((2, 2, H, HD, 128), BF16), pltpu.VMEM((2, 2, S, 128), BF16),
            pltpu.VMEM((NCH, 2 * C, 128), F32), pltpu.VMEM((NCH, 2 * C, 128), F32), pltpu.VMEM((NCH, 2 * C, 128), F32),
            pltpu.VMEM((2, S, 128), F32), pltpu.VMEM((NT, 128), F32), pltpu.VMEM((NT, 16, 128), F32), pltpu.VMEM((4, DM, 128), BF16),
            pltpu.SemaphoreType.DMA((2, 4, 4)), pltpu.SemaphoreType.DMA((3, 2)), pltpu.SemaphoreType.DMA((7, 2)),
            pltpu.SemaphoreType.DMA((2, 2)),
        ],
        compiler_params=pltpu.CompilerParams(vmem_limit_bytes=120 * 1024 * 1024),
    )(gate_w.reshape(NT, 128), A_shift_k.T.reshape(KS, NT, 128).transpose(1, 0, 2), A_ssm_D.reshape(NT, 128), _F, _G,
      A_q, A_k, A_v, A_ssm_k, B_c_kv, B_w_q, B_w_uk, B_w_uv, B_w_o)
    return out
```

```python
import numpy as np
import jax
import jax.numpy as jnp
from jax import lax
import jax.experimental.pallas as pl
import jax.experimental.pallas.tpu as pltpu
import ml_dtypes

S, DM, H, HD, DC, KS = 2048, 1024, 32, 128, 512, 4
C = 128
NCH = S // C
NP = H // 2
NT = DM // 128
HS = S // 2
QS = S // 4
F32, BF16, U32 = jnp.float32, jnp.bfloat16, jnp.uint32
NTD = (((1,), (1,)), ((), ()))

BQ = 128
NG = HS // BQ
A_TMP = 0
A_CT = A_TMP + S + 4 * BQ
A_END = A_CT + 7 * NP * (HS // 2)
ONLY1 = 0
ONLY2 = 0
OR = 128
GT = 1
LAG = 0
REV = 3
CLAG = 2
TOK0 = 0
SPL = 0
CH = 0
PP = ((1,1,2,3,(1,3,5,7,9,11,13,15)),(2,2,2,1,(0,2,3,4,5,8)))
NOPRO = 0
KVB = 2
ONLYL = 0
U1 = 1
LK = (2, 3, 2, 1)
RC = 64
PF = -1
CO = (1, 0)
EE = 1
AQ = 0
AO = 0
AI = 0
PB = (2,10,11,12,15,16,26)
PO = 0
UO = 1
PQ = ((0,), (1,), (2,), (3,))
CCH = 32
SL0 = (0,1,2,3,4,6,8,9,11,13)
SL1 = (10,12,14,16)

def _dft_consts():
    N = 2 * C
    f = np.concatenate([np.arange(0, C, 2), np.arange(1, C, 2)])[:, None] + 0.5
    t = np.arange(C, dtype=np.float64)[None, :]
    ang = 2 * np.pi * f * t / N
    Fm = np.concatenate([np.cos(ang), -np.sin(ang)], 0)
    Gm = np.concatenate([np.cos(ang).T, -np.sin(ang).T], 1) * (2.0 / N)
    return Fm.astype(ml_dtypes.bfloat16), Gm.astype(ml_dtypes.bfloat16)
_F, _G = _dft_consts()

def dot(a, b):
    return jnp.dot(a, b, preferred_element_type=F32)

def dot_nt(a, b):
    return lax.dot_general(a, b, NTD, preferred_element_type=F32)

def pack(x):
    return pltpu.bitcast(x.astype(BF16), U32)

def unpack(w):
    return pltpu.bitcast(w, BF16)

def halves(w):
    return pltpu.bitcast(w << 16, F32), pltpu.bitcast(w & jnp.uint32(0xFFFF0000), F32)

def lhs_ops(a11, a12, a21, a22):
    return [lambda: a11() + a22(), lambda: a21() + a22(), a11, a22,
            lambda: a11() + a12(), lambda: a21() - a11(), lambda: a12() - a22()]

def rhs_ops(b11, b12, b21, b22):
    return [lambda: b11() + b22(), b11, lambda: b12() - b22(), lambda: b21() - b11(),
            b22, lambda: b11() + b12(), lambda: b21() + b22()]

PORD = (2, 4, 1, 0, 5, 3, 6)
SKIP = (4, 10, 16)

def consume(i, v, emit, m, dyn, acc=0):
    if i == 2:
        m[0 + dyn] = v
    elif i == 4:
        emit(0, 1, m[0] + v)
        m[1 + dyn] = v
    elif i == 1:
        m[2 + dyn] = v
        if acc & 1:
            m[0 + dyn] = m[0] - v
    elif i == 0:
        m[3 + dyn] = v
        if acc & 2:
            m[1 + dyn] = v - m[1]
    elif i == 5:
        emit(1, 1, (m[0] if acc & 1 else m[0] - m[2]) + (m[3] + v))
    elif i == 3:
        emit(1, 0, m[2] + v)
        m[0 + dyn] = v
    else:
        emit(0, 0, (m[1] if acc & 2 else m[3] - m[1]) + (m[0] + v))

def kernel(gw, shk, ssmd, f_ref, g_ref, aq_hbm, ak_hbm, av_hbm, ssmk_hbm, c_hbm, wq_hbm, wk_hbm, wv_hbm, wo_hbm,
           o_hbm,
           x_s, c_s, xab, cab, wq_b, wk_b, wv_b, h0b, h1b, arb, s0, s1, mkv, mi, mq, gate_s, ak_b, av_b, hk_b, wo_b, o_b, uf, hf, zf, ga_s, dd_s, gw_s, wp,
           sem_x, sem_w, sem_t, sem_o):

    def wcopies(p, slot):
        return [pltpu.make_async_copy(src.bitcast(U32).at[:, p, :], dst.at[slot], sem_w.at[i, slot])
                for i, (src, dst) in enumerate(((wk_hbm, wk_b), (wv_hbm, wv_b), (wq_hbm, wq_b)))]

    def tcopies(t, slot):
        cps = [pltpu.make_async_copy(ssmk_hbm.at[pl.ds(pl.multiple_of(t * 256, 256), 256), :], hk_b.at[slot], sem_t.at[0, slot])]
        for c in range(2):
            cs = pl.ds(pl.multiple_of((2 * t + c) * 128, 128), 128)
            cps += [pltpu.make_async_copy(ak_hbm.at[0, :, cs], ak_b.at[slot, c, pl.ds(16, S)], sem_t.at[1 + c, slot]),
                    pltpu.make_async_copy(av_hbm.at[0, :, cs], av_b.at[slot, c], sem_t.at[3 + c, slot]),
                    pltpu.make_async_copy(wo_hbm.at[:, :, cs], wo_b.at[slot, c], sem_t.at[5 + c, slot])]
        return cps

    def ocopy(t, slot, c):
        cs = pl.ds(pl.multiple_of((2 * t + c) * 128, 128), 128)
        return pltpu.make_async_copy(o_b.at[slot, c], o_hbm.at[0, :, cs], sem_o.at[c, slot])

    RB = 128
    def rcopies(src, dst, which, r):
        rows = lambda a: pl.ds(pl.multiple_of(a * QS + r * RB, RB), RB)
        return [pltpu.make_async_copy(src.at[0, rows(a)], dst.at[rows(a)], sem_x.at[which, a, r]) for a in range(4)]
    ccopies = lambda r: rcopies(c_hbm, c_s, 0, r)
    xcopies = lambda r: rcopies(aq_hbm, x_s, 1, r)
    w0 = wcopies(0, 0)
    for cp in w0[:2] + ccopies(0):
        cp.start()

    qscale = float((HD ** -0.5) * np.log2(np.e))

    ar, xa, ca = arb.bitcast(U32), xab.bitcast(U32), cab.bitcast(U32)
    h0, h1 = h0b.bitcast(U32), h1b.bitcast(U32)

    def qkv_load(slot, which, hh, r0, n):
        rs = slice(r0 // 2, (r0 + n) // 2)
        return h0[which, rs] if hh == 0 else h1[slot, which, rs]

    def qkv_store(slot, which, hh, r0, val):
        rs = pl.ds(pl.multiple_of(r0, 32), val.shape[0])
        if hh == 0:
            h0b[which, rs] = val.astype(BF16)
        else:
            h1b[slot, which, rs] = val.astype(BF16)

    def proj_pieces(slot, dyn):
        def q_piece(i):
            def f():
                blk = lambda r, c: (lambda: halves(wq_b[slot, r * (DM // 2):(r + 1) * (DM // 2)])[c])
                w = rhs_ops(blk(0, 0), blk(0, 1), blk(1, 0), blk(1, 1))[i]().astype(BF16)
                a = jnp.concatenate([xa[i, b] for b in range(DM // 256)], axis=1)
                emit = lambda r, c, val: qkv_store(slot, 0, c, r * HS, val * qscale)
                consume(i, dot(unpack(a), w), emit, mq, dyn, AQ)
            return f
        def kv_piece(i):
            def f():
                def outer(kk, nn):
                    raw = lambda r, c: (lambda: halves((wk_b, wv_b)[nn][slot, (2 * r + kk) * 128:(2 * r + kk + 1) * 128])[c])
                    return rhs_ops(raw(0, 0), raw(0, 1), raw(1, 0), raw(1, 1))[i]
                rops = rhs_ops(outer(0, 0), outer(0, 1), outer(1, 0), outer(1, 1))
                def inner_emit(r2, c2, v):
                    def emit(r, c, val):
                        for t in range(0, QS, 128):
                            blk = val[t:t + 128]
                            qkv_store(slot, 1 + c2, c, r * HS + r2 * QS + t, blk.T if c2 else blk)
                    consume(i, v, emit, mkv.at[:, c2, r2 * QS:(r2 + 1) * QS], dyn, AO)
                if RC == 0:
                    for j in PORD:
                        w = rops[j]().astype(BF16)
                        v = jnp.concatenate([dot(unpack(ca[i, j, a * QS // 8:(a + 1) * QS // 8]), w) for a in range(4)], axis=0)
                        consume(j, v, inner_emit, mi, dyn, AI)
                    return
                for j in PORD:
                    wp[dyn, j * 128:(j + 1) * 128] = rops[j]().astype(BF16)
                for t0 in range(0, QS, 128):
                    blocks = {}
                    for a in range(t0, t0 + 128, RC):
                        v = {j: dot(unpack(ca[i, j, a // 2:(a + RC) // 2]), unpack(wp.bitcast(U32)[0, j * 64:(j + 1) * 64]))
                             for j in PORD}
                        for key, val in (((0, 1), v[2] + v[4]), ((1, 1), (v[2] - v[1]) + (v[0] + v[5])),
                                         ((1, 0), v[1] + v[3]), ((0, 0), (v[0] - v[4]) + (v[3] + v[6]))):
                            r2, c2 = key
                            def emit(r, c, val, r2=r2, c2=c2, a=a):
                                if c2 == 0:
                                    qkv_store(slot, 1, c, r * HS + r2 * QS + a, val)
                                else:
                                    blocks.setdefault((r, c, r2), []).append(val)
                            consume(i, val, emit, mkv.at[:, c2, r2 * QS + a:r2 * QS + a + RC], dyn, AO)
                    for (r, c, r2), vals in blocks.items():
                        qkv_store(slot, 2, c, r * HS + r2 * QS + t0, jnp.concatenate(vals, axis=0).T)
            return f
        return [kv_piece(i) for i in PORD], [q_piece(i) for i in PORD]

    def scores(slot, hh, i, buf, dyn):
        L = (i + 1) * BQ
        q = unpack(qkv_load(slot, 0, hh, i * BQ, BQ))
        m = None
        n = L // 4
        for a in range(4):
            st = dot_nt(unpack(qkv_load(slot, 1, hh, a * n, n)), q)
            d0 = max(L - BQ - a * n, 0)
            if d0 < n:
                row = lax.broadcasted_iota(jnp.int32, (n - d0, BQ), 0) + (a * n + d0 - (L - BQ))
                col = lax.broadcasted_iota(jnp.int32, (n - d0, BQ), 1)
                dg = jnp.where(row <= col, st[d0:], -1e9)
                st = dg if d0 == 0 else jnp.concatenate([st[:d0], dg], axis=0)
            (s0, s1)[buf][pl.ds(pl.multiple_of(a * n + dyn, 32), n)] = st
            ma = jnp.max(st.reshape(n // 8, 8, BQ), axis=0)
            m = ma if m is None else jnp.maximum(m, ma)
        return jnp.broadcast_to(jnp.max(m, axis=0, keepdims=True), (8, BQ))

    def weighted(slot, hh, i, buf, m, never, dyn2):
        l = ot = None
        for t0 in range(0, i + 1, GT):
            nt = min(GT, i + 1 - t0)
            pj = jnp.exp2((s0, s1)[buf][t0 * BQ:(t0 + nt) * BQ] - jnp.tile(m, (nt * BQ // 8, 1)))
            lj = jnp.sum(pj.reshape(nt * BQ // 8, 8, BQ), axis=0)
            if LAG and l is not None:
                pj = jnp.concatenate([jnp.where(never, l, pj[:8]), pj[8:]], axis=0)
            l = lj if l is None else l + lj
            pt = pj.astype(BF16)
            ns = 1 if nt == 4 else 2 if nt == 2 else 4
            if SPL and t0 < (i + 1) // SPL * SPL:
                ns = 4 // SPL
            parts = []
            for a in range(ns):
                vt = jnp.concatenate([qkv_load(slot, 2, hh, t * 128 + a * HD // ns, HD // ns)
                                      for t in range(t0, t0 + nt)], axis=1)
                parts.append(dot(unpack(vt), pt))
            d = jnp.concatenate(parts, axis=0)
            ot = d if ot is None else ot + d
        l = jnp.sum(l, axis=0, keepdims=True)
        r = pl.reciprocal(l, approx=True)
        r = r * (2.0 - l * r)
        return (ot * r).T

    def attention(p, slot, pieces, UO=UO, REV=REV, CLAG=CLAG, U1=0):
        pieces = list(pieces)
        dyn = lax.shift_right_logical(p, 8)
        never = jnp.broadcast_to(p, (8, BQ)) < 0
        dyn2 = lax.shift_right_logical(p, 9)
        tmp = lambda i: pl.ds(pl.multiple_of(A_TMP + i * BQ + dyn, 64), BQ)
        gs = lambda hh: range(NG) if not (REV >> hh) & 1 else reversed(range(NG))
        units = [(hh, g + a * NG) for hh in range(2) for g in gs(hh) for a in range(2)]
        if UO == 1:
            units[:2 * NG] = [(0, i) for g in range(NG) for i in (g, 2 * NG - 1 - g)]
        elif UO == 2:
            units[:2 * NG] = [(0, i) for i in range(2 * NG)]
        elif UO == 3:
            units[:2 * NG] = [(0, i) for g in range(NG) for i in (2 * NG - 1 - g, g)]
        if U1 == 1:
            units[2 * NG:] = [(1, g + a * NG) for g in gs(1) for a in (1, 0)]
        slot1 = lambda i: 2 * NG + (i % 2) * 2 + i // NG

        nxt = scores(slot, *units[0], 0, dyn)
        tok = {}
        for u, (hh, i) in enumerate(units):
            cur = nxt
            here = pieces and (u in SL0 or u - 2 * NG in SL1)
            if here and u in PB:
                pieces.pop(0)()
            if u + 1 < len(units):
                nxt = scores(slot, *units[u + 1], (u + 1) % 2, dyn)
            if here and u not in PB:
                pieces.pop(0)()
            if u in tok:
                cur = jnp.where(never, tok[u], cur)
            o = weighted(slot, hh, i, u % 2, cur, never, dyn2)
            if hh == 0 or u % 2 == 0:
                ar[tmp(i if hh == 0 else slot1(i))] = pltpu.bitcast(o, U32)
            else:
                g = i % NG
                for rc in range(0, BQ, CCH):
                    a11, a12, a21 = (pltpu.bitcast(ar[pl.ds(pl.multiple_of(A_TMP + t * BQ + rc + dyn, 16), CCH)], F32)
                                     for t in (g, slot1(units[u - 1][1]), g + NG))
                    a12, a22 = (a12, o[rc:rc + CCH]) if i >= NG else (o[rc:rc + CCH], a12)
                    for j, op in enumerate(lhs_ops(lambda: a11, lambda: a12, lambda: a21, lambda: a22)):
                        base = A_CT + (j * NP + p) * (HS // 2) + g * (BQ // 2)
                        arb[pl.ds(pl.multiple_of(base * 2 + rc, 16), CCH)] = op().astype(BF16)
            if CLAG and hh == 1 and u % 2:
                tok[u + CLAG] = pltpu.bitcast(ar[pl.ds(pl.multiple_of(A_TMP + dyn2, 8), 8)], F32)
        while pieces:
            pieces.pop(0)()

    def x_combos(r0, n):
        rows = [pl.ds(pl.multiple_of(a * HS + r0, n), n) for a in range(2)]
        gl = [None, None]
        for b in range(NT // 2):
            blk = [[x_s[rows[a], (c * NT // 2 + b) * 128:(c * NT // 2 + b + 1) * 128].astype(F32) for c in range(2)]
                   for a in range(2)]
            ops = lhs_ops(lambda: blk[0][0], lambda: blk[0][1], lambda: blk[1][0], lambda: blk[1][1])
            for j, op in enumerate(ops):
                xab[j, b, rows[0]] = op().astype(BF16)
            for a in range(2):
                for c in range(2):
                    term = blk[a][c] * gw_s[c * NT // 2 + b, 0:n]
                    gl[a] = term if gl[a] is None else gl[a] + term
        for a in range(2):
            gate_s[rows[a]] = jnp.broadcast_to(jax.nn.sigmoid(jnp.sum(gl[a], axis=-1, keepdims=True)), (n, 128))

    def c_combos(r0, n):
        quarter = [c_s[pl.ds(pl.multiple_of(a * QS + r0, n), n)].astype(F32) for a in range(4)]
        for i in range(7):
            def outer(r2, kk):
                raw = lambda r, c: (lambda: quarter[2 * r + r2][:, (2 * c + kk) * 128:(2 * c + kk + 1) * 128])
                val = lhs_ops(raw(0, 0), raw(0, 1), raw(1, 0), raw(1, 1))[i]()
                return lambda: val
            for j, op in enumerate(lhs_ops(outer(0, 0), outer(0, 1), outer(1, 0), outer(1, 1))):
                cab[i, j, pl.ds(pl.multiple_of(r0, n), n)] = op().astype(BF16)

    dd_s[...] = ssmd[...].astype(F32)
    ak_b[:, :, 0:16] = jnp.zeros((2, 2, 16, 128), BF16)
    for b in range(NT):
        gw_s[b] = jnp.broadcast_to(gw[...].astype(F32)[b:b + 1], (16, 128))
    NC = QS // RB
    for cp in w0[:2] + ccopies(0):
        cp.wait()
    for cp in w0[2:] + [cp for r in range(1, NC) for cp in ccopies(r)]:
        cp.start()
    rows_of = lambda ref, r: unpack(ref.bitcast(U32)[pl.ds(pl.multiple_of(r // 2, RB // 2), RB // 2)])
    def pro_kv(r, carry):
        r0 = r * RB
        @pl.when(r > 0)
        def _():
            for cp in ccopies(r):
                cp.wait()
            for cp in xcopies(r - 1):
                cp.start()
        w = unpack(jnp.concatenate([wp.bitcast(U32)[n, 0:DC // 2] for n in range(4)], axis=1))
        for a in range(4):
            val = dot(rows_of(c_s, a * QS + r0), w)
            for n in range(4):
                blk = val[:, n * 128:(n + 1) * 128]
                qkv_store(0, 1 + n // 2, n % 2, a * QS + r0, blk.T if n // 2 else blk)
            for b in range(a * RB // 4, (a + 1) * RB // 4, 16):
                c_combos(r0 + b, 16)
        return carry
    def pro_q(r, carry):
        r0 = r * RB
        for cp in xcopies(r):
            cp.wait()
        w = unpack(jnp.concatenate([wp.bitcast(U32)[n] for n in range(2)], axis=1))
        for a in range(4):
            val = dot(rows_of(x_s, a * QS + r0), w) * qscale
            for hh in range(2):
                qkv_store(0, 0, hh, a * QS + r0, val[:, hh * 128:(hh + 1) * 128])
            for b in range(a % 2 * RB // 2, (a % 2 + 1) * RB // 2, 16):
                x_combos(a // 2 * QS + r0 + b, 16)
        return carry
    for n, w in enumerate(halves(wk_b[0]) + halves(wv_b[0])):
        wp[n, 0:DC] = w.astype(BF16)
    lax.fori_loop(0, NC, pro_kv, 0) if not NOPRO else None
    w0[2].wait()
    for cp in xcopies(NC - 1):
        cp.start()
    for cp in wcopies(1, 1):
        cp.start()
    for n, w in enumerate(halves(wq_b[0])):
        wp[n] = w.astype(BF16)
    lax.fori_loop(0, NC, pro_q, 0) if not NOPRO else None

    def pair_step(p, carry):
        slot = p % 2
        for cp in wcopies(p + 1, 1 - slot):
            cp.wait()
        @pl.when(p + 2 < NP)
        def _():
            for cp in wcopies(p + 2, slot):
                cp.start()
        @pl.when(p == NP - 2)
        def _():
            for cp in tcopies(0, 0):
                cp.start()
        kvp, qp = proj_pieces(1 - slot, lax.shift_right_logical(p, 8))
        attention(p, slot, [f for pair in (zip(kvp, qp) if PO == 0 else zip(qp, kvp)) for f in pair], U1=U1)
        return carry + 1
    last = lax.fori_loop(0, NP - 1, pair_step if not ONLYL else (lambda p, c: c + pl.program_id(0) if 0 else c + 1), 0) if not ONLY2 else None
    if ONLY1:
        return
    if not ONLY2:
        attention(last, (NP - 1) % 2, [], *LK)

    if ONLYL:
        return
    def tile_step(t, carry):
        slot = t % 2
        for cp in tcopies(t, slot):
            cp.wait()
        def prefetch():
            @pl.when(t + 1 < NT // 2)
            def _():
                for cp in tcopies(t + 1, 1 - slot):
                    cp.start()
            @pl.when(t >= 2)
            def _():
                for c in range(2):
                    ocopy(t - 2, slot, c).wait()
        if PF < 0:
            prefetch()

        KC = 4
        def oprod(i):
            acc = None
            for j0 in range(0, NP, KC):
                def wblk(r, c):
                    return lambda: jnp.concatenate(
                        [unpack(wo_b.bitcast(U32)[slot, c, 2 * j + r]) for j in range(j0, j0 + KC)], axis=0).astype(F32)
                w = rhs_ops(wblk(0, 0), wblk(0, 1), wblk(1, 0), wblk(1, 1))[i]().astype(BF16)
                a = jnp.concatenate([ar[pl.ds(A_CT + (i * NP + j) * (HS // 2), HS // 2)] for j in range(j0, j0 + KC)], axis=1)
                d = dot(unpack(a), w)
                acc = d if acc is None else acc + d
                yield acc
        def emit_o(r, c, val):
            rs = slice(r * HS, (r + 1) * HS)
            o_b[slot, c, rs] = (ga_s[c, rs] + (1.0 - gate_s[rs]) * val).astype(BF16)
        def opieces():
            m = {}
            def second_tile():
                emit_o(0, 1, m[2] + m[4])
                emit_o(1, 1, (m[0] + m[5]) + (m[2] - m[1]))
                ocopy(t, slot, 1).start()
            for i in PORD:
                for acc in oprod(i):
                    m[i] = acc
                    yield
                if EE and i == PORD[3 + EE]:
                    second_tile()
            yield
            if not EE:
                second_tile()
            emit_o(1, 0, m[1] + m[3])
            emit_o(0, 0, (m[0] + m[6]) + (m[3] - m[4]))
            ocopy(t, slot, 0).start()
        gen = opieces()
        def piece(n=1):
            for _ in range(n * 4 // KC):
                next(gen)

        rows = lax.broadcasted_iota(jnp.int32, (8, 128), 0)
        sgn = (1 - 2 * (rows & 1)).astype(F32)
        Fm = f_ref[...]
        Gm = g_ref[...]
        for c, (n0, n1, n2, n3, fts) in zip(CO, PP):
            cs = slice(c * 128, (c + 1) * 128)
            piece(n0)
            if c == PF:
                prefetch()
            sh = shk[2 * t + c].astype(F32)
            if KVB < 2:
                kk = unpack(ak_b.bitcast(U32)[slot, c, 8:8 + S // 2]).astype(F32)
                ksf = kk * sh[0:1, :]
                for j in range(1, KS):
                    kr = pltpu.roll(kk, j, 0)
                    kr = jnp.concatenate([jnp.where(rows >= j, kr[:8], 0.0), kr[8:]], axis=0)
                    ksf = ksf + kr * sh[j:j + 1, :]
                kv = (ksf * unpack(av_b.bitcast(U32)[slot, c]).astype(F32))
            else:
                aku = ak_b.bitcast(U32)
                ke, ko = halves(aku[slot, c, 8:8 + S // 2])
                ke1, ko1 = halves(aku[slot, c, 7:7 + S // 2])
                ko2 = halves(aku[slot, c, 6:6 + S // 2])[1]
                ve, vo = halves(av_b.bitcast(U32)[slot, c])
                even = (ke * sh[0:1] + ko1 * sh[1:2] + ke1 * sh[2:3] + ko2 * sh[3:4]) * ve
                odd = (ko * sh[0:1] + ke * sh[1:2] + ko1 * sh[2:3] + ke1 * sh[3:4]) * vo
                if KVB == 2:
                    bits = lambda a: pltpu.bitcast(a.astype(BF16).astype(F32), U32)
                    kv = unpack((bits(even) >> 16) | bits(odd))
                else:
                    kv = unpack(pltpu.pack_elementwise([even, odd], packed_dtype=BF16))
            for j in range(0, NCH, 4):
                r = dot_nt(Fm, jnp.concatenate([hk_b[slot, cs, (j + a) * C:(j + a + 1) * C] for a in range(4)], axis=0))
                for a in range(4):
                    hf[j + a] = r[:, a * 128:(a + 1) * 128]
            piece(n1)
            for j in range(0, NCH, 4):
                r = dot(Fm, jnp.concatenate([kv[(j + a) * C:(j + a + 1) * C] for a in range(4)], axis=1).astype(BF16))
                for a in range(4):
                    uf[j + a] = r[:, a * 128:(a + 1) * 128]
            ga_s[c] = kv.astype(F32) * dd_s[pl.ds(2 * t + c, 1)]
            piece(n2)
            for ft in range(C // 8):
                re = slice(ft * 8, ft * 8 + 8)
                im = slice(C + ft * 8, C + ft * 8 + 8)
                sub, add = (jnp.subtract, jnp.add) if ft < C // 16 else (jnp.add, jnp.subtract)
                hc = [hf[0, re]] + [sub(hf[m, re], hf[m - 1, im]) for m in range(1, NCH)]
                hd = [hf[0, im]] + [add(hf[m, im], hf[m - 1, re]) for m in range(1, NCH)]
                ua = [uf[j, re] for j in range(NCH)]
                ub = [uf[j, im] for j in range(NCH)]
                def toep(u, h):
                    out = []
                    for i in range(NCH):
                        a = u[0] * h[i]
                        for j in range(1, i + 1):
                            a = a + u[j] * h[i - j]
                        out.append(a)
                    return out
                k1 = toep([a + b for a, b in zip(ua, ub)], hc)
                k2 = toep(ua, [d - c_ for c_, d in zip(hc, hd)])
                k3 = toep(ub, [d + c_ for c_, d in zip(hc, hd)])
                for i in range(NCH):
                    zf[i, re] = k1[i] - k3[i]
                    zf[i, im] = k1[i] + k2[i]
                if ft in fts:
                    piece()
            xcs = pl.ds(pl.multiple_of((2 * t + c) * 128, 128), 128)
            for j in range(0, NCH, 4):
                r = dot(Gm, jnp.concatenate([zf[j + a] for a in range(4)], axis=1).astype(BF16))
                for a in range(4):
                    ts = slice((j + a) * C, (j + a + 1) * C)
                    y = r[:, a * 128:(a + 1) * 128] + ga_s[c, ts]
                    ga_s[c, ts] = gate_s[ts] * (x_s[ts, xcs].astype(F32) * y)
                if j == 4:
                    piece(n3)
        for _ in gen:
            pass
        return carry
    lax.fori_loop(0, NT // 2, tile_step, 0)
    for t in range(NT // 2 - 2, NT // 2):
        for c in range(2):
            ocopy(t, t % 2, c).wait()

@jax.jit
def pallas_gated_mix__ssm_conv_h3__compressed_kv_cla__prompt_kernel(
        A_q, A_k, A_v, A_shift_k, A_ssm_k, A_ssm_D, B_x, B_c_kv, B_w_q, B_w_uk, B_w_uv, B_w_o, gate_w):
    any_ = pl.BlockSpec(memory_space=pl.ANY)
    vm = pl.BlockSpec(memory_space=pltpu.VMEM)
    out = pl.pallas_call(
        kernel,
        in_specs=[vm] * 5 + [any_] * 9,
        out_specs=any_,
        out_shape=jax.ShapeDtypeStruct((1, S, DM), BF16),
        scratch_shapes=[
            pltpu.VMEM((S, DM), BF16), pltpu.VMEM((S, DC), BF16),
            pltpu.VMEM((7, DM // 256, HS, 128), BF16), pltpu.VMEM((7, 7, QS, 128), BF16),
            pltpu.VMEM((2, DM, 128), U32), pltpu.VMEM((2, DC, 128), U32), pltpu.VMEM((2, DC, 128), U32),
            pltpu.VMEM((3, S, 128), BF16), pltpu.VMEM((2, 3, S, 128), BF16), pltpu.VMEM((2 * A_END, 128), BF16),
            pltpu.VMEM((S, 128), F32), pltpu.VMEM((S, 128), F32), pltpu.VMEM((4, 2, HS, 128), F32), pltpu.VMEM((4, QS, 128), F32), pltpu.VMEM((4, HS, 128), F32),
            pltpu.VMEM((S, 128), F32),
            pltpu.VMEM((2, 2, S + 16, 128), BF16), pltpu.VMEM((2, 2, S, 128), BF16), pltpu.VMEM((2, 256, S), BF16),
            pltpu.VMEM((2, 2, H, HD, 128), BF16), pltpu.VMEM((2, 2, S, 128), BF16),
            pltpu.VMEM((NCH, 2 * C, 128), F32), pltpu.VMEM((NCH, 2 * C, 128), F32), pltpu.VMEM((NCH, 2 * C, 128), F32),
            pltpu.VMEM((2, S, 128), F32), pltpu.VMEM((NT, 128), F32), pltpu.VMEM((NT, 16, 128), F32), pltpu.VMEM((4, DM, 128), BF16),
            pltpu.SemaphoreType.DMA((2, 4, 4)), pltpu.SemaphoreType.DMA((3, 2)), pltpu.SemaphoreType.DMA((7, 2)),
            pltpu.SemaphoreType.DMA((2, 2)),
        ],
        compiler_params=pltpu.CompilerParams(vmem_limit_bytes=120 * 1024 * 1024),
    )(gate_w.reshape(NT, 128), A_shift_k.T.reshape(KS, NT, 128).transpose(1, 0, 2), A_ssm_D.reshape(NT, 128), _F, _G,
      A_q, A_k, A_v, A_ssm_k, B_c_kv, B_w_q, B_w_uk, B_w_uv, B_w_o)
    return out
```

```python
import jax
import jax.experimental.pallas as pl
import jax.experimental.pallas.tpu as pltpu
import jax.numpy as jnp
import numpy as np
from jax import lax

S, DM, H, HD, DC, KS = 2048, 1024, 32, 128, 512, 4
NP = H // 2
NT = DM // 128
HS, QS = S // 2, S // 4
C = 128
NCH = S // C
BQ = 128
NG = HS // BQ
RB = 128
NC = QS // RB
F32, BF16, U32 = jnp.float32, jnp.bfloat16, jnp.uint32

A_TMP = 0
A_CT = A_TMP + S + 4 * BQ
A_END = A_CT + 7 * NP * (HS // 2)

PORD = (2, 4, 1, 0, 5, 3, 6)

PIECE_AT = (0, 1, 2, 3, 4, 6, 8, 9, 11, 13, 26, 28, 30)
PIECE_FIRST = (2, 11, 26)
TILE_PLAN = ((1, (1, 1, 2, 3), (1, 3, 5, 7, 9, 11, 13, 15)),
             (0, (2, 2, 2, 1), (0, 2, 3, 4, 5, 8)))


def _dft_consts():
    f = np.concatenate([np.arange(0, C, 2), np.arange(1, C, 2)])[:, None] + 0.5
    ang = 2 * np.pi * f * np.arange(C)[None, :] / (2 * C)
    fwd = np.concatenate([np.cos(ang), -np.sin(ang)], 0)
    inv = np.concatenate([np.cos(ang).T, -np.sin(ang).T], 1) / C
    return fwd.astype(BF16), inv.astype(BF16)


_FWD, _INV = _dft_consts()


def dot(a, b):
    return jnp.dot(a, b, preferred_element_type=F32)


def dot_nt(a, b):
    return lax.dot_general(a, b, (((1,), (1,)), ((), ())), preferred_element_type=F32)


def unpack(w):
    return pltpu.bitcast(w, BF16)


def halves(w):
    return pltpu.bitcast(w << 16, F32), pltpu.bitcast(w & jnp.uint32(0xFFFF0000), F32)


def lhs_ops(a11, a12, a21, a22):
    return [lambda: a11() + a22(), lambda: a21() + a22(), a11, a22,
            lambda: a11() + a12(), lambda: a21() - a11(), lambda: a12() - a22()]


def rhs_ops(b11, b12, b21, b22):
    return [lambda: b11() + b22(), b11, lambda: b12() - b22(), lambda: b21() - b11(),
            b22, lambda: b11() + b12(), lambda: b21() + b22()]


def consume(i, v, emit, m, dyn):
    if i == 2:
        m[0 + dyn] = v
    elif i == 4:
        emit(0, 1, m[0] + v)
        m[1 + dyn] = v
    elif i == 1:
        m[2 + dyn] = v
    elif i == 0:
        m[3 + dyn] = v
    elif i == 5:
        emit(1, 1, (m[0] - m[2]) + (m[3] + v))
    elif i == 3:
        emit(1, 0, m[2] + v)
        m[0 + dyn] = v
    else:
        emit(0, 0, (m[3] - m[1]) + (m[0] + v))


def kernel(gw, shk, ssmd, f_ref, g_ref, aq_hbm, ak_hbm, av_hbm, ssmk_hbm, c_hbm, wq_hbm, wk_hbm, wv_hbm, wo_hbm,
           o_hbm,
           x_s, c_s, xab, cab, wq_b, wk_b, wv_b, wp, h0b, h1b, arb, s0, s1, mkv, mq,
           gate_s, gw_s, dd_s, ak_b, av_b, hk_b, wo_b, o_b, uf, hf, zf, ga_s,
           sem_x, sem_w, sem_t, sem_o):
    ar, xa, ca, h0, h1 = (ref.bitcast(U32) for ref in (arb, xab, cab, h0b, h1b))
    qscale = float(HD ** -0.5 * np.log2(np.e))

    def wcopies(p, slot):
        return [pltpu.make_async_copy(src.bitcast(U32).at[:, p, :], dst.at[slot], sem_w.at[i, slot])
                for i, (src, dst) in enumerate(((wk_hbm, wk_b), (wv_hbm, wv_b), (wq_hbm, wq_b)))]

    def tcopies(t, slot):
        chans = pl.ds(pl.multiple_of(t * 256, 256), 256)
        cps = [pltpu.make_async_copy(ssmk_hbm.at[chans, :], hk_b.at[slot], sem_t.at[0, slot])]
        for c in range(2):
            cs = pl.ds(pl.multiple_of((2 * t + c) * 128, 128), 128)
            cps += [pltpu.make_async_copy(ak_hbm.at[0, :, cs], ak_b.at[slot, c, pl.ds(16, S)], sem_t.at[1 + c, slot]),
                    pltpu.make_async_copy(av_hbm.at[0, :, cs], av_b.at[slot, c], sem_t.at[3 + c, slot]),
                    pltpu.make_async_copy(wo_hbm.at[:, :, cs], wo_b.at[slot, c], sem_t.at[5 + c, slot])]
        return cps

    def ocopy(t, slot, c):
        cs = pl.ds(pl.multiple_of((2 * t + c) * 128, 128), 128)
        return pltpu.make_async_copy(o_b.at[slot, c], o_hbm.at[0, :, cs], sem_o.at[c, slot])

    def rcopies(src, dst, which, r):
        rows = lambda a: pl.ds(pl.multiple_of(a * QS + r * RB, RB), RB)
        return [pltpu.make_async_copy(src.at[0, rows(a)], dst.at[rows(a)], sem_x.at[which, a, r]) for a in range(4)]

    ccopies = lambda r: rcopies(c_hbm, c_s, 0, r)
    xcopies = lambda r: rcopies(aq_hbm, x_s, 1, r)

    def start(cps):
        for cp in cps:
            cp.start()

    def wait(cps):
        for cp in cps:
            cp.wait()

    def qkv_load(slot, which, hh, r0, n):
        rs = slice(r0 // 2, (r0 + n) // 2)
        return unpack(h0[which, rs] if hh == 0 else h1[slot, which, rs])

    def qkv_store(slot, which, hh, r0, val):
        rs = pl.ds(pl.multiple_of(r0, 32), val.shape[0])
        if hh == 0:
            h0b[which, rs] = val.astype(BF16)
        else:
            h1b[slot, which, rs] = val.astype(BF16)

    def proj_pieces(slot, dyn):
        def q_piece(i):
            def f():
                blk = lambda r, c: (lambda: halves(wq_b[slot, r * (DM // 2):(r + 1) * (DM // 2)])[c])
                w = rhs_ops(blk(0, 0), blk(0, 1), blk(1, 0), blk(1, 1))[i]().astype(BF16)
                a = jnp.concatenate([xa[i, b] for b in range(DM // 256)], axis=1)
                emit = lambda r, c, val: qkv_store(slot, 0, c, r * HS, val * qscale)
                consume(i, dot(unpack(a), w), emit, mq, dyn)
            return f

        def kv_piece(i):
            def f():
                def outer(kk, nn):
                    ref = (wk_b, wv_b)[nn]
                    raw = lambda r, c: (lambda: halves(ref[slot, (2 * r + kk) * 128:(2 * r + kk + 1) * 128])[c])
                    return rhs_ops(raw(0, 0), raw(0, 1), raw(1, 0), raw(1, 1))[i]
                rops = rhs_ops(outer(0, 0), outer(0, 1), outer(1, 0), outer(1, 1))
                for j in PORD:
                    wp[dyn, j * 128:(j + 1) * 128] = rops[j]().astype(BF16)
                for t0 in range(0, QS, 128):
                    vblocks = {}
                    for a in range(t0, t0 + 128, 64):
                        v = {j: dot(unpack(ca[i, j, a // 2:a // 2 + 32]), unpack(wp.bitcast(U32)[0, j * 64:(j + 1) * 64]))
                             for j in PORD}
                        for r2, c2, val in ((0, 1, v[2] + v[4]), (1, 1, (v[2] - v[1]) + (v[0] + v[5])),
                                            (1, 0, v[1] + v[3]), (0, 0, (v[0] - v[4]) + (v[3] + v[6]))):
                            def emit(r, c, out):
                                if c2 == 0:
                                    qkv_store(slot, 1, c, r * HS + r2 * QS + a, out)
                                else:
                                    vblocks.setdefault((r, c, r2), []).append(out)
                            consume(i, val, emit, mkv.at[:, c2, r2 * QS + a:r2 * QS + a + 64], dyn)
                    for (r, c, r2), vals in vblocks.items():
                        qkv_store(slot, 2, c, r * HS + r2 * QS + t0, jnp.concatenate(vals, axis=0).T)
            return f

        return [piece(i) for i in PORD for piece in (kv_piece, q_piece)]

    def scores(slot, hh, i, s_ref, dyn):
        L = (i + 1) * BQ
        q = qkv_load(slot, 0, hh, i * BQ, BQ)
        m = None
        n = L // 4
        for a in range(4):
            st = dot_nt(qkv_load(slot, 1, hh, a * n, n), q)
            d0 = max(L - BQ - a * n, 0)
            if d0 < n:
                row = lax.broadcasted_iota(jnp.int32, (n - d0, BQ), 0) + (a * n + d0 - (L - BQ))
                col = lax.broadcasted_iota(jnp.int32, (n - d0, BQ), 1)
                dg = jnp.where(row <= col, st[d0:], -1e9)
                st = dg if d0 == 0 else jnp.concatenate([st[:d0], dg], axis=0)
            s_ref[pl.ds(pl.multiple_of(a * n + dyn, 32), n)] = st
            ma = jnp.max(st.reshape(n // 8, 8, BQ), axis=0)
            m = ma if m is None else jnp.maximum(m, ma)
        return jnp.broadcast_to(jnp.max(m, axis=0, keepdims=True), (8, BQ))

    def weighted(slot, hh, i, s_ref, m):
        l = ot = None
        for t in range(i + 1):
            pj = jnp.exp2(s_ref[t * BQ:(t + 1) * BQ] - jnp.tile(m, (BQ // 8, 1)))
            lj = jnp.sum(pj.reshape(BQ // 8, 8, BQ), axis=0)
            l = lj if l is None else l + lj
            pt = pj.astype(BF16)
            d = jnp.concatenate([dot(qkv_load(slot, 2, hh, t * 128 + a * HD // 4, HD // 4), pt) for a in range(4)], axis=0)
            ot = d if ot is None else ot + d
        l = jnp.sum(l, axis=0, keepdims=True)
        r = pl.reciprocal(l, approx=True)
        r = r * (2.0 - l * r)
        return (ot * r).T

    def attention(p, slot, pieces, even_order):
        dyn = lax.shift_right_logical(p, 8)
        dyn2 = lax.shift_right_logical(p, 9)
        never = jnp.broadcast_to(p, (8, BQ)) < 0
        units = [(0, i) for i in even_order] + [(1, g + a * NG) for g in reversed(range(NG)) for a in (1, 0)]
        odd_tmp = lambda i: 2 * NG + (i % 2) * 2 + i // NG
        nxt = scores(slot, *units[0], s0, dyn)
        tok = {}
        for u, (hh, i) in enumerate(units):
            cur = nxt
            if pieces and u in PIECE_FIRST:
                pieces.pop(0)()
            if u + 1 < len(units):
                nxt = scores(slot, *units[u + 1], (s0, s1)[(u + 1) % 2], dyn)
            if pieces and u in PIECE_AT and u not in PIECE_FIRST:
                pieces.pop(0)()
            if u in tok:
                cur = jnp.where(never, tok[u], cur)
            o = weighted(slot, hh, i, (s0, s1)[u % 2], cur)
            if hh == 0 or u % 2 == 0:
                rows = pl.ds(pl.multiple_of(A_TMP + (i if hh == 0 else odd_tmp(i)) * BQ + dyn, 64), BQ)
                ar[rows] = pltpu.bitcast(o, U32)
            else:
                n = 32
                for rc in range(0, BQ, n):
                    a11, a22, a21 = (pltpu.bitcast(ar[pl.ds(pl.multiple_of(A_TMP + t * BQ + rc + dyn, 16), n)], F32)
                                     for t in (i, odd_tmp(i + NG), i + NG))
                    a12 = o[rc:rc + n]
                    for j, op in enumerate(lhs_ops(lambda: a11, lambda: a12, lambda: a21, lambda: a22)):
                        base = A_CT + (j * NP + p) * (HS // 2) + i * (BQ // 2)
                        arb[pl.ds(pl.multiple_of(base * 2 + rc, 16), n)] = op().astype(BF16)
                tok[u + 2] = pltpu.bitcast(ar[pl.ds(pl.multiple_of(A_TMP + dyn2, 8), 8)], F32)
        while pieces:
            pieces.pop(0)()

    def x_combos(r0, n):
        rows = [pl.ds(pl.multiple_of(a * HS + r0, n), n) for a in range(2)]
        gl = [None, None]
        for b in range(NT // 2):
            blk = [[x_s[rows[a], (c * NT // 2 + b) * 128:(c * NT // 2 + b + 1) * 128].astype(F32) for c in range(2)]
                   for a in range(2)]
            ops = lhs_ops(lambda: blk[0][0], lambda: blk[0][1], lambda: blk[1][0], lambda: blk[1][1])
            for j, op in enumerate(ops):
                xab[j, b, rows[0]] = op().astype(BF16)
            for a in range(2):
                for c in range(2):
                    term = blk[a][c] * gw_s[c * NT // 2 + b]
                    gl[a] = term if gl[a] is None else gl[a] + term
        for a in range(2):
            gate_s[rows[a]] = jnp.broadcast_to(jax.nn.sigmoid(jnp.sum(gl[a], axis=-1, keepdims=True)), (n, 128))

    def c_combos(r0, n):
        quarter = [c_s[pl.ds(pl.multiple_of(a * QS + r0, n), n)].astype(F32) for a in range(4)]
        for i in range(7):
            def outer(r2, kk):
                raw = lambda r, c: (lambda: quarter[2 * r + r2][:, (2 * c + kk) * 128:(2 * c + kk + 1) * 128])
                val = lhs_ops(raw(0, 0), raw(0, 1), raw(1, 0), raw(1, 1))[i]()
                return lambda: val
            for j, op in enumerate(lhs_ops(outer(0, 0), outer(0, 1), outer(1, 0), outer(1, 1))):
                cab[i, j, pl.ds(pl.multiple_of(r0, n), n)] = op().astype(BF16)

    rows_of = lambda ref, r: unpack(ref.bitcast(U32)[pl.ds(pl.multiple_of(r // 2, RB // 2), RB // 2)])

    def pro_kv(r, carry):
        r0 = r * RB

        @pl.when(r > 0)
        def _():
            wait(ccopies(r))
            start(xcopies(r - 1))
        w = unpack(jnp.concatenate([wp.bitcast(U32)[n, 0:DC // 2] for n in range(4)], axis=1))
        for a in range(4):
            val = dot(rows_of(c_s, a * QS + r0), w)
            for n in range(4):
                blk = val[:, n * 128:(n + 1) * 128]
                qkv_store(0, 1 + n // 2, n % 2, a * QS + r0, blk.T if n // 2 else blk)
            for b in range(a * RB // 4, (a + 1) * RB // 4, 16):
                c_combos(r0 + b, 16)
        return carry

    def pro_q(r, carry):
        r0 = r * RB
        wait(xcopies(r))
        w = unpack(jnp.concatenate([wp.bitcast(U32)[n] for n in range(2)], axis=1))
        for a in range(4):
            val = dot(rows_of(x_s, a * QS + r0), w) * qscale
            for hh in range(2):
                qkv_store(0, 0, hh, a * QS + r0, val[:, hh * 128:(hh + 1) * 128])
            for b in range(a % 2 * RB // 2, (a % 2 + 1) * RB // 2, 16):
                x_combos(a // 2 * QS + r0 + b, 16)
        return carry

    w0 = wcopies(0, 0)
    start(w0[:2] + ccopies(0))
    dd_s[...] = ssmd[...].astype(F32)
    ak_b[:, :, 0:16] = jnp.zeros((2, 2, 16, 128), BF16)
    for b in range(NT):
        gw_s[b] = jnp.broadcast_to(gw[...].astype(F32)[b:b + 1], (16, 128))
    wait(w0[:2] + ccopies(0))
    start(w0[2:] + [cp for r in range(1, NC) for cp in ccopies(r)])
    for n, w in enumerate(halves(wk_b[0]) + halves(wv_b[0])):
        wp[n, 0:DC] = w.astype(BF16)
    lax.fori_loop(0, NC, pro_kv, 0)
    wait(w0[2:])
    start(xcopies(NC - 1) + wcopies(1, 1))
    for n, w in enumerate(halves(wq_b[0])):
        wp[n] = w.astype(BF16)
    lax.fori_loop(0, NC, pro_q, 0)

    def pair_step(p, count):
        slot = p % 2
        wait(wcopies(p + 1, 1 - slot))

        @pl.when(p + 2 < NP)
        def _():
            start(wcopies(p + 2, slot))

        @pl.when(p == NP - 2)
        def _():
            start(tcopies(0, 0))
        attention(p, slot, proj_pieces(1 - slot, lax.shift_right_logical(p, 8)),
                  [i for g in range(NG) for i in (g, 2 * NG - 1 - g)])
        return count + 1

    last = lax.fori_loop(0, NP - 1, pair_step, 0)
    start(tcopies(1, 1))
    attention(last, (NP - 1) % 2, [], range(2 * NG))

    def tile_step(t, carry):
        slot = t % 2
        wait(tcopies(t, slot))

        @pl.when(t >= 2)
        def _():
            wait([ocopy(t - 2, slot, c) for c in range(2)])

        def mix(r, c, attn):
            rs = slice(r * HS, (r + 1) * HS)
            o_b[slot, c, rs] = (ga_s[c, rs] + (1.0 - gate_s[rs]) * attn).astype(BF16)

        def out_projection():
            m = {}
            for i in PORD:
                for j0 in range(0, NP, 4):
                    js = range(j0, j0 + 4)
                    blk = lambda r, c: (lambda: jnp.concatenate(
                        [unpack(wo_b.bitcast(U32)[slot, c, 2 * j + r]) for j in js], axis=0).astype(F32))
                    w = rhs_ops(blk(0, 0), blk(0, 1), blk(1, 0), blk(1, 1))[i]().astype(BF16)
                    a = jnp.concatenate([ar[pl.ds(A_CT + (i * NP + j) * (HS // 2), HS // 2)] for j in js], axis=1)
                    d = dot(unpack(a), w)
                    m[i] = d if j0 == 0 else m[i] + d
                    yield
                if i == 5:
                    mix(0, 1, m[2] + m[4])
                    mix(1, 1, (m[0] + m[5]) + (m[2] - m[1]))
                    ocopy(t, slot, 1).start()
            mix(1, 0, m[1] + m[3])
            mix(0, 0, (m[0] + m[6]) + (m[3] - m[4]))
            ocopy(t, slot, 0).start()

        steps = out_projection()

        def piece(n=1):
            for _ in range(n):
                next(steps)

        def toeplitz(u, h):
            out = []
            for i in range(NCH):
                acc = u[0] * h[i]
                for j in range(1, i + 1):
                    acc = acc + u[j] * h[i - j]
                out.append(acc)
            return out

        fwd, inv, aku = f_ref[...], g_ref[...], ak_b.bitcast(U32)
        for c, (n0, n1, n2, n3), piece_after in TILE_PLAN:
            piece(n0)
            sh = shk[2 * t + c].astype(F32)
            ke, ko = halves(aku[slot, c, 8:8 + S // 2])
            ke1, ko1 = halves(aku[slot, c, 7:7 + S // 2])
            ko2 = halves(aku[slot, c, 6:6 + S // 2])[1]
            ve, vo = halves(av_b.bitcast(U32)[slot, c])
            even = (ke * sh[0:1] + ko1 * sh[1:2] + ke1 * sh[2:3] + ko2 * sh[3:4]) * ve
            odd = (ko * sh[0:1] + ke * sh[1:2] + ko1 * sh[2:3] + ke1 * sh[3:4]) * vo
            bits = lambda a: pltpu.bitcast(a.astype(BF16).astype(F32), U32)
            kv = unpack((bits(even) >> 16) | bits(odd))
            cs = slice(c * 128, (c + 1) * 128)
            for j in range(0, NCH, 4):
                r = dot_nt(fwd, jnp.concatenate([hk_b[slot, cs, (j + a) * C:(j + a + 1) * C] for a in range(4)], axis=0))
                for a in range(4):
                    hf[j + a] = r[:, a * 128:(a + 1) * 128]
            piece(n1)
            for j in range(0, NCH, 4):
                r = dot(fwd, jnp.concatenate([kv[(j + a) * C:(j + a + 1) * C] for a in range(4)], axis=1))
                for a in range(4):
                    uf[j + a] = r[:, a * 128:(a + 1) * 128]
            ga_s[c] = kv.astype(F32) * dd_s[pl.ds(2 * t + c, 1)]
            piece(n2)
            for ft in range(C // 8):
                re = slice(ft * 8, ft * 8 + 8)
                im = slice(C + ft * 8, C + ft * 8 + 8)
                sub, add = (jnp.subtract, jnp.add) if ft < C // 16 else (jnp.add, jnp.subtract)
                hc = [hf[0, re]] + [sub(hf[m, re], hf[m - 1, im]) for m in range(1, NCH)]
                hd = [hf[0, im]] + [add(hf[m, im], hf[m - 1, re]) for m in range(1, NCH)]
                ua = [uf[j, re] for j in range(NCH)]
                ub = [uf[j, im] for j in range(NCH)]
                k1 = toeplitz([a + b for a, b in zip(ua, ub)], hc)
                k2 = toeplitz(ua, [d - e for e, d in zip(hc, hd)])
                k3 = toeplitz(ub, [d + e for e, d in zip(hc, hd)])
                for i in range(NCH):
                    zf[i, re] = k1[i] - k3[i]
                    zf[i, im] = k1[i] + k2[i]
                if ft in piece_after:
                    piece()
            xcs = pl.ds(pl.multiple_of((2 * t + c) * 128, 128), 128)
            for j in range(0, NCH, 4):
                r = dot(inv, jnp.concatenate([zf[j + a] for a in range(4)], axis=1).astype(BF16))
                for a in range(4):
                    ts = slice((j + a) * C, (j + a + 1) * C)
                    y = r[:, a * 128:(a + 1) * 128] + ga_s[c, ts]
                    ga_s[c, ts] = gate_s[ts] * (x_s[ts, xcs].astype(F32) * y)
                if j == 4:
                    piece(n3)
        for _ in steps:
            pass

        @pl.when(t + 2 < NT // 2)
        def _():
            start(tcopies(t + 2, slot))
        return carry

    lax.fori_loop(0, NT // 2, tile_step, 0)
    wait([ocopy(t, t % 2, c) for t in range(NT // 2 - 2, NT // 2) for c in range(2)])


@jax.jit
def pallas_gated_mix__ssm_conv_h3__compressed_kv_cla__prompt_kernel(
        A_q, A_k, A_v, A_shift_k, A_ssm_k, A_ssm_D, B_x, B_c_kv, B_w_q, B_w_uk, B_w_uv, B_w_o, gate_w):
    del B_x
    vmem = pltpu.VMEM
    return pl.pallas_call(
        kernel,
        in_specs=[pl.BlockSpec(memory_space=pltpu.VMEM)] * 5 + [pl.BlockSpec(memory_space=pl.ANY)] * 9,
        out_specs=pl.BlockSpec(memory_space=pl.ANY),
        out_shape=jax.ShapeDtypeStruct((1, S, DM), BF16),
        scratch_shapes=[
            vmem((S, DM), BF16), vmem((S, DC), BF16),
            vmem((7, DM // 256, HS, 128), BF16), vmem((7, 7, QS, 128), BF16),
            vmem((2, DM, 128), U32), vmem((2, DC, 128), U32), vmem((2, DC, 128), U32),
            vmem((4, DM, 128), BF16),
            vmem((3, S, 128), BF16), vmem((2, 3, S, 128), BF16),
            vmem((2 * A_END, 128), BF16),
            vmem((S, 128), F32), vmem((S, 128), F32),
            vmem((4, 2, HS, 128), F32), vmem((4, HS, 128), F32),
            vmem((S, 128), F32), vmem((NT, 16, 128), F32), vmem((NT, 128), F32),
            vmem((2, 2, S + 16, 128), BF16), vmem((2, 2, S, 128), BF16),
            vmem((2, 256, S), BF16), vmem((2, 2, H, HD, 128), BF16),
            vmem((2, 2, S, 128), BF16),
            vmem((NCH, 2 * C, 128), F32), vmem((NCH, 2 * C, 128), F32), vmem((NCH, 2 * C, 128), F32),
            vmem((2, S, 128), F32),
            pltpu.SemaphoreType.DMA((2, 4, NC)), pltpu.SemaphoreType.DMA((3, 2)),
            pltpu.SemaphoreType.DMA((7, 2)), pltpu.SemaphoreType.DMA((2, 2)),
        ],
        compiler_params=pltpu.CompilerParams(vmem_limit_bytes=120 * 1024 * 1024),
    )(gate_w.reshape(NT, 128), A_shift_k.T.reshape(KS, NT, 128).transpose(1, 0, 2), A_ssm_D.reshape(NT, 128),
      _FWD, _INV, A_q, A_k, A_v, A_ssm_k, B_c_kv, B_w_q, B_w_uk, B_w_uv, B_w_o)
```
